```python
import jax
import jax.numpy as jnp

def _softmax(x, axis=-1):
    return jax.nn.softmax(x, axis=axis)
def _gelu(x):
    return jax.nn.gelu(x, approximate=True)
def _silu(x):
    return jax.nn.silu(x)
def _sigmoid(x):
    return jax.nn.sigmoid(x)
def _layernorm(x, axis=-1, eps=1e-5):
    m = jnp.mean(x, axis=axis, keepdims=True)
    v = jnp.var(x, axis=axis, keepdims=True)
    return (x - m) / jnp.sqrt(v + eps)
def _scatter_add(tgt, idx, src, axis=0):
    return tgt.at[idx].add(src)
def _segment_sum(src, seg, n):
    return jax.ops.segment_sum(src, seg, n)
class _Rng:
    def __init__(self, key):
        self._k = key
    def _next(self):
        self._k, sub = jax.random.split(self._k)
        return sub
    def normal(self, shape):
        return jax.random.normal(self._next(), shape, dtype=jnp.bfloat16)
    def randint(self, lo, hi, shape):
        return jax.random.randint(self._next(), shape, lo, hi, dtype=jnp.int32)
    def uniform(self, shape, lo=0.0, hi=1.0):
        return jax.random.uniform(self._next(), shape, jnp.bfloat16, lo, hi)
    def permutation(self, n):
        return jax.random.permutation(self._next(), n)


kernel_name = 'sequential_preLN__sliding_local_dilated__moe_arch_mod__prompt'

def setup_inputs():
    _rng = _Rng(jax.random.key(int.from_bytes(__import__("os").urandom(4), "little")))
    _w = (lambda a: (lambda t: t.astype(jnp.bfloat16) if jnp.issubdtype(t.dtype, jnp.floating) else t)(jnp.asarray(a)))
    def _A_setup():
        B, S, D = 1, 2048, 640
        return {
            "x": _w((lambda *s: _rng.normal(s) * 0.05)(B, S, D)),
            "wqkv": _w((lambda *s: _rng.normal(s) * 0.05)(D, 3 * D)),
            "wo": _w((lambda *s: _rng.normal(s) * 0.05)(D, D)),
        }
    _A_in = _A_setup()

    def _B_setup():
        B, S, D, F, C = 1, 2048, 640, 1536, 1
        return {
            "x": _w((lambda *s: _rng.normal(s) * 0.05)(B, S, D)),
            "w_r": _w((lambda *s: _rng.normal(s) * 0.05)(D)),
            "w_gate": _w((lambda *s: _rng.normal(s) * 0.05)(D, F)),
            "w_up": _w((lambda *s: _rng.normal(s) * 0.05)(D, F)),
            "w_down": _w((lambda *s: _rng.normal(s) * 0.05)(F, D)),
        }
    _B_in = _B_setup()

    return {
        "A_x": _A_in["x"],
        "A_wqkv": _A_in["wqkv"],
        "A_wo": _A_in["wo"],
        "B_x": _B_in["x"],
        "B_w_r": _B_in["w_r"],
        "B_w_gate": _B_in["w_gate"],
        "B_w_up": _B_in["w_up"],
        "B_w_down": _B_in["w_down"],
    }

def reference(A_x, A_wqkv, A_wo, B_x, B_w_r, B_w_gate, B_w_up, B_w_down):
    def _A_ref(x, wqkv, wo):
        B, S, D = x.shape
        H = 32; Dh = D // H
        W, dil = 8, 2
        qkv = (lambda x, *d: x.transpose(*d))((x @ wqkv).reshape(B, S, 3, H, Dh), 2, 0, 3, 1, 4)
        q, k, v = qkv[0], qkv[1], qkv[2]
        scale = Dh ** -0.5
        pos = jnp.arange(S)
        off = jnp.arange(W) * dil
        idx = pos[:, None] - off[None, :]
        mask = idx >= 0
        idx_c = jnp.where(mask, idx, 0).reshape(-1)
        kg = k[:, :, idx_c, :].reshape(B, H, S, W, Dh)
        vg = v[:, :, idx_c, :].reshape(B, H, S, W, Dh)
        logits = jnp.einsum("bhsd,bhswd->bhsw", q, kg) * scale
        logits = jnp.where(mask[None, None, :, :], logits, -1e9)
        attn = _softmax(logits, axis=-1)
        o = jnp.einsum("bhsw,bhswd->bhsd", attn, vg)
        return (lambda x, *d: x.transpose(*d))(o, 0, 2, 1, 3).reshape(B, S, D) @ wo

    def _B_ref(x, w_r, w_gate, w_up, w_down):
        B, S, D = x.shape
        C = 1
        r = x @ w_r
        idx = jnp.argsort(-r, axis=-1)[:, :C]
        idx_e = jnp.repeat(idx.reshape(B, C, 1), D, axis=2)
        x_sel = jnp.take_along_axis(x, idx_e, axis=1)
        g = _silu(x_sel @ w_gate)
        u = x_sel @ w_up
        y = (g * u) @ w_down
        r_sel = _sigmoid(jnp.take_along_axis(r, idx, axis=1))
        y = y * r_sel.reshape(B, C, 1)
        b_off = (jnp.arange(B) * S).reshape(B, 1)
        flat_idx = (idx + b_off).reshape(B * C)
        zero = (x * 0.0).reshape(B * S, D)
        upd = _scatter_add(zero, flat_idx, y.reshape(B * C, D), axis=0)
        return x + upd.reshape(B, S, D)

    x = A_x
    h = x + _A_ref(_layernorm(x, axis=-1), A_wqkv, A_wo)
    h2 = h + _B_ref(_layernorm(h, axis=-1), B_w_r, B_w_gate, B_w_up, B_w_down)
    return h2
```

```python
import functools
import math
import jax
import jax.numpy as jnp
from jax.experimental import pallas as pl
from jax.experimental.pallas import tpu as pltpu

S, D, H, DH, F = 2048, 640, 32, 20, 1536
NW, DIL = 8, 2
HALO = 16
NJ = D // 128
EPS = 1e-5
QSCALE = (DH ** -0.5) * math.log2(math.e)
f32, bf16, u32, i32 = jnp.float32, jnp.bfloat16, jnp.uint32, jnp.int32


def make_kernel(T=128):
    NT = S // T

    def kernel(x_hbm, wqkv_hbm, wo_hbm, wr_hbm, wg_hbm, wu_hbm, wd_hbm, out_hbm,
               xs, wraw, wp, woraw, wof, wop, wr, wrf, wg, wu, wd,
               xn, qs, ks, vs, ls, os_, hs, outs, best,
               sem_x, sem_w, sem_o):
        def x_copy(i):
            return pltpu.make_async_copy(x_hbm.at[pl.ds(i * T, T)], xs.at[pl.ds(i * T, T)], sem_x.at[i])

        def w_copy(p):
            return pltpu.make_async_copy(wqkv_hbm.at[:, pl.ds(p * D, D)], wraw.at[:, pl.ds(p * D, D)], sem_w.at[p])

        wo_copy = pltpu.make_async_copy(wo_hbm, woraw, sem_w.at[3])
        wr_copy = pltpu.make_async_copy(wr_hbm, wr, sem_w.at[4])
        wg_copy = pltpu.make_async_copy(wg_hbm, wg, sem_w.at[5])
        wu_copy = pltpu.make_async_copy(wu_hbm, wu, sem_w.at[6])
        wd_copy = pltpu.make_async_copy(wd_hbm, wd, sem_w.at[7])

        def o_copy(i):
            return pltpu.make_async_copy(outs.at[pl.ds(i * T, T)], out_hbm.at[pl.ds(i * T, T)], sem_o.at[i])

        def row0(i):
            return i * T if isinstance(i, int) else pl.multiple_of(i * T, T)

        def prep_w(p):
            RB = 128
            lane = jax.lax.broadcasted_iota(i32, (RB // 2, 128), 1)
            r5 = (lane // 4) % 5
            g = lane // 32
            h = lane % 32
            for j in range(NJ):
                idx = (20 * h + 4 * j + g) % 128
                for rb in range(D // RB):
                    src = [pltpu.bitcast(wraw[rb * RB:(rb + 1) * RB, p * D + jj * 128: p * D + (jj + 1) * 128], u32)
                           for jj in range(NJ)]
                    t = src[4]
                    for jj in range(4):
                        t = jnp.where(r5 == (j - 2 * jj) % 5, src[jj], t)
                    t = jnp.take_along_axis(t, idx, axis=1)
                    wp[rb * RB // 2:(rb + 1) * RB // 2, p * D + j * 128: p * D + (j + 1) * 128] = t

        def prep_wo():
            for j in range(NJ):
                wof[j] = woraw[:, j * 128:(j + 1) * 128].astype(f32)
            for j in range(NJ):
                for d in range(DH):
                    blk = wof[j, pl.ds(d, H, stride=DH), :]
                    wop[d * 16:(d + 1) * 16, j * 128:(j + 1) * 128] = pltpu.bitcast(blk.astype(bf16), u32)

        def layernorm(x):
            m = jnp.sum(x, axis=-1, keepdims=True) * (1.0 / D)
            xc = x - m
            v = jnp.sum(xc * xc, axis=-1, keepdims=True) * (1.0 / D)
            return xc * jax.lax.rsqrt(v + EPS)

        def stage_a(i):
            r = row0(i)
            x = xs[pl.ds(r, T), :].astype(f32)
            y = layernorm(x).astype(bf16)
            for j in range(NJ):
                xn[j, pl.ds(r, T), :] = y[:, j * 128:(j + 1) * 128]

        def stage_b(i, parts=(0, 1, 2)):
            r = row0(i)
            lhs = jnp.concatenate([xn[j, pl.ds(r, T), :] for j in range(NJ)], axis=1)
            for p in parts:
                for j in range(NJ):
                    c = p * D + j * 128
                    w = pltpu.bitcast(wp[:, c:c + 128], bf16)
                    res = jnp.dot(lhs, w, preferred_element_type=f32)
                    if p == 0:
                        qs[j, pl.ds(r, T), :] = res * QSCALE
                    elif p == 1:
                        ks[j, pl.ds(r + HALO, T), :] = res
                    else:
                        vs[j, pl.ds(r + HALO, T), :] = res

        def stage_c(i, first=False):
            r = row0(i)
            for w in range(NW):
                a = None
                for j in range(NJ):
                    t = qs[j, pl.ds(r, T), :] * ks[j, pl.ds(r + HALO - DIL * w, T), :]
                    a = t if a is None else a + t
                a = a + pltpu.roll(a, 64, 1)
                a = a + pltpu.roll(a, 32, 1)
                if first and w > 0:
                    rows = jax.lax.broadcasted_iota(i32, (T, 128), 0)
                    a = jnp.where(rows >= DIL * w, a, -1e9)
                ls[w] = a
            RB = 8
            for rb in range(T // RB):
                r0 = rb * RB
                lw = [ls[w, r0:r0 + RB, :] for w in range(NW)]
                m = lw[0]
                for w in range(1, NW):
                    m = jnp.maximum(m, lw[w])
                es = [jnp.exp2(l - m) for l in lw]
                s = es[0]
                for w in range(1, NW):
                    s = s + es[w]
                inv = pl.reciprocal(s, approx=True)
                for j in range(NJ):
                    o = None
                    for w in range(NW):
                        t = es[w] * vs[j, pl.ds(r + HALO + r0 - DIL * w, RB), :]
                        o = t if o is None else o + t
                    os_[j, pl.ds(r + r0, RB), :] = (o * inv).astype(bf16)

        def stage_d(i):
            r = row0(i)
            lhs = jnp.concatenate([os_[j, pl.ds(r, T), :] for j in range(NJ)], axis=1)
            for j in range(NJ):
                w = pltpu.bitcast(wop[:, j * 128:(j + 1) * 128], bf16)
                res = jnp.dot(lhs, w, preferred_element_type=f32)
                hs[pl.ds(r, T), j * 128:(j + 1) * 128] = res + xs[pl.ds(r, T), j * 128:(j + 1) * 128].astype(f32)

        def stage_e(i):
            r = row0(i)
            h = hs[pl.ds(r, T), :]
            hn = layernorm(h)
            outs[pl.ds(r, T), :] = (h + hn).astype(bf16)
            rr = jnp.sum(hn * wrf[0:1, :], axis=-1, keepdims=True)
            bv = best[0]
            bi = best[1]
            rows = jax.lax.broadcasted_iota(i32, (8, 128), 0).astype(f32)
            for rb in range(T // 8):
                rv = jnp.broadcast_to(rr[rb * 8:(rb + 1) * 8, :], (8, 128))
                upd = rv > bv
                bv = jnp.where(upd, rv, bv)
                bi = jnp.where(upd, rows + (r + rb * 8).astype(f32) if not isinstance(r, int) else rows + float(r + rb * 8), bi)
            best[0] = bv
            best[1] = bi
            o_copy(i).start()

        x_copy(0).start()
        w_copy(0).start()
        x_copy(1).start()
        w_copy(1).start()
        w_copy(2).start()
        wr_copy.start()
        zeros16 = jnp.zeros((HALO, 128), f32)
        for j in range(NJ):
            ks[j, 0:HALO, :] = zeros16
            vs[j, 0:HALO, :] = zeros16
        best[0] = jnp.full((8, 128), -jnp.inf, f32)
        best[1] = jnp.zeros((8, 128), f32)
        x_copy(0).wait()
        stage_a(0)
        w_copy(0).wait()
        wo_copy.start()
        for i in range(2, NT):
            x_copy(i).start()
        prep_w(0)
        stage_b(0, (0,))
        w_copy(1).wait()
        prep_w(1)
        stage_b(0, (1,))
        w_copy(2).wait()
        wg_copy.start()
        wu_copy.start()
        wd_copy.start()
        prep_w(2)
        stage_b(0, (2,))
        x_copy(1).wait()
        stage_a(1)
        x_copy(2).wait()
        wo_copy.wait()
        wr_copy.wait()
        prep_wo()
        wrf[...] = jnp.broadcast_to(wr[...].astype(f32).reshape(1, D), (8, D))
        stage_b(1)
        stage_c(0, first=True)
        stage_a(2)

        def body(i, c):
            x_copy(i + 2).wait()
            stage_b(i + 1)
            stage_c(i)
            stage_d(i - 1)
            stage_e(i - 1)
            stage_a(i + 2)
            return c

        jax.lax.fori_loop(1, NT - 2, body, 0)
        stage_b(NT - 1)
        stage_c(NT - 2)
        stage_d(NT - 3)
        stage_e(NT - 3)
        stage_c(NT - 1)
        stage_d(NT - 2)
        stage_e(NT - 2)
        stage_d(NT - 1)
        stage_e(NT - 1)

        bv = best[0]
        bi = best[1]
        mx = jnp.max(bv, axis=0, keepdims=True)
        cand = jnp.where(bv == mx, bi, float(S))
        idx_v = jnp.min(cand, axis=0, keepdims=True)
        idx = jnp.minimum(jnp.min(idx_v).astype(i32), S - 1)
        base = pl.multiple_of((idx // 16) * 16, 16)
        h16 = hs[pl.ds(base, 16), :]
        hn16 = layernorm(h16)
        xb = hn16.astype(bf16)
        wg_copy.wait()
        wu_copy.wait()
        wd_copy.wait()
        g = jnp.dot(xb, wg[...], preferred_element_type=f32)
        u = jnp.dot(xb, wu[...], preferred_element_type=f32)
        act = (g * jax.nn.sigmoid(g) * u).astype(bf16)
        y = jnp.dot(act, wd[...], preferred_element_type=f32)
        gate = jax.nn.sigmoid(mx[:, 0:1])
        rows16 = jax.lax.broadcasted_iota(i32, (16, D), 0)
        y = jnp.where(rows16 == idx - base, y * gate, 0.0)
        for i in range(NT):
            o_copy(i).wait()
        outs[pl.ds(base, 16), :] = (h16 + hn16 + y).astype(bf16)
        fix = pltpu.make_async_copy(outs.at[pl.ds(base, 16)], out_hbm.at[pl.ds(base, 16)], sem_w.at[8])
        fix.start()
        fix.wait()

    scratch = [
        pltpu.VMEM((S, D), bf16),
        pltpu.VMEM((D, 3 * D), bf16),
        pltpu.VMEM((D // 2, 3 * D), u32),
        pltpu.VMEM((D, D), bf16),
        pltpu.VMEM((NJ, D, 128), f32),
        pltpu.VMEM((D // 2, D), u32),
        pltpu.VMEM((D,), bf16),
        pltpu.VMEM((8, D), f32),
        pltpu.VMEM((D, F), bf16),
        pltpu.VMEM((D, F), bf16),
        pltpu.VMEM((F, D), bf16),
        pltpu.VMEM((NJ, S, 128), bf16),
        pltpu.VMEM((NJ, S, 128), f32),
        pltpu.VMEM((NJ, S + HALO, 128), f32),
        pltpu.VMEM((NJ, S + HALO, 128), f32),
        pltpu.VMEM((NW, T, 128), f32),
        pltpu.VMEM((NJ, S, 128), bf16),
        pltpu.VMEM((S, D), f32),
        pltpu.VMEM((S, D), bf16),
        pltpu.VMEM((2, 8, 128), f32),
        pltpu.SemaphoreType.DMA((NT,)),
        pltpu.SemaphoreType.DMA((9,)),
        pltpu.SemaphoreType.DMA((NT,)),
    ]
    return kernel, scratch


def build(T=128):
    kernel, scratch = make_kernel(T)

    def fn(A_x, A_wqkv, A_wo, B_x, B_w_r, B_w_gate, B_w_up, B_w_down):
        x2 = A_x.reshape(S, D)
        out = pl.pallas_call(
            kernel,
            in_specs=[pl.BlockSpec(memory_space=pl.ANY)] * 7,
            out_specs=pl.BlockSpec(memory_space=pl.ANY),
            out_shape=jax.ShapeDtypeStruct((S, D), bf16),
            scratch_shapes=scratch,
            name="fused",
            compiler_params=pltpu.CompilerParams(vmem_limit_bytes=100 * 2**20),
        )(x2, A_wqkv, A_wo, B_w_r, B_w_gate, B_w_up, B_w_down)
        return out.reshape(1, S, D)
    return fn


_fn = build(T=128)


@jax.jit
def pallas_sequential_preLN__sliding_local_dilated__moe_arch_mod__prompt_kernel(
    A_x: jax.Array,
    A_wqkv: jax.Array,
    A_wo: jax.Array,
    B_x: jax.Array,
    B_w_r: jax.Array,
    B_w_gate: jax.Array,
    B_w_up: jax.Array,
    B_w_down: jax.Array,
):
    return _fn(A_x, A_wqkv, A_wo, B_x, B_w_r, B_w_gate, B_w_up, B_w_down)
```

```python
import functools
import math
import jax
import jax.numpy as jnp
from jax.experimental import pallas as pl
from jax.experimental.pallas import tpu as pltpu

S, D, H, DH, F = 2048, 640, 32, 20, 1536
NW, DIL = 8, 2
HALO = 16
NJ = D // 128
EPS = 1e-5
QSCALE = (DH ** -0.5) * math.log2(math.e)
f32, bf16, u32, i32 = jnp.float32, jnp.bfloat16, jnp.uint32, jnp.int32


def interleave(slots, pieces):
    pieces = sorted(pieces, key=lambda kp: kp[0])
    for k, p in pieces:
        if k < 0:
            p()
    for c, s in enumerate(slots):
        s()
        for k, p in pieces:
            if k == c:
                p()
    for k, p in pieces:
        if k >= len(slots):
            p()


def spread(pieces, lo, hi):
    n = len(pieces)
    return [(lo + (k * (hi - lo)) // n, p) for k, p in enumerate(pieces)]


def rsqrt(v):
    return jnp.exp2(jnp.log2(v) * -0.5)


def make_kernel(T=128, LNB=64, RB=16, unroll=2, onepass=True, pv_sched=(2, 3, 4, 5, 6, 7, 8, 9), a_sched=(16, 17), a_tok=True, a_d=2, pv_lag=2, qk_gate=True, qk_d=0, e_d=4, e_sched=(-1, 0), QB=16, tok_row=0, qk_sched=(10, 10, 11, 12, 13, 14, 15, 15)):
    NT = S // T

    def kernel(x_hbm, wqkv_hbm, wo_hbm, wr_hbm, wg_hbm, wu_hbm, wd_hbm, out_hbm,
               xs, wraw, wt, wp, woraw, wof, wop, wr, wrf, wg, wu, wd,
               xn0, xn1, qs, ks, vs, ls, os_, hs, outs, best, zv,
               sem_x, sem_w, sem_o):
        xn = (xn0, xn1)
        pending = []
        hist = []

        def emit_token(val_u32, d=1):
            pending.append((len(hist) + d - 1, val_u32))

        def gated(w_u32):
            due = [v for (c, v) in pending if c <= len(hist)]
            pending[:] = [(c, v) for (c, v) in pending if c > len(hist)]
            if not due:
                return w_u32
            t = due.pop()
            while due:
                t = t | due.pop()
            return jnp.concatenate([w_u32[0:8] | (t & zv[...]), w_u32[8:]], axis=0)

        def row0(i):
            return i * T if isinstance(i, int) else pl.multiple_of(i * T, T)

        def x_copy(i):
            return pltpu.make_async_copy(x_hbm.at[pl.ds(row0(i), T)], xs.at[pl.ds(row0(i), T)], sem_x.at[i])

        def w_copy(p):
            return pltpu.make_async_copy(wqkv_hbm.at[:, pl.ds(p * D, D)], wraw.at[:, pl.ds(p * D, D)], sem_w.at[p])

        wo_copy = pltpu.make_async_copy(wo_hbm, woraw, sem_w.at[3])
        wr_copy = pltpu.make_async_copy(wr_hbm, wr, sem_w.at[4])
        wg_copy = pltpu.make_async_copy(wg_hbm, wg, sem_w.at[5])
        wu_copy = pltpu.make_async_copy(wu_hbm, wu, sem_w.at[6])
        wd_copy = pltpu.make_async_copy(wd_hbm, wd, sem_w.at[7])

        def o_copy(i):
            return pltpu.make_async_copy(outs.at[pl.ds(row0(i), T)], out_hbm.at[pl.ds(row0(i), T)], sem_o.at[i])

        def prep_w_pieces(p):
            PB = 128

            def sel(rb):
                lane = jax.lax.broadcasted_iota(i32, (PB // 2, 128), 1)
                r5 = (lane // 4) % 5
                src = [pltpu.bitcast(wraw[rb * PB:(rb + 1) * PB, p * D + jj * 128: p * D + (jj + 1) * 128], u32)
                       for jj in range(NJ)]
                for j in range(NJ):
                    t = src[4]
                    for jj in range(4):
                        t = jnp.where(r5 == (j - 2 * jj) % 5, src[jj], t)
                    wt[rb * PB // 2:(rb + 1) * PB // 2, j * 128:(j + 1) * 128] = t

            def perm(j):
                lane = jax.lax.broadcasted_iota(i32, (D // 2, 128), 1)
                idx = (20 * (lane % 32) + 4 * j + lane // 32) % 128
                wp[:, p * D + j * 128: p * D + (j + 1) * 128] = jnp.take_along_axis(
                    wt[:, j * 128:(j + 1) * 128], idx, axis=1)
            return ([functools.partial(sel, rb) for rb in range(D // PB)]
                    + [functools.partial(perm, j) for j in range(NJ)])

        def prep_wo_pieces():
            def piece(j):
                wof[j] = woraw[:, j * 128:(j + 1) * 128].astype(f32)
                for d in range(DH):
                    blk = wof[j, pl.ds(d, H, stride=DH), :]
                    wop[d * 16:(d + 1) * 16, j * 128:(j + 1) * 128] = pltpu.bitcast(blk.astype(bf16), u32)
            return [functools.partial(piece, j) for j in range(NJ)]

        def ln_stats(x):
            m = jnp.sum(x, axis=-1, keepdims=True) * (1.0 / D)
            if onepass:
                v = jnp.maximum(jnp.sum(x * x, axis=-1, keepdims=True) * (1.0 / D) - m * m, 0.0)
            else:
                xc = x - m
                v = jnp.sum(xc * xc, axis=-1, keepdims=True) * (1.0 / D)
            return m, rsqrt(v + EPS)

        def a_pieces(i, dst, tok=False):
            r = row0(i)

            def piece(b):
                x = xs[pl.ds(r + b * LNB, LNB), :].astype(f32)
                m, rs = ln_stats(x)
                y = (x * rs - m * rs).astype(bf16)
                yu = pltpu.bitcast(y, u32)
                dst[b * LNB // 2:(b + 1) * LNB // 2, :] = yu
                if tok:
                    for r8 in range(LNB // 16):
                        emit_token(yu[r8 * 8:r8 * 8 + 8, D - 128:D], a_d)
            return [functools.partial(piece, b) for b in range(T // LNB)]

        def b_slots(p, par, first=False):
            def slot(j):
                lhs = pltpu.bitcast(xn[par][...], bf16)
                c = p * D + j * 128
                w = pltpu.bitcast(gated(wp[:, c:c + 128]), bf16)
                res = jnp.dot(lhs, w, preferred_element_type=f32)
                hist.append(res[tok_row:tok_row + 8])
                if p == 0:
                    qs[j] = res
                else:
                    dst = ks if p == 1 else vs
                    if first:
                        dst[j, 0:HALO, :] = jnp.zeros((HALO, 128), f32)
                    else:
                        dst[j, 0:HALO, :] = dst[j, T:T + HALO, :]
                    dst[j, HALO:HALO + T, :] = res
            return [functools.partial(slot, j) for j in range(NJ)]

        def qk_pieces(first=False, tok=False):
            def piece(rb):
                r0 = rb * QB
                sv = jnp.full((8, 128), QSCALE, f32)
                if tok and qk_gate:
                    sv = pltpu.bitcast(pltpu.bitcast(sv, u32) | (pltpu.bitcast(hist[-1], u32) & zv[...]), f32)
                q = [(qs[j, r0:r0 + QB, :].reshape(QB // 8, 8, 128) * sv[None]).reshape(QB, 128) for j in range(NJ)]
                for w in range(NW):
                    lo = HALO + r0 - DIL * w
                    a = None
                    for j in range(NJ):
                        t = q[j] * ks[j, lo:lo + QB, :]
                        a = t if a is None else a + t
                    a = a + pltpu.roll(a, 64, 1)
                    a = a + pltpu.roll(a, 32, 1)
                    if first and r0 < DIL * w:
                        rows = jax.lax.broadcasted_iota(i32, (QB, 128), 0) + r0
                        a = jnp.where(rows >= DIL * w, a, -1e9)
                    ls[w, r0:r0 + QB, :] = a
                    if tok and qk_d:
                        for r8 in range(QB // 8):
                            emit_token(pltpu.bitcast(a[r8 * 8:r8 * 8 + 8], u32), qk_d)
            return [functools.partial(piece, rb) for rb in range(T // QB)]

        def pv_pieces(tok=False):
            def piece(rb):
                r0 = rb * RB
                lw = [ls[w, r0:r0 + RB, :] for w in range(NW)]
                m = lw[0]
                for w in range(1, NW):
                    m = jnp.maximum(m, lw[w])
                if tok and len(hist) > pv_lag:
                    g = pltpu.bitcast(hist[-1 - pv_lag], u32) & zv[...]
                    m = pltpu.bitcast((pltpu.bitcast(m, u32).reshape(RB // 8, 8, 128) | g[None]).reshape(RB, 128), f32)
                es = [jnp.exp2(l - m) for l in lw]
                s = es[0]
                for w in range(1, NW):
                    s = s + es[w]
                inv = pl.reciprocal(s, approx=True)
                for j in range(NJ):
                    o = None
                    for w in range(NW):
                        lo = HALO + r0 - DIL * w
                        t = es[w] * vs[j, lo:lo + RB, :]
                        o = t if o is None else o + t
                    ob = pltpu.bitcast((o * inv).astype(bf16), u32)
                    os_[r0 // 2:(r0 + RB) // 2, j * 128:(j + 1) * 128] = ob
                    if tok:
                        emit_token(ob[0:8])
            return [functools.partial(piece, rb) for rb in range(T // RB)]

        def d_slots(i):
            r = row0(i)

            def slot(j):
                lhs = pltpu.bitcast(os_[...], bf16)
                w = pltpu.bitcast(gated(wop[:, j * 128:(j + 1) * 128]), bf16)
                res = jnp.dot(lhs, w, preferred_element_type=f32)
                hist.append(res[tok_row:tok_row + 8])
                hs[pl.ds(r, T), j * 128:(j + 1) * 128] = res + xs[pl.ds(r, T), j * 128:(j + 1) * 128].astype(f32)
            return [functools.partial(slot, j) for j in range(NJ)]

        def e_pieces(i, par=0, e_d=0):
            r = row0(i)

            def piece(b):
                rr = r + b * LNB
                h = hs[pl.ds(rr, LNB), :]
                m, rs = ln_stats(h)
                hw = (h.reshape(LNB // 8, 8, D) * wrf[0:8, :][None]).reshape(LNB, D)
                rr_ = (jnp.sum(hw, axis=-1, keepdims=True) - m * wrf[8:9, 0:1]) * rs
                ov = h * (1.0 + rs) - m * rs
                outs[pl.ds(rr, LNB), :] = ov.astype(bf16)
                if e_d:
                    for r8 in range(LNB // 8):
                        emit_token(pltpu.bitcast(ov[r8 * 8:r8 * 8 + 8, D - 128:D], u32), e_d)
                bv = best[2 * par]
                bi = best[2 * par + 1]
                rows = (jax.lax.broadcasted_iota(i32, (8, 128), 0) + rr).astype(f32)
                for rb in range(LNB // 8):
                    rv = jnp.broadcast_to(rr_[rb * 8:(rb + 1) * 8, :], (8, 128))
                    upd = rv > bv
                    bv = jnp.where(upd, rv, bv)
                    bi = jnp.where(upd, rows + float(rb * 8), bi)
                if e_d:
                    emit_token(pltpu.bitcast(bv, u32), e_d)
                best[2 * par] = bv
                best[2 * par + 1] = bi
                if b == T // LNB - 1:
                    o_copy(i).start()
            return [functools.partial(piece, b) for b in range(T // LNB)]

        def step(i, par, has_b=True, has_a=True, has_e=True, extra=()):
            pieces = []
            if has_b:
                slots = b_slots(0, 1 - par) + b_slots(1, 1 - par) + d_slots(i) + b_slots(2, 1 - par)
                pieces += spread(list(extra), 0, 5)
                if has_e:
                    pieces += list(zip(e_sched, e_pieces(i - 1, par, e_d)))
                pieces += list(zip(pv_sched, pv_pieces(True)))
                pieces += list(zip(qk_sched, qk_pieces(tok=True)))
                if has_a:
                    pieces += list(zip(a_sched, a_pieces(i + 2, xn[par], a_tok)))
            else:
                slots = d_slots(i)
                pieces += spread(pv_pieces(), -1, 0)
                pieces += spread(e_pieces(i - 1, par), 0, 2)
                pieces += spread(e_pieces(i, 1 - par), 5, 6)
            interleave(slots, pieces)

        x_copy(0).start()
        w_copy(0).start()
        w_copy(1).start()
        x_copy(1).start()
        w_copy(2).start()
        wr_copy.start()
        x_copy(2).start()
        wo_copy.start()
        for i in range(3, NT):
            x_copy(i).start()
        wg_copy.start()
        wu_copy.start()
        wd_copy.start()
        zv[...] = jnp.zeros((8, 128), u32)
        for par in range(2):
            best[2 * par] = jnp.full((8, 128), -jnp.inf, f32)
            best[2 * par + 1] = jnp.zeros((8, 128), f32)
        x_copy(0).wait()
        for p in a_pieces(0, xn[0]):
            p()
        w_copy(0).wait()
        for p in prep_w_pieces(0):
            p()
        w_copy(1).wait()
        interleave(b_slots(0, 0), spread(prep_w_pieces(1), 0, 5))
        w_copy(2).wait()
        x_copy(1).wait()
        interleave(b_slots(1, 0, True) + b_slots(2, 0, True),
                   spread(prep_w_pieces(2), 0, 5) + list(zip((5, 5, 6, 6, 7, 7, 8, 8), qk_pieces(True, True)))
                   + spread(a_pieces(1, xn[1]), 8, 10))
        x_copy(2).wait()
        wo_copy.wait()
        wr_copy.wait()
        wrv = jnp.broadcast_to(wr[...].astype(f32).reshape(1, D), (8, D))
        wrf[0:8, :] = wrv
        wrf[8:16, :] = jnp.broadcast_to(jnp.sum(wrv, axis=-1, keepdims=True), (8, D))
        hist.clear(); pending.clear()
        step(0, 0, has_e=False, extra=prep_wo_pieces())

        nloop = (NT - 3) // unroll

        def body(k, c):
            i0 = 1 + k * unroll
            hist.clear(); pending.clear()
            for u in range(unroll):
                x_copy(i0 + u + 2).wait()
            for u in range(unroll):
                step(i0 + u, (1 + u) % 2)
            return c

        jax.lax.fori_loop(0, nloop, body, 0)
        rest = list(range(1 + nloop * unroll, NT - 2))
        hist.clear(); pending.clear()
        for i in rest:
            x_copy(i + 2).wait()
        for i in rest:
            step(i, i % 2)
        step(NT - 2, NT % 2, has_a=False)
        step(NT - 1, (NT - 1) % 2, has_a=False, has_b=False)

        bv = jnp.concatenate([best[0], best[2]], axis=0)
        bi = jnp.concatenate([best[1], best[3]], axis=0)
        mx = jnp.max(bv, axis=0, keepdims=True)
        cand = jnp.where(bv == mx, bi, float(S))
        idx_v = jnp.min(cand, axis=0, keepdims=True)
        idx = jnp.minimum(jnp.min(idx_v).astype(i32), S - 1)
        base = pl.multiple_of((idx // 16) * 16, 16)
        h16 = hs[pl.ds(base, 16), :]
        m16, rs16 = ln_stats(h16)
        hn16 = (h16 - m16) * rs16
        xb = hn16.astype(bf16)
        wg_copy.wait()
        wu_copy.wait()
        wd_copy.wait()
        g = jnp.dot(xb, wg[...], preferred_element_type=f32)
        u = jnp.dot(xb, wu[...], preferred_element_type=f32)
        act = (g * jax.nn.sigmoid(g) * u).astype(bf16)
        y = jnp.dot(act, wd[...], preferred_element_type=f32)
        gate = jax.nn.sigmoid(mx[:, 0:1])
        rows16 = jax.lax.broadcasted_iota(i32, (16, D), 0)
        y = jnp.where(rows16 == idx - base, y * gate, 0.0)
        for i in range(NT):
            o_copy(i).wait()
        outs[pl.ds(base, 16), :] = (h16 + hn16 + y).astype(bf16)
        fix = pltpu.make_async_copy(outs.at[pl.ds(base, 16)], out_hbm.at[pl.ds(base, 16)], sem_w.at[8])
        fix.start()
        fix.wait()

    scratch = [
        pltpu.VMEM((S, D), bf16),
        pltpu.VMEM((D, 3 * D), bf16),
        pltpu.VMEM((D // 2, D), u32),
        pltpu.VMEM((D // 2, 3 * D), u32),
        pltpu.VMEM((D, D), bf16),
        pltpu.VMEM((NJ, D, 128), f32),
        pltpu.VMEM((D // 2, D), u32),
        pltpu.VMEM((D,), bf16),
        pltpu.VMEM((16, D), f32),
        pltpu.VMEM((D, F), bf16),
        pltpu.VMEM((D, F), bf16),
        pltpu.VMEM((F, D), bf16),
        pltpu.VMEM((T // 2, D), u32),
        pltpu.VMEM((T // 2, D), u32),
        pltpu.VMEM((NJ, T, 128), f32),
        pltpu.VMEM((NJ, T + HALO, 128), f32),
        pltpu.VMEM((NJ, T + HALO, 128), f32),
        pltpu.VMEM((NW, T, 128), f32),
        pltpu.VMEM((T // 2, D), u32),
        pltpu.VMEM((S, D), f32),
        pltpu.VMEM((S, D), bf16),
        pltpu.VMEM((4, 8, 128), f32),
        pltpu.VMEM((8, 128), u32),
        pltpu.SemaphoreType.DMA((NT,)),
        pltpu.SemaphoreType.DMA((9,)),
        pltpu.SemaphoreType.DMA((NT,)),
    ]
    return kernel, scratch


def build(**kw):
    kernel, scratch = make_kernel(**kw)

    def fn(A_x, A_wqkv, A_wo, B_x, B_w_r, B_w_gate, B_w_up, B_w_down):
        x2 = A_x.reshape(S, D)
        out = pl.pallas_call(
            kernel,
            in_specs=[pl.BlockSpec(memory_space=pl.ANY)] * 7,
            out_specs=pl.BlockSpec(memory_space=pl.ANY),
            out_shape=jax.ShapeDtypeStruct((S, D), bf16),
            scratch_shapes=scratch,
            name="fused",
            compiler_params=pltpu.CompilerParams(vmem_limit_bytes=100 * 2**20),
        )(x2, A_wqkv, A_wo, B_w_r, B_w_gate, B_w_up, B_w_down)
        return out.reshape(1, S, D)
    return fn


_fn = build(unroll=4)


@jax.jit
def pallas_sequential_preLN__sliding_local_dilated__moe_arch_mod__prompt_kernel(
    A_x: jax.Array,
    A_wqkv: jax.Array,
    A_wo: jax.Array,
    B_x: jax.Array,
    B_w_r: jax.Array,
    B_w_gate: jax.Array,
    B_w_up: jax.Array,
    B_w_down: jax.Array,
):
    return _fn(A_x, A_wqkv, A_wo, B_x, B_w_r, B_w_gate, B_w_up, B_w_down)
```

```python
import functools
import math
import jax
import jax.numpy as jnp
from jax.experimental import pallas as pl
from jax.experimental.pallas import tpu as pltpu

S, D, H, DH, F = 2048, 640, 32, 20, 1536
NW, DIL = 8, 2
HALO = 16
NJ = D // 128
EPS = 1e-5
QSCALE = (DH ** -0.5) * math.log2(math.e)
f32, bf16, u32, i32 = jnp.float32, jnp.bfloat16, jnp.uint32, jnp.int32


def interleave(slots, pieces):
    pieces = sorted(pieces, key=lambda kp: kp[0])
    for k, p in pieces:
        if k < 0:
            p()
    for c, s in enumerate(slots):
        s()
        for k, p in pieces:
            if k == c:
                p()
    for k, p in pieces:
        if k >= len(slots):
            p()


def spread(pieces, lo, hi):
    n = len(pieces)
    return [(lo + (k * (hi - lo)) // n, p) for k, p in enumerate(pieces)]


def at(sched, pieces, off=0):
    k = len(pieces) // len(sched)
    sched = [c for c in sched for _ in range(k)]
    return [(c + off, p) for c, p in zip(sched, pieces, strict=True)]


def pack2(even, odd):
    p = pltpu.pack_elementwise([even, odd], packed_dtype=bf16)
    return p if p.dtype == u32 else pltpu.bitcast(p, u32)


def rsqrt(v):
    return jnp.exp2(jnp.log2(v) * -0.5)


def make_kernel(T=128, LNB=64, RB=16, QB=16, unroll=4,
                pv_sched=(3, 4, 6, 7, 8, 10, 11, 12), pv_lag=2,
                a_sched=(20, 21), a_d=3,
                e_sched=(-1, 1), e_d=5,
                qk_sched=(12, 13, 14, 15, 16, 17, 18, 19), NWQ=4, only=None, ksplit=True, opaque=(), smqk=0, ilv_a=True, ilv_pv=True, qkpar=True, areload=False, pv_ng=1, nobc=True, padq=8, padl=8, padk=8, t_e0=(-1, 0), t_ed0=4,
                y_qk0=(1, 2, 3, 4, 5, 5, 5, 8), y_qk1=(6, 7, 7, 8, 10, 11, 12, 12), y_pv=(10, 10, 11, 11, 12, 12, 13, 13), y_pvtok=False,
                z_pv=(2, 3, 4, 5, 6, 7, 8, 9), z_qk=(9, 10, 11, 12, 13, 14, 15, 15), z_e=(13, 14), z_ed=0, z_a=(16, 17), z_ad=2,
                t_pvtok=False, t_pv0=(3, 4, 5, 6, 7, 8, 9, 10), t_ed=2,
                t_qk=(9, 10, 11, 11, 11, 11, 12, 13), t_pv=(15, 16, 17, 18, 18, 18, 19, 19), t_e=(22, 22), scopes=False):
    NT = S // T

    def kernel(x_hbm, wqkv_hbm, wo_hbm, wr_hbm, wg_hbm, wu_hbm, wd_hbm, out_hbm,
               xs, wraw, wt, wp, woraw, wof, wop, wr, wrf, wg, wu, wd,
               xn0, xn1, xna, qs, qa, qb, ks, ka, vs, va, ls, lsa, os_, osa, hs, outs, best, zv, pk, zs,
               sem_x, sem_w, sem_q, sem_o):
        xn = (xn0, xn1)
        qq, kk = (qs, qa), (ks, ka)
        pending = []
        hist = []

        zz = [0]

        def new_block():
            hist.clear()
            pending.clear()
            zz[0] = pl.multiple_of(zs[0], 8)

        def dyn(name, start, n):
            if name in opaque:
                return pl.ds(zz[0] + start, n)
            return pl.ds(start, n)

        def emit_token(val_u32, d=1):
            pending.append((len(hist) + d - 1, val_u32))

        def take_due(t_now):
            due = [v for (c, v) in pending if c <= t_now]
            pending[:] = [(c, v) for (c, v) in pending if c > t_now]
            if not due:
                return None
            t = due.pop()
            while due:
                t = t | due.pop()
            return t & zv[...]

        def gated(w_u32):
            t = take_due(len(hist))
            if t is None:
                return w_u32
            return jnp.concatenate([w_u32[0:8] | t, w_u32[8:]], axis=0)

        def gate_after(lag):
            if len(hist) > lag:
                return pltpu.bitcast(hist[-1 - lag], u32) & zv[...]
            return None

        def row0(i):
            return i * T if isinstance(i, int) else pl.multiple_of(i * T, T)

        def x_copy(i):
            return pltpu.make_async_copy(x_hbm.at[pl.ds(row0(i), T)], xs.at[pl.ds(row0(i), T)], sem_x.at[i])

        def w_copy(p):
            return pltpu.make_async_copy(wqkv_hbm.at[:, pl.ds(p * D, D)], wraw.at[:, pl.ds(p * D, D)], sem_w.at[p])

        WQR = D // NWQ

        def wq_copy(c):
            return pltpu.make_async_copy(wqkv_hbm.at[pl.ds(c * WQR, WQR), pl.ds(0, D)],
                                         wraw.at[pl.ds(c * WQR, WQR), pl.ds(0, D)], sem_q.at[c])

        wo_copy = pltpu.make_async_copy(wo_hbm, woraw, sem_w.at[3])
        wr_copy = pltpu.make_async_copy(wr_hbm, wr, sem_w.at[4])
        wg_copy = pltpu.make_async_copy(wg_hbm, wg, sem_w.at[5])
        wu_copy = pltpu.make_async_copy(wu_hbm, wu, sem_w.at[6])
        wd_copy = pltpu.make_async_copy(wd_hbm, wd, sem_w.at[7])

        def o_copy(i):
            return pltpu.make_async_copy(outs.at[pl.ds(row0(i), T)], out_hbm.at[pl.ds(row0(i), T)], sem_o.at[i])

        def prep_w_pieces(p, lo=0, hi=D, PB=128):
            def sel(r0):
                lane = jax.lax.broadcasted_iota(i32, (PB // 2, 128), 1)
                r5 = (lane // 4) % 5
                src = [pltpu.bitcast(wraw[r0:r0 + PB, p * D + jj * 128: p * D + (jj + 1) * 128], u32)
                       for jj in range(NJ)]
                for j in range(NJ):
                    t = src[4]
                    for jj in range(4):
                        t = jnp.where(r5 == (j - 2 * jj) % 5, src[jj], t)
                    wt[r0 // 2:(r0 + PB) // 2, j * 128:(j + 1) * 128] = t

            def perm(j):
                lane = jax.lax.broadcasted_iota(i32, ((hi - lo) // 2, 128), 1)
                idx = (20 * (lane % 32) + 4 * j + lane // 32) % 128
                wp[lo // 2:hi // 2, p * D + j * 128: p * D + (j + 1) * 128] = jnp.take_along_axis(
                    wt[lo // 2:hi // 2, j * 128:(j + 1) * 128], idx, axis=1)
            return ([functools.partial(sel, r0) for r0 in range(lo, hi, PB)]
                    + [functools.partial(perm, j) for j in range(NJ)])

        def prep_wo_pieces():
            def piece(j):
                wof[j] = woraw[:, j * 128:(j + 1) * 128].astype(f32)
                for d in range(DH):
                    wop[d * 16:(d + 1) * 16, j * 128:(j + 1) * 128] = pack2(
                        wof[j, pl.ds(d, H // 2, stride=2 * DH), :], wof[j, pl.ds(d + DH, H // 2, stride=2 * DH), :])
            return [functools.partial(piece, j) for j in range(NJ)]

        def ln_stats(x):
            m = jnp.sum(x, axis=-1, keepdims=True) * (1.0 / D)
            v = jnp.maximum(jnp.sum(x * x, axis=-1, keepdims=True) * (1.0 / D) - m * m, 0.0)
            return m, rsqrt(v + EPS)

        def a_pieces(i, dst, d=0):
            r = row0(i)

            def piece(b):
                if ilv_a:
                    xu = pltpu.bitcast(xs[pl.ds(r + b * LNB, LNB), :], u32)
                    ys = []
                    for half in range(2):
                        x = pltpu.unpack_elementwise(xu, index=half, packed_dtype=bf16, unpacked_dtype=f32)
                        m, rs = ln_stats(x)
                        ys.append(x * rs - m * rs)
                    yu = pack2(ys[0], ys[1])
                else:
                    x = xs[pl.ds(r + b * LNB, LNB), :].astype(f32)
                    m, rs = ln_stats(x)
                    yu = pltpu.bitcast((x * rs - m * rs).astype(bf16), u32)
                dst[dyn('xn', b * LNB // 2, LNB // 2), :] = yu
                if d:
                    for r8 in range(LNB // 16):
                        emit_token(yu[r8 * 8:r8 * 8 + 8, D - 128:D], d)
            return [functools.partial(piece, b) for b in range(T // LNB)]

        def b_slots(p, src, dst, halo=None):
            def slot(j):
                lhs = pltpu.bitcast(src[...], bf16)
                c = p * D + j * 128
                w = pltpu.bitcast(gated(wp[:, c:c + 128]), bf16)
                res = jnp.dot(lhs, w, preferred_element_type=f32)
                hist.append(res[0:8])
                if p == 0:
                    dst[j, dyn('q', 0, T), :] = res
                else:
                    if halo is None:
                        dst[j, 0:HALO, :] = jnp.zeros((HALO, 128), f32)
                    else:
                        dst[j, 0:HALO, :] = halo[j, T:T + HALO, :]
                    dst[j, dyn('kv', HALO, T), :] = res
            return [functools.partial(slot, j) for j in range(NJ)]

        def ldw(ref, j, start, n):
            if not ilv_pv:
                return ref[j, start:start + n, :]
            parts = []
            for g0 in range(start, start + n, 16):
                parts += [ref[j, pl.ds(g0, 8, stride=2), :], ref[j, pl.ds(g0 + 1, 8, stride=2), :]]
            return jnp.concatenate(parts, axis=0)

        def qk_pieces(qr, kr, lr, first=False):
            def piece(rb):
                r0 = rb * QB
                sv = jnp.full((8, 128), QSCALE, f32)
                g = gate_after(0)
                if g is not None:
                    sv = pltpu.bitcast(pltpu.bitcast(sv, u32) | g, f32)
                lw = []
                q = [(ldw(qr, j, r0, QB).reshape(QB // 8, 8, 128) * sv[None]).reshape(QB, 128) for j in range(NJ)]
                for w in range(NW):
                    lo = HALO + r0 - DIL * w
                    a = None
                    for j in range(NJ):
                        t = q[j] * ldw(kr, j, lo, QB)
                        a = t if a is None else a + t
                    a = a + pltpu.roll(a, 64, 1)
                    a = a + pltpu.roll(a, 32, 1)
                    if first and r0 < DIL * w:
                        rows = jax.lax.broadcasted_iota(i32, (QB, 128), 0)
                        if ilv_pv:
                            rows = (rows // 16) * 16 + (rows % 8) * 2 + (rows % 16) // 8
                        rows = rows + r0
                        a = jnp.where(rows >= DIL * w, a, -1e9)
                    if smqk:
                        lw.append(a)
                    else:
                        lr[w, dyn('ls', r0, QB), :] = a
                if smqk:
                    m = lw[0]
                    for w in range(1, NW):
                        m = jnp.maximum(m, lw[w])
                    es = [jnp.exp2(l - m) for l in lw]
                    s = es[0]
                    for w in range(1, NW):
                        s = s + es[w]
                    inv = pl.reciprocal(s, approx=True)
                    if smqk == 1:
                        for w in range(NW):
                            lr[w, dyn('ls', r0, QB), :] = es[w] * inv
                    else:
                        for w in range(NW):
                            lr[w, dyn('ls', r0, QB), :] = es[w]
                        lr[NW, dyn('ls', r0, QB), :] = inv
            return [functools.partial(piece, rb) for rb in range(T // QB)]

        def pv_pieces(lr, vr, orf, tok=True):
            def piece(rb):
                r0 = rb * RB
                lw = [lr[w, r0:r0 + RB, :] for w in range(NW)]
                g = gate_after(pv_lag) if tok else None

                def gt(m):
                    if g is None:
                        return m
                    return pltpu.bitcast((pltpu.bitcast(m, u32).reshape(RB // 8, 8, 128) | g[None]).reshape(RB, 128), f32)
                if smqk:
                    es = [gt(l) if w < pv_ng else l for w, l in enumerate(lw)]
                    inv = None if smqk == 1 else lr[NW, r0:r0 + RB, :]
                else:
                    m = lw[0]
                    for w in range(1, NW):
                        m = jnp.maximum(m, lw[w])
                    m = gt(m)
                    es = [jnp.exp2(l - m) for l in lw]
                    s = es[0]
                    for w in range(1, NW):
                        s = s + es[w]
                    inv = pl.reciprocal(s, approx=True)
                for j in range(NJ):
                    o = None
                    for w in range(NW):
                        lo = HALO + r0 - DIL * w
                        t = es[w] * ldw(vr, j, lo, RB)
                        o = t if o is None else o + t
                    o = o if inv is None else o * inv
                    if ilv_pv:
                        ob = jnp.concatenate([pack2(o[g0:g0 + 8], o[g0 + 8:g0 + 16]) for g0 in range(0, RB, 16)], axis=0)
                    else:
                        ob = pltpu.bitcast(o.astype(bf16), u32)
                    orf[dyn('os', r0 // 2, RB // 2), j * 128:(j + 1) * 128] = ob
                    if tok:
                        emit_token(ob[0:8])
            return [functools.partial(piece, rb) for rb in range(T // RB)]

        def d_slots(i, orf):
            r = row0(i)

            def slot(j):
                lhs = pltpu.bitcast(orf[...], bf16)
                w = pltpu.bitcast(gated(wop[:, j * 128:(j + 1) * 128]), bf16)
                res = jnp.dot(lhs, w, preferred_element_type=f32)
                hist.append(res[0:8])
                hs[pl.ds(r, T), j * 128:(j + 1) * 128] = res + xs[pl.ds(r, T), j * 128:(j + 1) * 128].astype(f32)
            return [functools.partial(slot, j) for j in range(NJ)]

        def e_pieces(i, par, d=0):
            r = row0(i)

            def piece(b):
                rr = r + b * LNB
                h = hs[pl.ds(pl.multiple_of(rr + zz[0], 8) if 'hs' in opaque else rr, LNB), :]
                m, rs = ln_stats(h)
                hw = (h.reshape(LNB // 8, 8, D) * wrf[0:8, :][None]).reshape(LNB, D)
                rv_all = (jnp.sum(hw, axis=-1, keepdims=True) - m * wrf[8:9, 0:1]) * rs
                ov = h * (1.0 + rs) - m * rs
                outs[pl.ds(rr, LNB), :] = ov.astype(bf16)
                bv = best[2 * par]
                bi = best[2 * par + 1]
                rows = (jax.lax.broadcasted_iota(i32, (8, 128), 0) + rr).astype(f32)
                for rb in range(LNB // 8):
                    rv = jnp.broadcast_to(rv_all[rb * 8:(rb + 1) * 8, :], (8, 128))
                    upd = rv > bv
                    bv = jnp.where(upd, rv, bv)
                    bi = jnp.where(upd, rows + float(rb * 8), bi)
                if d:
                    for r8 in range(LNB // 8):
                        emit_token(pltpu.bitcast(ov[r8 * 8:r8 * 8 + 8, D - 128:D], u32), d)
                    emit_token(pltpu.bitcast(bv, u32), d)
                best[2 * par] = bv
                best[2 * par + 1] = bi
                if b == T // LNB - 1:
                    o_copy(i).start()
            return [functools.partial(piece, b) for b in range(T // LNB)]

        K4 = 512

        def g_dot(src, wref, c0, n, slot0, add_x=None, tok=True):
            wu = wref[K4 // 2:, c0 * 128:(c0 + n) * 128]
            if tok:
                t = take_due(len(hist))
                if t is not None:
                    top = jnp.concatenate([wu[0:8, 0:128] | t, wu[0:8, 128:]], axis=1) if n > 1 else wu[0:8] | t
                    wu = jnp.concatenate([top, wu[8:]], axis=0)
            lhs = pltpu.bitcast(src[:, K4:], bf16)
            res = jnp.dot(lhs, pltpu.bitcast(wu, bf16), preferred_element_type=f32)
            for u in range(n):
                r = res[:, u * 128:(u + 1) * 128]
                if add_x is not None:
                    r = r + xs[pl.ds(add_x, T), (c0 + u) * 128:(c0 + u + 1) * 128].astype(f32)
                pk[slot0 + u, dyn('pk', 0, T), :] = r
            return res[0:8, 0:128]

        def gb_slot(src, c0):
            def slot():
                hist.append(g_dot(src, wp, c0, 4, c0))
            return slot

        def gd_slots(i, src, orf):
            r = row0(i)

            def s0():
                hist.append(g_dot(orf, wop, 0, 4, 15, r))

            def s1():
                hist.append(g_dot(orf, wop, 4, 1, 19, r))
                g_dot(src, wp, 12, 3, 12, tok=False)
            return [s0, s1]

        def b4_slots(p, src, dst, halo):
            def slot(j):
                c = p * D + j * 128
                w = pltpu.bitcast(gated(wp[0:K4 // 2, c:c + 128]), bf16)
                lhs = pltpu.bitcast(src[:, 0:K4], bf16)
                res = jnp.dot(lhs, w, preferred_element_type=f32)
                hist.append(res[0:8])
                res = res + pk[p * NJ + j, 0:T, :]
                if p == 0:
                    dst[j, dyn('q', 0, T), :] = res
                else:
                    dst[j, 0:HALO, :] = halo[j, T:T + HALO, :]
                    dst[j, dyn('kv', HALO, T), :] = res
            return [functools.partial(slot, j) for j in range(NJ)]

        def d4_slots(i, orf):
            r = row0(i)

            def slot(j):
                w = pltpu.bitcast(gated(wop[0:K4 // 2, j * 128:(j + 1) * 128]), bf16)
                lhs = pltpu.bitcast(orf[:, 0:K4], bf16)
                res = jnp.dot(lhs, w, preferred_element_type=f32)
                hist.append(res[0:8])
                hs[pl.ds(r, T), j * 128:(j + 1) * 128] = res + pk[15 + j, 0:T, :]
            return [functools.partial(slot, j) for j in range(NJ)]

        def step(i, par, has_a=True):
            pieces = []
            src = xn[1 - par]
            qn, kn, kp = (qq[1 - par], kk[1 - par], kk[par]) if qkpar else (qs, ks, ks)
            if ksplit:
                slots = ([gb_slot(src, 0), gb_slot(src, 4), gb_slot(src, 8)]
                         + b4_slots(0, src, qn, None) + b4_slots(1, src, kn, kp)
                         + gd_slots(i, src, os_) + d4_slots(i, os_) + b4_slots(2, src, vs, vs))
            else:
                slots = b_slots(0, src, qn) + b_slots(1, src, kn, kp) + d_slots(i, os_) + b_slots(2, src, vs, vs)
            pieces += at(e_sched, e_pieces(i - 1, par, e_d))
            pieces += at(pv_sched, pv_pieces(ls, vs, os_))
            pieces += at(qk_sched, qk_pieces(qn, kn, ls))
            if has_a:
                pieces += at(a_sched, a_pieces(i + 2, xn[par], a_d))
            interleave(slots, pieces)

        def blk(name, f):
            return f if only in (None, name) else (lambda *a, **k: None)

        cur = [None]

        def mark(name):
            if not scopes:
                return
            if cur[0] is not None:
                cur[0].__exit__(None, None, None)
                cur[0] = None
            if name:
                cur[0] = jax.named_scope(name)
                cur[0].__enter__()

        mark("s0_start")
        x_copy(0).start()
        for c in range(NWQ):
            wq_copy(c).start()
        x_copy(1).start()
        x_copy(2).start()
        w_copy(1).start()
        zv[...] = jnp.zeros((8, 128), u32)
        zs[0] = 0
        for par in range(2):
            best[2 * par] = jnp.full((8, 128), -jnp.inf, f32)
            best[2 * par + 1] = jnp.zeros((8, 128), f32)
        x_copy(0).wait()
        for p in a_pieces(0, xna):
            p()
        for c in range(NWQ):
            wq_copy(c).wait()
            for p in prep_w_pieces(0, c * WQR, (c + 1) * WQR, WQR // 2 if WQR % 32 == 0 else WQR):
                p()
        x_copy(1).wait()
        x_copy(2).wait()
        mark('s1_X')
        w_copy(2).start()
        new_block()
        blk('X', interleave)(b_slots(0, xna, qa) + b_slots(0, xn[1], qb),
                   spread(a_pieces(1, xn[1]), 0, 2) + spread(a_pieces(2, xn[0], 2), 5, 8))
        mark('s2_waitWk')
        w_copy(1).wait()
        mark('s3_X2')
        wr_copy.start()
        wo_copy.start()
        x_copy(3).start()
        new_block()
        blk('X2', interleave)(b_slots(0, xn[0], qs) + b_slots(1, xna, ka), spread(prep_w_pieces(1), -1, 4))
        mark('s4_waitWv')
        w_copy(2).wait()
        mark('s5_Y')
        for i in range(4, NT):
            x_copy(i).start()
        new_block()
        blk('Y', interleave)(b_slots(1, xn[1], ks, ka) + b_slots(2, xna, va) + b_slots(2, xn[1], vs, va),
                   spread(prep_w_pieces(2), -1, 4)
                   + at(y_qk0, qk_pieces(qa, ka, lsa, True))
                   + at(y_qk1, qk_pieces(qb, ks, ls))
                   + at(y_pv, pv_pieces(lsa, va, osa, y_pvtok)))
        mark('s6_waitWo')
        wo_copy.wait()
        wr_copy.wait()
        x_copy(3).wait()
        mark('s7_Z')
        wg_copy.start()
        wu_copy.start()
        wd_copy.start()
        new_block()
        wrv = jnp.broadcast_to(wr[...].astype(f32).reshape(1, D), (8, D))
        wrf[0:8, :] = wrv
        wrf[8:16, :] = jnp.broadcast_to(jnp.sum(wrv, axis=-1, keepdims=True), (8, D))
        blk('Z', interleave)(b_slots(1, xn[0], ks, ks) + d_slots(0, osa) + d_slots(1, os_) + b_slots(2, xn[0], vs, vs),
                   spread(prep_wo_pieces(), -1, 4)
                   + at(z_pv, pv_pieces(ls, vs, os_))
                   + at(z_qk, qk_pieces(qs, ks, ls))
                   + at(z_e, e_pieces(0, 0, z_ed))
                   + at(z_a, a_pieces(3, xn[1], z_ad)))

        first = 2
        nloop = (NT - 2 - first) // unroll

        def body(k, c):
            i0 = first + k * unroll
            for u in range(unroll):
                x_copy(i0 + u + 2).wait()
            new_block()
            for u in range(unroll):
                blk('loop', step)(i0 + u, (first + u) % 2)
            return c

        mark('s8_loop')
        jax.lax.fori_loop(0, nloop, body, 0)
        mark('s9_tail')
        rest = list(range(first + nloop * unroll, NT - 2))
        for i in rest:
            x_copy(i + 2).wait()
        new_block()
        for i in rest:
            step(i, i % 2)
        L = NT - 1
        src = xn[L % 2]
        qn, kn, kp = (qq[L % 2], kk[L % 2], kk[1 - L % 2]) if qkpar else (qs, ks, ks)
        blk('tail', interleave)(b_slots(0, src, qn) + b_slots(1, src, kn, kp) + b_slots(2, src, va, vs)
                   + d_slots(L - 1, os_) + d_slots(L, osa),
                   at(t_e0, e_pieces(L - 2, L % 2, t_ed0))
                   + at(t_pv0, pv_pieces(ls, vs, os_))
                   + at(t_qk, qk_pieces(qn, kn, lsa))
                   + at(t_pv, pv_pieces(lsa, va, osa, t_pvtok))
                   + at(t_e, e_pieces(L - 1, (L - 1) % 2, t_ed))
                   + spread(e_pieces(L, L % 2), 25, 26))

        mark('sa_ffn')
        bv = jnp.concatenate([best[0], best[2]], axis=0)
        bi = jnp.concatenate([best[1], best[3]], axis=0)
        mx = jnp.max(bv, axis=0, keepdims=True)
        cand = jnp.where(bv == mx, bi, float(S))
        idx_v = jnp.min(cand, axis=0, keepdims=True)
        idx = jnp.minimum(jnp.min(idx_v).astype(i32), S - 1)
        base = pl.multiple_of((idx // 16) * 16, 16)
        h16 = hs[pl.ds(base, 16), :]
        m16, rs16 = ln_stats(h16)
        hn16 = (h16 - m16) * rs16
        xb = hn16.astype(bf16)
        wg_copy.wait()
        wu_copy.wait()
        wd_copy.wait()
        g = jnp.dot(xb, wg[...], preferred_element_type=f32)
        u = jnp.dot(xb, wu[...], preferred_element_type=f32)
        act = (g * jax.nn.sigmoid(g) * u).astype(bf16)
        y = jnp.dot(act, wd[...], preferred_element_type=f32)
        gate = jax.nn.sigmoid(mx[:, 0:1])
        rows16 = jax.lax.broadcasted_iota(i32, (16, D), 0)
        y = jnp.where(rows16 == idx - base, y * gate, 0.0)
        mark('sb_owait')
        for i in range(NT):
            o_copy(i).wait()
        mark('sc_fix')
        outs[pl.ds(base, 16), :] = (h16 + hn16 + y).astype(bf16)
        fix = pltpu.make_async_copy(outs.at[pl.ds(base, 16)], out_hbm.at[pl.ds(base, 16)], sem_w.at[8])
        fix.start()
        fix.wait()
        mark(None)

    lhs_buf = pltpu.VMEM((T // 2, D), u32)
    q_buf = pltpu.VMEM((NJ, T + padq, 128), f32)
    kv_buf = pltpu.VMEM((NJ, T + HALO + padk, 128), f32)
    l_buf = pltpu.VMEM((NW + 1, T + padl, 128), f32)
    scratch = [
        pltpu.VMEM((S, D), bf16),
        pltpu.VMEM((D, 3 * D), bf16),
        pltpu.VMEM((D // 2, D), u32),
        pltpu.VMEM((D // 2, 3 * D), u32),
        pltpu.VMEM((D, D), bf16),
        pltpu.VMEM((NJ, D, 128), f32),
        pltpu.VMEM((D // 2, D), u32),
        pltpu.VMEM((D,), bf16),
        pltpu.VMEM((16, D), f32),
        pltpu.VMEM((D, F), bf16),
        pltpu.VMEM((D, F), bf16),
        pltpu.VMEM((F, D), bf16),
        lhs_buf, lhs_buf, lhs_buf,
        q_buf, q_buf, q_buf,
        kv_buf, kv_buf, kv_buf, kv_buf,
        l_buf, l_buf,
        lhs_buf, lhs_buf,
        pltpu.VMEM((S, D), f32),
        pltpu.VMEM((S, D), bf16),
        pltpu.VMEM((4, 8, 128), f32),
        pltpu.VMEM((8, 128), u32),
        pltpu.VMEM((20, T + padq, 128), f32),
        pltpu.SMEM((1,), i32),
        pltpu.SemaphoreType.DMA((NT,)),
        pltpu.SemaphoreType.DMA((9,)),
        pltpu.SemaphoreType.DMA((NWQ,)),
        pltpu.SemaphoreType.DMA((NT,)),
    ]
    return kernel, scratch


def build(**kw):
    nobc = kw.get('nobc', True)
    kernel, scratch = make_kernel(**kw)

    def fn(A_x, A_wqkv, A_wo, B_x, B_w_r, B_w_gate, B_w_up, B_w_down):
        x2 = A_x.reshape(S, D)
        out = pl.pallas_call(
            kernel,
            in_specs=[pl.BlockSpec(memory_space=pl.ANY)] * 7,
            out_specs=pl.BlockSpec(memory_space=pl.ANY),
            out_shape=jax.ShapeDtypeStruct((S, D), bf16),
            scratch_shapes=scratch,
            name="fused",
            compiler_params=pltpu.CompilerParams(vmem_limit_bytes=100 * 2**20, disable_bounds_checks=nobc),
        )(x2, A_wqkv, A_wo, B_w_r, B_w_gate, B_w_up, B_w_down)
        return out.reshape(1, S, D)
    return fn


_fn = build()


@jax.jit
def pallas_sequential_preLN__sliding_local_dilated__moe_arch_mod__prompt_kernel(
    A_x: jax.Array,
    A_wqkv: jax.Array,
    A_wo: jax.Array,
    B_x: jax.Array,
    B_w_r: jax.Array,
    B_w_gate: jax.Array,
    B_w_up: jax.Array,
    B_w_down: jax.Array,
):
    return _fn(A_x, A_wqkv, A_wo, B_x, B_w_r, B_w_gate, B_w_up, B_w_down)
```

```python
import functools
import math
import jax
import jax.numpy as jnp
from jax.experimental import pallas as pl
from jax.experimental.pallas import tpu as pltpu

S, D, H, DH, F = 2048, 640, 32, 20, 1536
NW, DIL = 8, 2
HALO = 16
NJ = D // 128
EPS = 1e-5
QSCALE = (DH ** -0.5) * math.log2(math.e)
f32, bf16, u32, i32 = jnp.float32, jnp.bfloat16, jnp.uint32, jnp.int32


def interleave(slots, pieces):
    pieces = sorted(pieces, key=lambda kp: kp[0])
    for k, p in pieces:
        if k < 0:
            p()
    for c, s in enumerate(slots):
        s()
        for k, p in pieces:
            if k == c:
                p()
    for k, p in pieces:
        if k >= len(slots):
            p()


def spread(pieces, lo, hi):
    n = len(pieces)
    return [(lo + (k * (hi - lo)) // n, p) for k, p in enumerate(pieces)]


def at(sched, pieces, off=0):
    k = len(pieces) // len(sched)
    sched = [c for c in sched for _ in range(k)]
    return [(c + off, p) for c, p in zip(sched, pieces, strict=True)]


def pack2(even, odd):
    p = pltpu.pack_elementwise([even, odd], packed_dtype=bf16)
    return p if p.dtype == u32 else pltpu.bitcast(p, u32)


def rsqrt(v):
    return jnp.exp2(jnp.log2(v) * -0.5)


def make_kernel(T=128, LNB=64, RB=16, QB=16, unroll=4,
                pv_sched=(3, 4, 6, 7, 8, 10, 11, 12), pv_lag=2,
                a_sched=(20, 21), a_d=3,
                e_sched=(-1, 1), e_d=5,
                qk_sched=(12, 13, 14, 15, 16, 17, 18, 19), NWQ=4, only=None, ksplit=True, opaque=(), smqk=0, sel_pb=64, sel_d=0, sel_hi=2, perm_sched=(2, 2, 3, 3, 4), z_wo=(-1, 0, 1, 2, 3), z_wod=0, ilv_a=True, ilv_pv=True, qkpar=True, areload=False, pv_ng=1, nobc=True, padq=8, padl=8, padk=8, t_e0=(-1, 0), t_ed0=4,
                y_qk0=(1, 2, 3, 4, 5, 5, 5, 8), y_qk1=(6, 7, 7, 8, 10, 11, 12, 12), y_pv=(10, 10, 11, 11, 12, 12, 13, 13), y_pvtok=False,
                z_pv=(2, 3, 4, 5, 6, 7, 8, 9), z_qk=(10, 11, 12, 13, 14, 15, 16, 16), z_e=(13, 16), z_ed=1, z_a=(16, 17), z_ad=2,
                t_pvtok=False, t_pv0=(3, 4, 5, 6, 7, 8, 9, 10), t_ed=2,
                t_qk=(9, 10, 11, 11, 11, 11, 12, 13), t_pv=(15, 16, 17, 18, 18, 18, 19, 19), t_e=(22, 22), scopes=False):
    NT = S // T

    def kernel(x_hbm, wqkv_hbm, wo_hbm, wr_hbm, wg_hbm, wu_hbm, wd_hbm, out_hbm,
               xs, wraw, wt, wp, woraw, wof, wop, wr, wrf, wg, wu, wd,
               xn0, xn1, xna, qs, qa, qb, ks, ka, vs, va, ls, lsa, os_, osa, hs, outs, best, zv, pk, zs,
               sems):
        xn = (xn0, xn1)
        qq, kk = (qs, qa), (ks, ka)
        pending = []
        hist = []

        zz = [0]

        def new_block():
            hist.clear()
            pending.clear()
            zz[0] = pl.multiple_of(zs[0], 8)

        def dyn(name, start, n):
            if name in opaque:
                return pl.ds(zz[0] + start, n)
            return pl.ds(start, n)

        def emit_token(val_u32, d=1):
            pending.append((len(hist) + d - 1, val_u32))

        def take_due(t_now):
            due = [v for (c, v) in pending if c <= t_now]
            pending[:] = [(c, v) for (c, v) in pending if c > t_now]
            if not due:
                return None
            t = due.pop()
            while due:
                t = t | due.pop()
            return t & zv[...]

        def gated(w_u32):
            t = take_due(len(hist))
            if t is None:
                return w_u32
            return jnp.concatenate([w_u32[0:8] | t, w_u32[8:]], axis=0)

        def gate_after(lag):
            if len(hist) > lag:
                return pltpu.bitcast(hist[-1 - lag], u32) & zv[...]
            return None

        def row0(i):
            return i * T if isinstance(i, int) else pl.multiple_of(i * T, T)

        S_A, S_B, S_C = 0, 1, 2
        S_Q = [3 + c for c in range(NWQ)]

        def x_copy(t0, t1, sem):
            return pltpu.make_async_copy(x_hbm.at[pl.ds(t0 * T, (t1 - t0) * T)], xs.at[pl.ds(t0 * T, (t1 - t0) * T)],
                                         sems.at[sem])

        def w_copy(p, sem):
            return pltpu.make_async_copy(wqkv_hbm.at[:, pl.ds(p * D, D)], wraw.at[:, pl.ds(p * D, D)], sems.at[sem])

        WQR = D // NWQ

        def wq_copy(c):
            return pltpu.make_async_copy(wqkv_hbm.at[pl.ds(c * WQR, WQR), pl.ds(0, D)],
                                         wraw.at[pl.ds(c * WQR, WQR), pl.ds(0, D)], sems.at[S_Q[c]])

        x0_copy = x_copy(0, 1, S_A)
        x12_copy = x_copy(1, 3, S_B)
        wk_copy = w_copy(1, S_C)
        wv_copy = w_copy(2, S_A)
        grp_wo = [pltpu.make_async_copy(wr_hbm, wr, sems.at[S_Q[0]]),
                  pltpu.make_async_copy(wo_hbm, woraw, sems.at[S_Q[0]]),
                  x_copy(3, 4, S_Q[0])]
        xr_copy = x_copy(4, NT, S_Q[1])
        grp_ffn = [pltpu.make_async_copy(wg_hbm, wg, sems.at[S_B]),
                   pltpu.make_async_copy(wu_hbm, wu, sems.at[S_B]),
                   pltpu.make_async_copy(wd_hbm, wd, sems.at[S_B])]

        def o_copy(i):
            return pltpu.make_async_copy(outs.at[pl.ds(row0(i), T)], out_hbm.at[pl.ds(row0(i), T)], sems.at[S_C])

        def prep_w_pieces(p, lo=0, hi=D, PB=128, d=0):
            def sel(r0):
                lane = jax.lax.broadcasted_iota(i32, (PB // 2, 128), 1)
                r5 = (lane // 4) % 5
                src = [pltpu.bitcast(wraw[r0:r0 + PB, p * D + jj * 128: p * D + (jj + 1) * 128], u32)
                       for jj in range(NJ)]
                for j in range(NJ):
                    t = src[4]
                    for jj in range(4):
                        t = jnp.where(r5 == (j - 2 * jj) % 5, src[jj], t)
                    wt[r0 // 2:(r0 + PB) // 2, j * 128:(j + 1) * 128] = t
                    if d:
                        emit_token(t[PB // 2 - 8:PB // 2], d)

            def perm(j):
                lane = jax.lax.broadcasted_iota(i32, ((hi - lo) // 2, 128), 1)
                head = (lane % 32) // 2 + 16 * (lane % 2)
                idx = (20 * head + 4 * j + lane // 32) % 128
                wp[lo // 2:hi // 2, p * D + j * 128: p * D + (j + 1) * 128] = jnp.take_along_axis(
                    wt[lo // 2:hi // 2, j * 128:(j + 1) * 128], idx, axis=1)
            return ([functools.partial(sel, r0) for r0 in range(lo, hi, PB)]
                    + [functools.partial(perm, j) for j in range(NJ)])

        def prep_sched(p):
            ps = prep_w_pieces(p, 0, D, sel_pb, sel_d)
            return spread(ps[:-NJ], -1, sel_hi) + at(perm_sched, ps[-NJ:])

        def prep_wo_pieces(dl=0):
            def piece(j):
                wof[j] = woraw[:, j * 128:(j + 1) * 128].astype(f32)
                for d in range(DH):
                    blk = pack2(wof[j, pl.ds(d, H // 2, stride=DH), :],
                                wof[j, pl.ds(d + DH * (H // 2), H // 2, stride=DH), :])
                    wop[d * 16:(d + 1) * 16, j * 128:(j + 1) * 128] = blk
                    if dl and d % 4 == 3:
                        emit_token(blk[8:16], dl)
            return [functools.partial(piece, j) for j in range(NJ)]

        def ln_stats(x):
            m = jnp.sum(x, axis=-1, keepdims=True) * (1.0 / D)
            v = jnp.maximum(jnp.sum(x * x, axis=-1, keepdims=True) * (1.0 / D) - m * m, 0.0)
            return m, rsqrt(v + EPS)

        def a_pieces(i, dst, d=0):
            r = row0(i)

            def piece(b):
                if ilv_a:
                    xu = pltpu.bitcast(xs[pl.ds(r + b * LNB, LNB), :], u32)
                    ys = []
                    for half in range(2):
                        x = pltpu.unpack_elementwise(xu, index=half, packed_dtype=bf16, unpacked_dtype=f32)
                        m, rs = ln_stats(x)
                        ys.append(x * rs - m * rs)
                    yu = pack2(ys[0], ys[1])
                else:
                    x = xs[pl.ds(r + b * LNB, LNB), :].astype(f32)
                    m, rs = ln_stats(x)
                    yu = pltpu.bitcast((x * rs - m * rs).astype(bf16), u32)
                dst[dyn('xn', b * LNB // 2, LNB // 2), :] = yu
                if d:
                    for r8 in range(LNB // 16):
                        emit_token(yu[r8 * 8:r8 * 8 + 8, D - 128:D], d)
            return [functools.partial(piece, b) for b in range(T // LNB)]

        def b_slots(p, src, dst, halo=None):
            def slot(j):
                lhs = pltpu.bitcast(src[...], bf16)
                c = p * D + j * 128
                w = pltpu.bitcast(gated(wp[:, c:c + 128]), bf16)
                res = jnp.dot(lhs, w, preferred_element_type=f32)
                hist.append(res[0:8])
                if p == 0:
                    dst[j, dyn('q', 0, T), :] = res
                else:
                    if halo is None:
                        dst[j, 0:HALO, :] = jnp.zeros((HALO, 128), f32)
                    else:
                        dst[j, 0:HALO, :] = halo[j, T:T + HALO, :]
                    dst[j, dyn('kv', HALO, T), :] = res
            return [functools.partial(slot, j) for j in range(NJ)]

        def ldw(ref, j, start, n):
            if not ilv_pv:
                return ref[j, start:start + n, :]
            parts = []
            for g0 in range(start, start + n, 16):
                parts += [ref[j, pl.ds(g0, 8, stride=2), :], ref[j, pl.ds(g0 + 1, 8, stride=2), :]]
            return jnp.concatenate(parts, axis=0)

        def qk_pieces(qr, kr, lr, first=False):
            def piece(rb):
                r0 = rb * QB
                sv = jnp.full((8, 128), QSCALE, f32)
                g = gate_after(0)
                if g is not None:
                    sv = pltpu.bitcast(pltpu.bitcast(sv, u32) | g, f32)
                lw = []
                q = [(ldw(qr, j, r0, QB).reshape(QB // 8, 8, 128) * sv[None]).reshape(QB, 128) for j in range(NJ)]
                for w in range(NW):
                    lo = HALO + r0 - DIL * w
                    a = None
                    for j in range(NJ):
                        t = q[j] * ldw(kr, j, lo, QB)
                        a = t if a is None else a + t
                    a = a + pltpu.roll(a, 64, 1)
                    a = a + pltpu.roll(a, 32, 1)
                    if first and r0 < DIL * w:
                        rows = jax.lax.broadcasted_iota(i32, (QB, 128), 0)
                        if ilv_pv:
                            rows = (rows // 16) * 16 + (rows % 8) * 2 + (rows % 16) // 8
                        rows = rows + r0
                        a = jnp.where(rows >= DIL * w, a, -1e9)
                    if smqk:
                        lw.append(a)
                    else:
                        lr[w, dyn('ls', r0, QB), :] = a
                if smqk:
                    m = lw[0]
                    for w in range(1, NW):
                        m = jnp.maximum(m, lw[w])
                    es = [jnp.exp2(l - m) for l in lw]
                    s = es[0]
                    for w in range(1, NW):
                        s = s + es[w]
                    inv = pl.reciprocal(s, approx=True)
                    if smqk == 1:
                        for w in range(NW):
                            lr[w, dyn('ls', r0, QB), :] = es[w] * inv
                    else:
                        for w in range(NW):
                            lr[w, dyn('ls', r0, QB), :] = es[w]
                        lr[NW, dyn('ls', r0, QB), :] = inv
            return [functools.partial(piece, rb) for rb in range(T // QB)]

        def pv_pieces(lr, vr, orf, tok=True):
            def piece(rb):
                r0 = rb * RB
                lw = [lr[w, r0:r0 + RB, :] for w in range(NW)]
                g = gate_after(pv_lag) if tok else None

                def gt(m):
                    if g is None:
                        return m
                    return pltpu.bitcast((pltpu.bitcast(m, u32).reshape(RB // 8, 8, 128) | g[None]).reshape(RB, 128), f32)
                if smqk:
                    es = [gt(l) if w < pv_ng else l for w, l in enumerate(lw)]
                    inv = None if smqk == 1 else lr[NW, r0:r0 + RB, :]
                else:
                    m = lw[0]
                    for w in range(1, NW):
                        m = jnp.maximum(m, lw[w])
                    m = gt(m)
                    es = [jnp.exp2(l - m) for l in lw]
                    s = es[0]
                    for w in range(1, NW):
                        s = s + es[w]
                    inv = pl.reciprocal(s, approx=True)
                for j in range(NJ):
                    o = None
                    for w in range(NW):
                        lo = HALO + r0 - DIL * w
                        t = es[w] * ldw(vr, j, lo, RB)
                        o = t if o is None else o + t
                    o = o if inv is None else o * inv
                    if ilv_pv:
                        ob = jnp.concatenate([pack2(o[g0:g0 + 8], o[g0 + 8:g0 + 16]) for g0 in range(0, RB, 16)], axis=0)
                    else:
                        ob = pltpu.bitcast(o.astype(bf16), u32)
                    orf[dyn('os', r0 // 2, RB // 2), j * 128:(j + 1) * 128] = ob
                    if tok:
                        emit_token(ob[0:8])
            return [functools.partial(piece, rb) for rb in range(T // RB)]

        def d_slots(i, orf):
            r = row0(i)

            def slot(j):
                lhs = pltpu.bitcast(orf[...], bf16)
                w = pltpu.bitcast(gated(wop[:, j * 128:(j + 1) * 128]), bf16)
                res = jnp.dot(lhs, w, preferred_element_type=f32)
                hist.append(res[0:8])
                hs[pl.ds(r, T), j * 128:(j + 1) * 128] = res + xs[pl.ds(r, T), j * 128:(j + 1) * 128].astype(f32)
            return [functools.partial(slot, j) for j in range(NJ)]

        def e_pieces(i, par, d=0):
            r = row0(i)

            def piece(b):
                rr = r + b * LNB
                h = hs[pl.ds(pl.multiple_of(rr + zz[0], 8) if 'hs' in opaque else rr, LNB), :]
                m, rs = ln_stats(h)
                hw = (h.reshape(LNB // 8, 8, D) * wrf[0:8, :][None]).reshape(LNB, D)
                rv_all = (jnp.sum(hw, axis=-1, keepdims=True) - m * wrf[8:9, 0:1]) * rs
                ov = h * (1.0 + rs) - m * rs
                outs[pl.ds(rr, LNB), :] = ov.astype(bf16)
                bv = best[2 * par]
                bi = best[2 * par + 1]
                rows = (jax.lax.broadcasted_iota(i32, (8, 128), 0) + rr).astype(f32)
                for rb in range(LNB // 8):
                    rv = jnp.broadcast_to(rv_all[rb * 8:(rb + 1) * 8, :], (8, 128))
                    upd = rv > bv
                    bv = jnp.where(upd, rv, bv)
                    bi = jnp.where(upd, rows + float(rb * 8), bi)
                if d:
                    for r8 in range(LNB // 8):
                        emit_token(pltpu.bitcast(ov[r8 * 8:r8 * 8 + 8, D - 128:D], u32), d)
                    emit_token(pltpu.bitcast(bv, u32), d)
                best[2 * par] = bv
                best[2 * par + 1] = bi
                if b == T // LNB - 1:
                    o_copy(i).start()
            return [functools.partial(piece, b) for b in range(T // LNB)]

        K4 = 512

        def g_dot(src, wref, c0, n, slot0, add_x=None, tok=True):
            wu = wref[K4 // 2:, c0 * 128:(c0 + n) * 128]
            if tok:
                t = take_due(len(hist))
                if t is not None:
                    top = jnp.concatenate([wu[0:8, 0:128] | t, wu[0:8, 128:]], axis=1) if n > 1 else wu[0:8] | t
                    wu = jnp.concatenate([top, wu[8:]], axis=0)
            lhs = pltpu.bitcast(src[:, K4:], bf16)
            res = jnp.dot(lhs, pltpu.bitcast(wu, bf16), preferred_element_type=f32)
            for u in range(n):
                r = res[:, u * 128:(u + 1) * 128]
                if add_x is not None:
                    r = r + xs[pl.ds(add_x, T), (c0 + u) * 128:(c0 + u + 1) * 128].astype(f32)
                pk[slot0 + u, dyn('pk', 0, T), :] = r
            return res[0:8, 0:128]

        def gb_slot(src, c0):
            def slot():
                hist.append(g_dot(src, wp, c0, 4, c0))
            return slot

        def gd_slots(i, src, orf):
            r = row0(i)

            def s0():
                hist.append(g_dot(orf, wop, 0, 4, 15, r))

            def s1():
                hist.append(g_dot(orf, wop, 4, 1, 19, r))
                g_dot(src, wp, 12, 3, 12, tok=False)
            return [s0, s1]

        def b4_slots(p, src, dst, halo):
            def slot(j):
                c = p * D + j * 128
                w = pltpu.bitcast(gated(wp[0:K4 // 2, c:c + 128]), bf16)
                lhs = pltpu.bitcast(src[:, 0:K4], bf16)
                res = jnp.dot(lhs, w, preferred_element_type=f32)
                hist.append(res[0:8])
                res = res + pk[p * NJ + j, 0:T, :]
                if p == 0:
                    dst[j, dyn('q', 0, T), :] = res
                else:
                    dst[j, 0:HALO, :] = halo[j, T:T + HALO, :]
                    dst[j, dyn('kv', HALO, T), :] = res
            return [functools.partial(slot, j) for j in range(NJ)]

        def d4_slots(i, orf):
            r = row0(i)

            def slot(j):
                w = pltpu.bitcast(gated(wop[0:K4 // 2, j * 128:(j + 1) * 128]), bf16)
                lhs = pltpu.bitcast(orf[:, 0:K4], bf16)
                res = jnp.dot(lhs, w, preferred_element_type=f32)
                hist.append(res[0:8])
                hs[pl.ds(r, T), j * 128:(j + 1) * 128] = res + pk[15 + j, 0:T, :]
            return [functools.partial(slot, j) for j in range(NJ)]

        def step(i, par, has_a=True):
            pieces = []
            src = xn[1 - par]
            qn, kn, kp = (qq[1 - par], kk[1 - par], kk[par]) if qkpar else (qs, ks, ks)
            if ksplit:
                slots = ([gb_slot(src, 0), gb_slot(src, 4), gb_slot(src, 8)]
                         + b4_slots(0, src, qn, None) + b4_slots(1, src, kn, kp)
                         + gd_slots(i, src, os_) + d4_slots(i, os_) + b4_slots(2, src, vs, vs))
            else:
                slots = b_slots(0, src, qn) + b_slots(1, src, kn, kp) + d_slots(i, os_) + b_slots(2, src, vs, vs)
            pieces += at(e_sched, e_pieces(i - 1, par, e_d))
            pieces += at(pv_sched, pv_pieces(ls, vs, os_))
            pieces += at(qk_sched, qk_pieces(qn, kn, ls))
            if has_a:
                pieces += at(a_sched, a_pieces(i + 2, xn[par], a_d))
            interleave(slots, pieces)

        def blk(name, f):
            return f if only in (None, name) else (lambda *a, **k: None)

        cur = [None]

        def mark(name):
            if not scopes:
                return
            if cur[0] is not None:
                cur[0].__exit__(None, None, None)
                cur[0] = None
            if name:
                cur[0] = jax.named_scope(name)
                cur[0].__enter__()

        mark("s0_start")
        x0_copy.start()
        for c in range(NWQ):
            wq_copy(c).start()
        x12_copy.start()
        wk_copy.start()
        zv[...] = jnp.zeros((8, 128), u32)
        zs[0] = 0
        for par in range(2):
            best[2 * par] = jnp.full((8, 128), -jnp.inf, f32)
            best[2 * par + 1] = jnp.zeros((8, 128), f32)
        x0_copy.wait()
        for p in a_pieces(0, xna):
            p()
        for c in range(NWQ):
            wq_copy(c).wait()
            for p in prep_w_pieces(0, c * WQR, (c + 1) * WQR, WQR // 2 if WQR % 32 == 0 else WQR):
                p()
        x12_copy.wait()
        mark('s1_X')
        wv_copy.start()
        new_block()
        blk('X', interleave)(b_slots(0, xna, qa) + b_slots(0, xn[1], qb),
                   spread(a_pieces(1, xn[1]), 0, 2) + spread(a_pieces(2, xn[0], 2), 5, 8))
        mark('s2_waitWk')
        wk_copy.wait()
        mark('s3_X2')
        for c in grp_wo:
            c.start()
        new_block()
        blk('X2', interleave)(b_slots(0, xn[0], qs) + b_slots(1, xna, ka), prep_sched(1))
        mark('s4_waitWv')
        wv_copy.wait()
        mark('s5_Y')
        xr_copy.start()
        new_block()
        blk('Y', interleave)(b_slots(1, xn[1], ks, ka) + b_slots(2, xna, va) + b_slots(2, xn[1], vs, va),
                   prep_sched(2)
                   + at(y_qk0, qk_pieces(qa, ka, lsa, True))
                   + at(y_qk1, qk_pieces(qb, ks, ls))
                   + at(y_pv, pv_pieces(lsa, va, osa, y_pvtok)))
        mark('s6_waitWo')
        for c in grp_wo:
            c.wait()
        mark('s7_Z')
        for c in grp_ffn:
            c.start()
        new_block()
        wrv = jnp.broadcast_to(wr[...].astype(f32).reshape(1, D), (8, D))
        wrf[0:8, :] = wrv
        wrf[8:16, :] = jnp.broadcast_to(jnp.sum(wrv, axis=-1, keepdims=True), (8, D))
        blk('Z', interleave)(b_slots(1, xn[0], ks, ks) + d_slots(0, osa) + d_slots(1, os_) + b_slots(2, xn[0], vs, vs),
                   at(z_wo, prep_wo_pieces(z_wod))
                   + at(z_pv, pv_pieces(ls, vs, os_))
                   + at(z_qk, qk_pieces(qs, ks, ls))
                   + at(z_e, e_pieces(0, 0, z_ed))
                   + at(z_a, a_pieces(3, xn[1], z_ad)))

        first = 2
        nloop = (NT - 2 - first) // unroll

        def body(k, c):
            i0 = first + k * unroll
            new_block()
            for u in range(unroll):
                blk('loop', step)(i0 + u, (first + u) % 2)
            return c

        xr_copy.wait()
        mark('s8_loop')
        jax.lax.fori_loop(0, nloop, body, 0)
        mark('s9_tail')
        rest = list(range(first + nloop * unroll, NT - 2))
        new_block()
        for i in rest:
            step(i, i % 2)
        L = NT - 1
        src = xn[L % 2]
        qn, kn, kp = (qq[L % 2], kk[L % 2], kk[1 - L % 2]) if qkpar else (qs, ks, ks)
        blk('tail', interleave)(b_slots(0, src, qn) + b_slots(1, src, kn, kp) + b_slots(2, src, va, vs)
                   + d_slots(L - 1, os_) + d_slots(L, osa),
                   at(t_e0, e_pieces(L - 2, L % 2, t_ed0))
                   + at(t_pv0, pv_pieces(ls, vs, os_))
                   + at(t_qk, qk_pieces(qn, kn, lsa))
                   + at(t_pv, pv_pieces(lsa, va, osa, t_pvtok))
                   + at(t_e, e_pieces(L - 1, (L - 1) % 2, t_ed))
                   + spread(e_pieces(L, L % 2), 25, 26))

        mark('sa_ffn')
        bv = jnp.concatenate([best[0], best[2]], axis=0)
        bi = jnp.concatenate([best[1], best[3]], axis=0)
        mx = jnp.max(bv, axis=0, keepdims=True)
        cand = jnp.where(bv == mx, bi, float(S))
        idx_v = jnp.min(cand, axis=0, keepdims=True)
        idx = jnp.minimum(jnp.min(idx_v).astype(i32), S - 1)
        base = pl.multiple_of((idx // 16) * 16, 16)
        h16 = hs[pl.ds(base, 16), :]
        m16, rs16 = ln_stats(h16)
        hn16 = (h16 - m16) * rs16
        xb = hn16.astype(bf16)
        for c in grp_ffn:
            c.wait()
        g = jnp.dot(xb, wg[...], preferred_element_type=f32)
        u = jnp.dot(xb, wu[...], preferred_element_type=f32)
        act = (g * jax.nn.sigmoid(g) * u).astype(bf16)
        y = jnp.dot(act, wd[...], preferred_element_type=f32)
        gate = jax.nn.sigmoid(mx[:, 0:1])
        rows16 = jax.lax.broadcasted_iota(i32, (16, D), 0)
        y = jnp.where(rows16 == idx - base, y * gate, 0.0)
        mark('sb_owait')
        pltpu.make_async_copy(outs, out_hbm, sems.at[S_C]).wait()
        mark('sc_fix')
        outs[pl.ds(base, 16), :] = (h16 + hn16 + y).astype(bf16)
        fix = pltpu.make_async_copy(outs.at[pl.ds(base, 16)], out_hbm.at[pl.ds(base, 16)], sems.at[S_A])
        fix.start()
        fix.wait()
        mark(None)

    lhs_buf = pltpu.VMEM((T // 2, D), u32)
    q_buf = pltpu.VMEM((NJ, T + padq, 128), f32)
    kv_buf = pltpu.VMEM((NJ, T + HALO + padk, 128), f32)
    l_buf = pltpu.VMEM((NW + 1, T + padl, 128), f32)
    scratch = [
        pltpu.VMEM((S, D), bf16),
        pltpu.VMEM((D, 3 * D), bf16),
        pltpu.VMEM((D // 2, D), u32),
        pltpu.VMEM((D // 2, 3 * D), u32),
        pltpu.VMEM((D, D), bf16),
        pltpu.VMEM((NJ, D, 128), f32),
        pltpu.VMEM((D // 2, D), u32),
        pltpu.VMEM((D,), bf16),
        pltpu.VMEM((16, D), f32),
        pltpu.VMEM((D, F), bf16),
        pltpu.VMEM((D, F), bf16),
        pltpu.VMEM((F, D), bf16),
        lhs_buf, lhs_buf, lhs_buf,
        q_buf, q_buf, q_buf,
        kv_buf, kv_buf, kv_buf, kv_buf,
        l_buf, l_buf,
        lhs_buf, lhs_buf,
        pltpu.VMEM((S, D), f32),
        pltpu.VMEM((S, D), bf16),
        pltpu.VMEM((4, 8, 128), f32),
        pltpu.VMEM((8, 128), u32),
        pltpu.VMEM((20, T + padq, 128), f32),
        pltpu.SMEM((1,), i32),
        pltpu.SemaphoreType.DMA((3 + NWQ,)),
    ]
    return kernel, scratch


def build(**kw):
    nobc = kw.get('nobc', True)
    kernel, scratch = make_kernel(**kw)

    def fn(A_x, A_wqkv, A_wo, B_x, B_w_r, B_w_gate, B_w_up, B_w_down):
        x2 = A_x.reshape(S, D)
        out = pl.pallas_call(
            kernel,
            in_specs=[pl.BlockSpec(memory_space=pl.ANY)] * 7,
            out_specs=pl.BlockSpec(memory_space=pl.ANY),
            out_shape=jax.ShapeDtypeStruct((S, D), bf16),
            scratch_shapes=scratch,
            name="fused",
            compiler_params=pltpu.CompilerParams(vmem_limit_bytes=100 * 2**20, disable_bounds_checks=nobc),
        )(x2, A_wqkv, A_wo, B_w_r, B_w_gate, B_w_up, B_w_down)
        return out.reshape(1, S, D)
    return fn


_fn = build()


@jax.jit
def pallas_sequential_preLN__sliding_local_dilated__moe_arch_mod__prompt_kernel(
    A_x: jax.Array,
    A_wqkv: jax.Array,
    A_wo: jax.Array,
    B_x: jax.Array,
    B_w_r: jax.Array,
    B_w_gate: jax.Array,
    B_w_up: jax.Array,
    B_w_down: jax.Array,
):
    return _fn(A_x, A_wqkv, A_wo, B_x, B_w_r, B_w_gate, B_w_up, B_w_down)
```

```python
import functools
import math
import jax
import jax.numpy as jnp
from jax.experimental import pallas as pl
from jax.experimental.pallas import tpu as pltpu

S, D, H, DH, F = 2048, 640, 32, 20, 1536
NW, DIL = 8, 2
HALO = 16
NJ = D // 128
EPS = 1e-5
QSCALE = (DH ** -0.5) * math.log2(math.e)
f32, bf16, u32, i32 = jnp.float32, jnp.bfloat16, jnp.uint32, jnp.int32


def interleave(slots, pieces):
    pieces = sorted(pieces, key=lambda kp: kp[0])
    for k, p in pieces:
        if k < 0:
            p()
    for c, s in enumerate(slots):
        s()
        for k, p in pieces:
            if k == c:
                p()
    for k, p in pieces:
        if k >= len(slots):
            p()


def spread(pieces, lo, hi):
    n = len(pieces)
    return [(lo + (k * (hi - lo)) // n, p) for k, p in enumerate(pieces)]


def at(sched, pieces, off=0):
    k = len(pieces) // len(sched)
    sched = [c for c in sched for _ in range(k)]
    return [(c + off, p) for c, p in zip(sched, pieces, strict=True)]


def pack2(even, odd):
    p = pltpu.pack_elementwise([even, odd], packed_dtype=bf16)
    return p if p.dtype == u32 else pltpu.bitcast(p, u32)


def rsqrt(v):
    return jnp.exp2(jnp.log2(v) * -0.5)


def make_kernel(T=128, LNB=64, RB=16, QB=16, unroll=4,
                pv_sched=(3, 4, 6, 7, 8, 10, 11, 12), pv_lag=2,
                a_sched=(20, 21), a_d=3,
                e_sched=(-1, 1), e_d=5,
                qk_sched=(12, 13, 14, 15, 16, 17, 18, 19), NWQ=4, only=None, ksplit=True, opaque=(), smqk=0, dlag=1, t_in=6,
                t_act=(8, 9, 10, 11, 12, 13, 14, 15, 16, 17, 18, 19, 20, 21, 22, 23, 23, 24, 24, 24, 24, 24, 24, 24), sel_pb=64, sel_d=0, sel_hi=2, perm_sched=(2, 2, 3, 3, 4), z_wo=(-1, 0, 1, 2, 3), z_wod=0, ilv_a=True, ilv_pv=True, qkpar=True, areload=False, pv_ng=1, nobc=True, padq=8, padl=8, padk=24, padp=8, t_e0=(-1, 0), t_ed0=4,
                y_qk0=(1, 2, 3, 4, 5, 5, 5, 8), y_qk1=(6, 7, 7, 8, 10, 11, 12, 12), y_pv=(10, 10, 11, 11, 12, 12, 13, 13), y_pvtok=False,
                z_pv=(2, 3, 4, 5, 6, 7, 8, 9), z_qk=(10, 11, 12, 13, 14, 15, 16, 16), z_e=(13, 16), z_ed=1, z_a=(16, 17), z_ad=2,
                t_pvtok=False, t_pv0=(3, 4, 5, 6, 7, 8, 9, 10), t_ed=2,
                t_qk=(9, 10, 11, 11, 11, 11, 12, 13), t_pv=(16, 17, 18, 19, 19, 19, 19, 19), t_e=(21, 22), scopes=False):
    NT = S // T

    def kernel(x_hbm, wqkv_hbm, wo_hbm, wr_hbm, wg_hbm, wu_hbm, wd_hbm, out_hbm,
               xs, wraw, wt, wp, woraw, wof, wop, wr, wrf, wg, wu, wd,
               xn0, xn1, xna, qs, qa, qb, ks, ka, vs, va, ls, lsa, os_, osa, hs, outs, best, zv, pk, zs, fixbuf,
               sems):
        x_u, wqkv_u, wo_u, wg_u, wu_u, wd_u = [r.bitcast(u32) for r in (x_hbm, wqkv_hbm, wo_hbm, wg_hbm, wu_hbm, wd_hbm)]
        xn = (xn0, xn1)
        qq, kk = (qs, qa), (ks, ka)
        pending = []
        hist = []

        zz = [0]

        def new_block():
            hist.clear()
            pending.clear()
            zz[0] = pl.multiple_of(zs[0], 8)

        def dyn(name, start, n):
            if name in opaque:
                return pl.ds(zz[0] + start, n)
            return pl.ds(start, n)

        def emit_token(val_u32, d=1):
            pending.append((len(hist) + d - 1, val_u32))

        def take_due(t_now):
            due = [v for (c, v) in pending if c <= t_now]
            pending[:] = [(c, v) for (c, v) in pending if c > t_now]
            if not due:
                return None
            t = due.pop()
            while due:
                t = t | due.pop()
            return t & zv[...]

        def gated(w_u32):
            t = take_due(len(hist))
            if t is None:
                return w_u32
            return jnp.concatenate([w_u32[0:8] | t, w_u32[8:]], axis=0)

        def gate_after(lag):
            if len(hist) > lag:
                return pltpu.bitcast(hist[-1 - lag], u32) & zv[...]
            return None

        def xrows(r, n):
            h = r // 2 if isinstance(r, int) else pl.multiple_of(r // 2, 8)
            return pl.ds(h, n // 2)

        def row0(i):
            return i * T if isinstance(i, int) else pl.multiple_of(i * T, T)

        S_A, S_B, S_C = 0, 1, 2
        S_Q = [3 + c for c in range(NWQ)]

        def x_copy(t0, t1, sem):
            rows = pl.ds(t0 * T // 2, (t1 - t0) * T // 2)
            return pltpu.make_async_copy(x_u.at[rows], xs.at[rows], sems.at[sem])

        def w_copy(p, sem):
            return pltpu.make_async_copy(wqkv_u.at[:, pl.ds(p * D, D)], wraw.at[:, pl.ds(p * D, D)], sems.at[sem])

        WQR = D // NWQ

        def wq_copy(c):
            rows = pl.ds(c * WQR // 2, WQR // 2)
            return pltpu.make_async_copy(wqkv_u.at[rows, pl.ds(0, D)], wraw.at[rows, pl.ds(0, D)], sems.at[S_Q[c]])

        x0_copy = x_copy(0, 1, S_A)
        x12_copy = x_copy(1, 3, S_B)
        wk_copy = w_copy(1, S_C)
        wv_copy = w_copy(2, S_A)
        grp_wo = [pltpu.make_async_copy(wr_hbm, wr, sems.at[S_Q[0]]),
                  pltpu.make_async_copy(wo_u, woraw, sems.at[S_Q[0]]),
                  x_copy(3, 4, S_Q[0])]
        xr_copy = x_copy(4, NT, S_Q[1])
        grp_ffn = [pltpu.make_async_copy(wg_u, wg, sems.at[S_B]),
                   pltpu.make_async_copy(wu_u, wu, sems.at[S_B]),
                   pltpu.make_async_copy(wd_u, wd, sems.at[S_B])]

        NLAST = 2

        def o_copy(r, n, late):
            return pltpu.make_async_copy(outs.at[pl.ds(r, n)], out_hbm.at[pl.ds(r, n)], sems.at[S_B if late else S_C])

        def prep_w_pieces(p, lo=0, hi=D, PB=128, d=0):
            def sel(r0):
                lane = jax.lax.broadcasted_iota(i32, (PB // 2, 128), 1)
                r5 = (lane // 4) % 5
                src = [wraw[r0 // 2:(r0 + PB) // 2, p * D + jj * 128: p * D + (jj + 1) * 128] for jj in range(NJ)]
                for j in range(NJ):
                    t = src[4]
                    for jj in range(4):
                        t = jnp.where(r5 == (j - 2 * jj) % 5, src[jj], t)
                    wt[r0 // 2:(r0 + PB) // 2, j * 128:(j + 1) * 128] = t
                    if d:
                        emit_token(t[PB // 2 - 8:PB // 2], d)

            def perm(j):
                lane = jax.lax.broadcasted_iota(i32, ((hi - lo) // 2, 128), 1)
                head = (lane % 32) // 2 + 16 * (lane % 2)
                idx = (20 * head + 4 * j + lane // 32) % 128
                wp[lo // 2:hi // 2, p * D + j * 128: p * D + (j + 1) * 128] = jnp.take_along_axis(
                    wt[lo // 2:hi // 2, j * 128:(j + 1) * 128], idx, axis=1)
            return ([functools.partial(sel, r0) for r0 in range(lo, hi, PB)]
                    + [functools.partial(perm, j) for j in range(NJ)])

        def prep_sched(p):
            ps = prep_w_pieces(p, 0, D, sel_pb, sel_d)
            return spread(ps[:-NJ], -1, sel_hi) + at(perm_sched, ps[-NJ:])

        def prep_wo_pieces(dl=0):
            def piece(j):
                wof[j] = pltpu.bitcast(woraw[:, j * 128:(j + 1) * 128], bf16).astype(f32)
                for d in range(DH):
                    blk = pack2(wof[j, pl.ds(d, H // 2, stride=DH), :],
                                wof[j, pl.ds(d + DH * (H // 2), H // 2, stride=DH), :])
                    wop[d * 16:(d + 1) * 16, j * 128:(j + 1) * 128] = blk
                    if dl and d % 4 == 3:
                        emit_token(blk[8:16], dl)
            return [functools.partial(piece, j) for j in range(NJ)]

        def ln_stats(x):
            m = jnp.sum(x, axis=-1, keepdims=True) * (1.0 / D)
            v = jnp.maximum(jnp.sum(x * x, axis=-1, keepdims=True) * (1.0 / D) - m * m, 0.0)
            return m, rsqrt(v + EPS)

        def a_pieces(i, dst, d=0):
            r = row0(i)

            def piece(b):
                if ilv_a:
                    xu = xs[xrows(r + b * LNB, LNB), :]
                    ys = []
                    for half in range(2):
                        x = pltpu.unpack_elementwise(xu, index=half, packed_dtype=bf16, unpacked_dtype=f32)
                        m, rs = ln_stats(x)
                        ys.append(x * rs - m * rs)
                    yu = pack2(ys[0], ys[1])
                else:
                    x = pltpu.bitcast(xs[xrows(r + b * LNB, LNB), :], bf16).astype(f32)
                    m, rs = ln_stats(x)
                    yu = pltpu.bitcast((x * rs - m * rs).astype(bf16), u32)
                dst[dyn('xn', b * LNB // 2, LNB // 2), :] = yu
                if d:
                    for r8 in range(LNB // 16):
                        emit_token(yu[r8 * 8:r8 * 8 + 8, D - 128:D], d)
            return [functools.partial(piece, b) for b in range(T // LNB)]

        def b_slots(p, src, dst, halo=None):
            def slot(j):
                lhs = pltpu.bitcast(src[...], bf16)
                c = p * D + j * 128
                w = pltpu.bitcast(gated(wp[:, c:c + 128]), bf16)
                res = jnp.dot(lhs, w, preferred_element_type=f32)
                hist.append(res[0:8])
                if p == 0:
                    dst[j, dyn('q', 0, T), :] = res
                else:
                    if halo is None:
                        dst[j, 0:HALO, :] = jnp.zeros((HALO, 128), f32)
                    else:
                        dst[j, 0:HALO, :] = halo[j, T:T + HALO, :]
                    dst[j, dyn('kv', HALO, T), :] = res
            return [functools.partial(slot, j) for j in range(NJ)]

        def ldw(ref, j, start, n):
            if not ilv_pv:
                return ref[j, start:start + n, :]
            parts = []
            for g0 in range(start, start + n, 16):
                parts += [ref[j, pl.ds(g0, 8, stride=2), :], ref[j, pl.ds(g0 + 1, 8, stride=2), :]]
            return jnp.concatenate(parts, axis=0)

        def qk_pieces(qr, kr, lr, first=False):
            def piece(rb):
                r0 = rb * QB
                sv = jnp.full((8, 128), QSCALE, f32)
                g = gate_after(0)
                if g is not None:
                    sv = pltpu.bitcast(pltpu.bitcast(sv, u32) | g, f32)
                lw = []
                q = [(ldw(qr, j, r0, QB).reshape(QB // 8, 8, 128) * sv[None]).reshape(QB, 128) for j in range(NJ)]
                for w in range(NW):
                    lo = HALO + r0 - DIL * w
                    a = None
                    for j in range(NJ):
                        t = q[j] * ldw(kr, j, lo, QB)
                        a = t if a is None else a + t
                    a = a + pltpu.roll(a, 64, 1)
                    a = a + pltpu.roll(a, 32, 1)
                    if first and r0 < DIL * w:
                        rows = jax.lax.broadcasted_iota(i32, (QB, 128), 0)
                        if ilv_pv:
                            rows = (rows // 16) * 16 + (rows % 8) * 2 + (rows % 16) // 8
                        rows = rows + r0
                        a = jnp.where(rows >= DIL * w, a, -1e9)
                    if smqk:
                        lw.append(a)
                    else:
                        lr[w, dyn('ls', r0, QB), :] = a
                if smqk:
                    m = lw[0]
                    for w in range(1, NW):
                        m = jnp.maximum(m, lw[w])
                    es = [jnp.exp2(l - m) for l in lw]
                    s = es[0]
                    for w in range(1, NW):
                        s = s + es[w]
                    inv = pl.reciprocal(s, approx=True)
                    if smqk == 1:
                        for w in range(NW):
                            lr[w, dyn('ls', r0, QB), :] = es[w] * inv
                    else:
                        for w in range(NW):
                            lr[w, dyn('ls', r0, QB), :] = es[w]
                        lr[NW, dyn('ls', r0, QB), :] = inv
            return [functools.partial(piece, rb) for rb in range(T // QB)]

        def pv_pieces(lr, vr, orf, tok=True):
            def piece(rb):
                r0 = rb * RB
                lw = [lr[w, r0:r0 + RB, :] for w in range(NW)]
                g = gate_after(pv_lag) if tok else None

                def gt(m):
                    if g is None:
                        return m
                    return pltpu.bitcast((pltpu.bitcast(m, u32).reshape(RB // 8, 8, 128) | g[None]).reshape(RB, 128), f32)
                if smqk:
                    es = [gt(l) if w < pv_ng else l for w, l in enumerate(lw)]
                    inv = None if smqk == 1 else lr[NW, r0:r0 + RB, :]
                else:
                    m = lw[0]
                    for w in range(1, NW):
                        m = jnp.maximum(m, lw[w])
                    m = gt(m)
                    es = [jnp.exp2(l - m) for l in lw]
                    s = es[0]
                    for w in range(1, NW):
                        s = s + es[w]
                    inv = pl.reciprocal(s, approx=True)
                for j in range(NJ):
                    o = None
                    for w in range(NW):
                        lo = HALO + r0 - DIL * w
                        t = es[w] * ldw(vr, j, lo, RB)
                        o = t if o is None else o + t
                    o = o if inv is None else o * inv
                    if ilv_pv:
                        ob = jnp.concatenate([pack2(o[g0:g0 + 8], o[g0 + 8:g0 + 16]) for g0 in range(0, RB, 16)], axis=0)
                    else:
                        ob = pltpu.bitcast(o.astype(bf16), u32)
                    orf[dyn('os', r0 // 2, RB // 2), j * 128:(j + 1) * 128] = ob
                    if tok:
                        emit_token(ob[0:8])
            return [functools.partial(piece, rb) for rb in range(T // RB)]

        def d_slots(i, orf):
            r = row0(i)

            def slot(j):
                lhs = pltpu.bitcast(orf[...], bf16)
                w = pltpu.bitcast(gated(wop[:, j * 128:(j + 1) * 128]), bf16)
                res = jnp.dot(lhs, w, preferred_element_type=f32)
                hist.append(res[0:8])
                hs[pl.ds(r, T), j * 128:(j + 1) * 128] = res + pltpu.bitcast(xs[xrows(r, T), j * 128:(j + 1) * 128], bf16).astype(f32)
            return [functools.partial(slot, j) for j in range(NJ)]

        def e_pieces(i, par, d=0):
            r = row0(i)

            def piece(b):
                rr = r + b * LNB
                h = hs[pl.ds(pl.multiple_of(rr + zz[0], 8) if 'hs' in opaque else rr, LNB), :]
                m, rs = ln_stats(h)
                hw = (h.reshape(LNB // 8, 8, D) * wrf[0:8, :][None]).reshape(LNB, D)
                rv_all = (jnp.sum(hw, axis=-1, keepdims=True) - m * wrf[8:9, 0:1]) * rs
                ov = h * (1.0 + rs) - m * rs
                outs[pl.ds(rr, LNB), :] = ov.astype(bf16)
                bv = best[2 * par]
                bi = best[2 * par + 1]
                rows = (jax.lax.broadcasted_iota(i32, (8, 128), 0) + rr).astype(f32)
                for rb in range(LNB // 8):
                    rv = jnp.broadcast_to(rv_all[rb * 8:(rb + 1) * 8, :], (8, 128))
                    upd = rv > bv
                    bv = jnp.where(upd, rv, bv)
                    bi = jnp.where(upd, rows + float(rb * 8), bi)
                if d:
                    for r8 in range(LNB // 8):
                        emit_token(pltpu.bitcast(ov[r8 * 8:r8 * 8 + 8, D - 128:D], u32), d)
                    emit_token(pltpu.bitcast(bv, u32), d)
                best[2 * par] = bv
                best[2 * par + 1] = bi
                late = isinstance(i, int) and i >= NT - NLAST
                if isinstance(i, int) and i == NT - 1:
                    o_copy(rr, LNB, late).start()
                elif b == T // LNB - 1:
                    o_copy(r, T, late).start()
            return [functools.partial(piece, b) for b in range(T // LNB)]

        K4 = 512

        def g_dot(src, wref, c0, n, slot0, add_x=None, tok=True):
            wu = wref[K4 // 2:, c0 * 128:(c0 + n) * 128]
            if tok:
                t = take_due(len(hist))
                if t is not None:
                    top = jnp.concatenate([wu[0:8, 0:128] | t, wu[0:8, 128:]], axis=1) if n > 1 else wu[0:8] | t
                    wu = jnp.concatenate([top, wu[8:]], axis=0)
            lhs = pltpu.bitcast(src[:, K4:], bf16)
            res = jnp.dot(lhs, pltpu.bitcast(wu, bf16), preferred_element_type=f32)
            for u in range(n):
                r = res[:, u * 128:(u + 1) * 128]
                if add_x is not None:
                    r = r + pltpu.bitcast(xs[xrows(add_x, T), (c0 + u) * 128:(c0 + u + 1) * 128], bf16).astype(f32)
                pk[slot0 + u, dyn('pk', 0, T), :] = r
            return res[0:8, 0:128]

        def gb_slot(src, c0):
            def slot():
                hist.append(g_dot(src, wp, c0, 4, c0))
            return slot

        def gd_slots(i, src, orf):
            r = row0(i)

            def s0():
                hist.append(g_dot(orf, wop, 0, 4, 15, r))

            def s1():
                hist.append(g_dot(orf, wop, 4, 1, 19, r))
                g_dot(src, wp, 12, 3, 12, tok=False)
            return [s0, s1]

        def b4_slots(p, src, dst, halo):
            def slot(j):
                c = p * D + j * 128
                w = pltpu.bitcast(gated(wp[0:K4 // 2, c:c + 128]), bf16)
                lhs = pltpu.bitcast(src[:, 0:K4], bf16)
                res = jnp.dot(lhs, w, preferred_element_type=f32)
                hist.append(res[0:8])
                res = res + pk[p * NJ + j, 0:T, :]
                if p == 0:
                    dst[j, dyn('q', 0, T), :] = res
                else:
                    dst[j, 0:HALO, :] = halo[j, T:T + HALO, :]
                    dst[j, dyn('kv', HALO, T), :] = res
            return [functools.partial(slot, j) for j in range(NJ)]

        def d4_slots(i, orf):
            r = row0(i)

            def slot(j):
                w = pltpu.bitcast(gated(wop[0:K4 // 2, j * 128:(j + 1) * 128]), bf16)
                lhs = pltpu.bitcast(orf[:, 0:K4], bf16)
                res = jnp.dot(lhs, w, preferred_element_type=f32)
                hist.append(res[0:8])
                hs[pl.ds(r, T), j * 128:(j + 1) * 128] = res + pk[15 + j, 0:T, :]
            return [functools.partial(slot, j) for j in range(NJ)]

        def step(i, par, has_a=True):
            pieces = []
            src = xn[1 - par]
            qn, kn, kp = (qq[1 - par], kk[1 - par], kk[par]) if qkpar else (qs, ks, ks)
            if ksplit:
                slots = ([gb_slot(src, 0), gb_slot(src, 4), gb_slot(src, 8)]
                         + b4_slots(0, src, qn, None) + b4_slots(1, src, kn, kp)
                         + gd_slots(i, src, os_) + d4_slots(i, os_) + b4_slots(2, src, vs, vs))
            else:
                slots = b_slots(0, src, qn) + b_slots(1, src, kn, kp) + d_slots(i, os_) + b_slots(2, src, vs, vs)
            pieces += at(e_sched, e_pieces(i - 1, par, e_d))
            pieces += at(pv_sched, pv_pieces(ls, vs, os_))
            pieces += at(qk_sched, qk_pieces(qn, kn, ls))
            if has_a:
                pieces += at(a_sched, a_pieces(i + 2, xn[par], a_d))
            interleave(slots, pieces)

        def blk(name, f):
            return f if only is None or name in only else (lambda *a, **k: None)

        cur = [None]

        def mark(name):
            if not scopes:
                return
            if cur[0] is not None:
                cur[0].__exit__(None, None, None)
                cur[0] = None
            if name:
                cur[0] = jax.named_scope(name)
                cur[0].__enter__()

        mark("s0_start")
        x0_copy.start()
        for c in range(NWQ):
            wq_copy(c).start()
        x12_copy.start()
        wk_copy.start()
        zv[...] = jnp.zeros((8, 128), u32)
        zs[0] = 0
        for par in range(2):
            best[2 * par] = jnp.full((8, 128), -jnp.inf, f32)
            best[2 * par + 1] = jnp.zeros((8, 128), f32)
        x0_copy.wait()
        for p in a_pieces(0, xna):
            p()
        for c in range(NWQ):
            wq_copy(c).wait()
            for p in prep_w_pieces(0, c * WQR, (c + 1) * WQR, WQR // 2 if WQR % 32 == 0 else WQR):
                p()
        x12_copy.wait()
        mark('s1_X')
        wv_copy.start()
        new_block()
        blk('X', interleave)(b_slots(0, xna, qa) + b_slots(0, xn[1], qb),
                   spread(a_pieces(1, xn[1]), 0, 2) + spread(a_pieces(2, xn[0], 2), 5, 8))
        mark('s2_waitWk')
        wk_copy.wait()
        mark('s3_X2')
        for c in grp_wo:
            c.start()
        new_block()
        blk('X2', interleave)(b_slots(0, xn[0], qs) + b_slots(1, xna, ka), prep_sched(1))
        mark('s4_waitWv')
        wv_copy.wait()
        mark('s5_Y')
        xr_copy.start()
        new_block()
        blk('Y', interleave)(b_slots(1, xn[1], ks, ka) + b_slots(2, xna, va) + b_slots(2, xn[1], vs, va),
                   prep_sched(2)
                   + at(y_qk0, qk_pieces(qa, ka, lsa, True))
                   + at(y_qk1, qk_pieces(qb, ks, ls))
                   + at(y_pv, pv_pieces(lsa, va, osa, y_pvtok)))
        mark('s6_waitWo')
        for c in grp_wo:
            c.wait()
        mark('s7_Z')
        for c in grp_ffn:
            c.start()
        new_block()
        wrv = jnp.broadcast_to(wr[...].astype(f32).reshape(1, D), (8, D))
        wrf[0:8, :] = wrv
        wrf[8:16, :] = jnp.broadcast_to(jnp.sum(wrv, axis=-1, keepdims=True), (8, D))
        blk('Z', interleave)(b_slots(1, xn[0], ks, ks) + d_slots(0, osa) + d_slots(1, os_) + b_slots(2, xn[0], vs, vs),
                   at(z_wo, prep_wo_pieces(z_wod))
                   + at(z_pv, pv_pieces(ls, vs, os_))
                   + at(z_qk, qk_pieces(qs, ks, ls))
                   + at(z_e, e_pieces(0, 0, z_ed))
                   + at(z_a, a_pieces(3, xn[1], z_ad)))

        first = 2
        nloop = (NT - 2 - first) // unroll

        def body(k, c):
            i0 = first + k * unroll
            new_block()
            for u in range(unroll):
                blk('loop', step)(i0 + u, (first + u) % 2)
            return c

        xr_copy.wait()
        mark('s8_loop')
        jax.lax.fori_loop(0, nloop, body, 0)
        mark('s9_tail')
        rest = list(range(first + nloop * unroll, NT - 2))
        new_block()
        for i in rest:
            step(i, i % 2)
        def pick():
            bv = jnp.concatenate([best[0], best[2]], axis=0)
            bi = jnp.concatenate([best[1], best[3]], axis=0)
            mx = jnp.max(bv, axis=0, keepdims=True)
            cand = jnp.where(bv == mx, bi, float(S))
            idx_v = jnp.min(cand, axis=0, keepdims=True)
            return jnp.clip(jnp.min(idx_v).astype(i32), 0, S - 1), mx

        def ffn_in(idx):
            base = pl.multiple_of(jnp.clip(idx >> 4, 0, S // 16 - 1) * 16, 16)
            h16 = hs[pl.ds(base, 16), :]
            m16, rs16 = ln_stats(h16)
            hn16 = (h16 - m16) * rs16
            return base, h16 + hn16, hn16.astype(bf16)

        def ffn_act(xb, c0, n):
            g = jnp.dot(xb, pltpu.bitcast(wg[:, c0:c0 + n], bf16), preferred_element_type=f32)
            u = jnp.dot(xb, pltpu.bitcast(wu[:, c0:c0 + n], bf16), preferred_element_type=f32)
            return (g * jax.nn.sigmoid(g) * u).astype(bf16)

        def ffn_out(act, idx, base, mx, o16, y=None):
            if y is None:
                y = jnp.dot(act, pltpu.bitcast(wd[...], bf16), preferred_element_type=f32)
            gate = jax.nn.sigmoid(mx[:, 0:1])
            rows16 = jax.lax.broadcasted_iota(i32, (16, D), 0)
            fixbuf[...] = (o16 + jnp.where(rows16 == idx - base, y * gate, 0.0)).astype(bf16)

        def fix_copy(base):
            return pltpu.make_async_copy(fixbuf, out_hbm.at[pl.ds(base, 16)], sems.at[S_A])

        for c in grp_ffn:
            c.wait()
        new_block()
        L = NT - 1
        src = xn[L % 2]
        qn, kn, kp = (qq[L % 2], kk[L % 2], kk[1 - L % 2]) if qkpar else (qs, ks, ks)
        sp = {}

        def sp_in():
            sp['idx'], sp['mx'] = pick()
            sp['base'], sp['o16'], sp['xb'] = ffn_in(sp['idx'])
            sp['act'] = []

        def sp_act(c0, n):
            sp['act'].append(ffn_act(sp['xb'], c0, n))

        def sp_half(k):
            c0 = (k // 2) * 128
            r = jnp.dot(sp['xb'], pltpu.bitcast((wu if k % 2 else wg)[:, c0:c0 + 128], bf16),
                        preferred_element_type=f32)
            if k % 2:
                g = sp['g']
                sp['act'].append((g * jax.nn.sigmoid(g) * r).astype(bf16))
            else:
                sp['g'] = r

        def sp_down(n):
            r = jnp.dot(sp['act'][n], pltpu.bitcast(wd[n * 64:(n + 1) * 64, :], bf16), preferred_element_type=f32)
            sp['y'] = r if n == 0 else sp['y'] + r

        def sp_out():
            if len(t_act) == 36:
                ffn_out(None, sp['idx'], sp['base'], sp['mx'], sp['o16'], sp['y'])
            else:
                ffn_out(jnp.concatenate(sp['act'], axis=1), sp['idx'], sp['base'], sp['mx'], sp['o16'])

        FC = F // len(t_act)
        seq36 = []
        for n in range(12 + dlag):
            if n < 12:
                seq36 += [functools.partial(sp_half, 2 * n), functools.partial(sp_half, 2 * n + 1)]
            if n >= dlag:
                seq36.append(functools.partial(sp_down, n - dlag))
        act_pieces = (seq36 if len(t_act) == 36 else [functools.partial(sp_half, k) for k in range(24)] if len(t_act) == 24 else
                      [functools.partial(sp_act, c0, FC) for c0 in range(0, F, FC)])
        blk('tail', interleave)(b_slots(0, src, qn) + b_slots(1, src, kn, kp) + b_slots(2, src, va, vs)
                   + d_slots(L - 1, os_) + d_slots(L, osa),
                   at(t_e0, e_pieces(L - 2, L % 2, t_ed0))
                   + [(t_in, sp_in)]
                   + at(t_pv0, pv_pieces(ls, vs, os_))
                   + at(t_qk, qk_pieces(qn, kn, lsa))
                   + at(t_pv, pv_pieces(lsa, va, osa, t_pvtok))
                   + at(t_act, act_pieces)
                   + at(t_e, e_pieces(L - 1, (L - 1) % 2, t_ed))
                   + [(25, sp_out)]
                   + spread(e_pieces(L, L % 2), 25, 26))

        mark('sa_final')
        idx, mx = pick()
        o_copy(0, S - NLAST * T, False).wait()
        late_copies = o_copy(S - NLAST * T, NLAST * T, True)
        hit = idx == sp['idx'] if sp else idx < 0

        @pl.when(hit)
        def _():
            fix_copy(sp['base'] if sp else 0).start()
            late_copies.wait()
            fix_copy(sp['base'] if sp else 0).wait()

        @pl.when(jnp.logical_not(hit))
        def _():
            base, o16, xb = ffn_in(idx)
            ffn_out(ffn_act(xb, 0, F), idx, base, mx, o16)
            late_copies.wait()
            fix_copy(base).start()
            fix_copy(base).wait()
        mark(None)

    lhs_buf = pltpu.VMEM((T // 2, D), u32)
    q_buf = pltpu.VMEM((NJ, T + padq, 128), f32)
    kv_buf = pltpu.VMEM((NJ, T + HALO + padk, 128), f32)
    l_buf = pltpu.VMEM((NW + 1, T + padl, 128), f32)
    scratch = [
        pltpu.VMEM((S // 2, D), u32),
        pltpu.VMEM((D // 2, 3 * D), u32),
        pltpu.VMEM((D // 2, D), u32),
        pltpu.VMEM((D // 2, 3 * D), u32),
        pltpu.VMEM((D // 2, D), u32),
        pltpu.VMEM((NJ, D, 128), f32),
        pltpu.VMEM((D // 2, D), u32),
        pltpu.VMEM((D,), bf16),
        pltpu.VMEM((16, D), f32),
        pltpu.VMEM((D // 2, F), u32),
        pltpu.VMEM((D // 2, F), u32),
        pltpu.VMEM((F // 2, D), u32),
        lhs_buf, lhs_buf, lhs_buf,
        q_buf, q_buf, q_buf,
        kv_buf, kv_buf, kv_buf, kv_buf,
        l_buf, l_buf,
        lhs_buf, lhs_buf,
        pltpu.VMEM((S, D), f32),
        pltpu.VMEM((S, D), bf16),
        pltpu.VMEM((4, 8, 128), f32),
        pltpu.VMEM((8, 128), u32),
        pltpu.VMEM((20, T + padp, 128), f32),
        pltpu.SMEM((1,), i32),
        pltpu.VMEM((16, D), bf16),
        pltpu.SemaphoreType.DMA((3 + NWQ,)),
    ]
    return kernel, scratch


def build(**kw):
    nobc = kw.get('nobc', True)
    kernel, scratch = make_kernel(**kw)

    def fn(A_x, A_wqkv, A_wo, B_x, B_w_r, B_w_gate, B_w_up, B_w_down):
        x2 = A_x.reshape(S, D)
        out = pl.pallas_call(
            kernel,
            in_specs=[pl.BlockSpec(memory_space=pl.ANY)] * 7,
            out_specs=pl.BlockSpec(memory_space=pl.ANY),
            out_shape=jax.ShapeDtypeStruct((S, D), bf16),
            scratch_shapes=scratch,
            name="fused",
            compiler_params=pltpu.CompilerParams(vmem_limit_bytes=100 * 2**20, disable_bounds_checks=nobc),
        )(x2, A_wqkv, A_wo, B_w_r, B_w_gate, B_w_up, B_w_down)
        return out.reshape(1, S, D)
    return fn


_fn = build()


@jax.jit
def pallas_sequential_preLN__sliding_local_dilated__moe_arch_mod__prompt_kernel(
    A_x: jax.Array,
    A_wqkv: jax.Array,
    A_wo: jax.Array,
    B_x: jax.Array,
    B_w_r: jax.Array,
    B_w_gate: jax.Array,
    B_w_up: jax.Array,
    B_w_down: jax.Array,
):
    return _fn(A_x, A_wqkv, A_wo, B_x, B_w_r, B_w_gate, B_w_up, B_w_down)
```

```python
import functools
import math
import jax
import jax.numpy as jnp
from jax.experimental import pallas as pl
from jax.experimental.pallas import tpu as pltpu

S, D, H, DH, F = 2048, 640, 32, 20, 1536
NW, DIL = 8, 2
HALO = 16
NJ = D // 128
EPS = 1e-5
QSCALE = (DH ** -0.5) * math.log2(math.e)
f32, bf16, u32, i32 = jnp.float32, jnp.bfloat16, jnp.uint32, jnp.int32


def interleave(slots, pieces):
    pieces = sorted(pieces, key=lambda kp: kp[0])
    for k, p in pieces:
        if k < 0:
            p()
    for c, s in enumerate(slots):
        s()
        for k, p in pieces:
            if k == c:
                p()
    for k, p in pieces:
        if k >= len(slots):
            p()


def spread(pieces, lo, hi):
    n = len(pieces)
    return [(lo + (k * (hi - lo)) // n, p) for k, p in enumerate(pieces)]


def at(sched, pieces, off=0):
    k = len(pieces) // len(sched)
    sched = [c for c in sched for _ in range(k)]
    return [(c + off, p) for c, p in zip(sched, pieces, strict=True)]


def pack2(even, odd):
    p = pltpu.pack_elementwise([even, odd], packed_dtype=bf16)
    return p if p.dtype == u32 else pltpu.bitcast(p, u32)


def rsqrt(v):
    return jnp.exp2(jnp.log2(v) * -0.5)


def make_kernel(T=128, LNB=64, RB=16, QB=16, unroll=4,
                pv_sched=(2, 3, 4, 5, 6, 7, 8, 9), pv_lag=2,
                a_sched=(16, 17), a_d=2,
                e_sched=(0, 3), e_d=4,
                qk_sched=(9, 10, 11, 11, 12, 13, 13, 14), NWQ=4, only=None, ksplit=False, opaque=(), smqk=0, dlag=1, t_in=6,
                t_act=(8, 9, 10, 11, 12, 13, 14, 15, 16, 17, 18, 19, 20, 21, 22, 23, 23, 24, 24, 24, 24, 24, 24, 24), sel_pb=64, sel_d=0, sel_hi=2, perm_sched=(2, 2, 3, 3, 4), z_wo=(-1, 0, 1, 2, 3), z_wod=0, ilv_a=True, ilv_pv=True, qkpar=True, areload=False, pv_ng=1, nobc=True, padq=8, padl=8, padk=24, padp=8, t_e0=(-1, 0), t_ed0=4,
                y_qk0=(1, 2, 3, 4, 5, 5, 5, 8), y_qk1=(6, 7, 7, 8, 10, 11, 12, 12), y_pv=(10, 10, 11, 11, 12, 12, 13, 13), y_pvtok=False,
                z_pv=(2, 3, 4, 5, 6, 7, 8, 9), z_qk=(10, 11, 12, 13, 14, 15, 16, 16), z_e=(13, 16), z_ed=1, z_a=(16, 17), z_ad=2,
                t_pvtok=False, t_pv0=(3, 4, 5, 6, 7, 8, 9, 10), t_ed=2,
                t_qk=(9, 10, 11, 11, 11, 11, 12, 13), t_pv=(16, 17, 18, 19, 19, 19, 19, 19), t_e=(21, 22), scopes=False):
    NT = S // T

    def kernel(x_hbm, wqkv_hbm, wo_hbm, wr_hbm, wg_hbm, wu_hbm, wd_hbm, out_hbm,
               xs, wraw, wt, wp, woraw, wof, wop, wr, wrf, wg, wu, wd,
               xn0, xn1, xna, qs, qa, qb, ks, ka, vs, va, ls, lsa, os_, osa, hs, outs, best, zv, pk, zs, fixbuf,
               sems):
        x_u, wqkv_u, wo_u, wg_u, wu_u, wd_u = [r.bitcast(u32) for r in (x_hbm, wqkv_hbm, wo_hbm, wg_hbm, wu_hbm, wd_hbm)]
        xn = (xn0, xn1)
        qq, kk = (qs, qa), (ks, ka)
        pending = []
        hist = []

        zz = [0]

        def new_block():
            hist.clear()
            pending.clear()
            zz[0] = pl.multiple_of(zs[0], 8)

        def dyn(name, start, n):
            if name in opaque:
                return pl.ds(zz[0] + start, n)
            return pl.ds(start, n)

        def emit_token(val_u32, d=1):
            pending.append((len(hist) + d - 1, val_u32))

        def take_due(t_now):
            due = [v for (c, v) in pending if c <= t_now]
            pending[:] = [(c, v) for (c, v) in pending if c > t_now]
            if not due:
                return None
            t = due.pop()
            while due:
                t = t | due.pop()
            return t & zv[...]

        def gated(w_u32):
            t = take_due(len(hist))
            if t is None:
                return w_u32
            return jnp.concatenate([w_u32[0:8] | t, w_u32[8:]], axis=0)

        def gate_after(lag):
            if len(hist) > lag:
                return pltpu.bitcast(hist[-1 - lag], u32) & zv[...]
            return None

        def xrows(r, n):
            h = r // 2 if isinstance(r, int) else pl.multiple_of(r // 2, 8)
            return pl.ds(h, n // 2)

        def row0(i):
            return i * T if isinstance(i, int) else pl.multiple_of(i * T, T)

        S_A, S_B, S_C = 0, 1, 2
        S_Q = [3 + c for c in range(NWQ)]

        def x_copy(t0, t1, sem):
            rows = pl.ds(t0 * T // 2, (t1 - t0) * T // 2)
            return pltpu.make_async_copy(x_u.at[rows], xs.at[rows], sems.at[sem])

        def w_copy(p, sem):
            return pltpu.make_async_copy(wqkv_u.at[:, pl.ds(p * D, D)], wraw.at[:, pl.ds(p * D, D)], sems.at[sem])

        WQR = D // NWQ

        def wq_copy(c):
            rows = pl.ds(c * WQR // 2, WQR // 2)
            return pltpu.make_async_copy(wqkv_u.at[rows, pl.ds(0, D)], wraw.at[rows, pl.ds(0, D)], sems.at[S_Q[c]])

        x0_copy = x_copy(0, 1, S_A)
        x12_copy = x_copy(1, 3, S_B)
        wk_copy = w_copy(1, S_C)
        wv_copy = w_copy(2, S_A)
        grp_wo = [pltpu.make_async_copy(wr_hbm, wr, sems.at[S_Q[0]]),
                  pltpu.make_async_copy(wo_u, woraw, sems.at[S_Q[0]]),
                  x_copy(3, 4, S_Q[0])]
        xr_copy = x_copy(4, NT, S_Q[1])
        grp_ffn = [pltpu.make_async_copy(wg_u, wg, sems.at[S_B]),
                   pltpu.make_async_copy(wu_u, wu, sems.at[S_B]),
                   pltpu.make_async_copy(wd_u, wd, sems.at[S_B])]

        NLAST = 2

        def o_copy(r, n, late):
            return pltpu.make_async_copy(outs.at[pl.ds(r, n)], out_hbm.at[pl.ds(r, n)], sems.at[S_B if late else S_C])

        def prep_w_pieces(p, lo=0, hi=D, PB=128, d=0):
            def sel(r0):
                lane = jax.lax.broadcasted_iota(i32, (PB // 2, 128), 1)
                r5 = (lane // 4) % 5
                src = [wraw[r0 // 2:(r0 + PB) // 2, p * D + jj * 128: p * D + (jj + 1) * 128] for jj in range(NJ)]
                for j in range(NJ):
                    t = src[4]
                    for jj in range(4):
                        t = jnp.where(r5 == (j - 2 * jj) % 5, src[jj], t)
                    wt[r0 // 2:(r0 + PB) // 2, j * 128:(j + 1) * 128] = t
                    if d:
                        emit_token(t[PB // 2 - 8:PB // 2], d)

            def perm(j):
                lane = jax.lax.broadcasted_iota(i32, ((hi - lo) // 2, 128), 1)
                head = (lane % 32) // 2 + 16 * (lane % 2)
                idx = (20 * head + 4 * j + lane // 32) % 128
                wp[lo // 2:hi // 2, p * D + j * 128: p * D + (j + 1) * 128] = jnp.take_along_axis(
                    wt[lo // 2:hi // 2, j * 128:(j + 1) * 128], idx, axis=1)
            return ([functools.partial(sel, r0) for r0 in range(lo, hi, PB)]
                    + [functools.partial(perm, j) for j in range(NJ)])

        def prep_sched(p):
            ps = prep_w_pieces(p, 0, D, sel_pb, sel_d)
            return spread(ps[:-NJ], -1, sel_hi) + at(perm_sched, ps[-NJ:])

        def prep_wo_pieces(dl=0):
            def piece(j):
                wof[j] = pltpu.bitcast(woraw[:, j * 128:(j + 1) * 128], bf16).astype(f32)
                for d in range(DH):
                    blk = pack2(wof[j, pl.ds(d, H // 2, stride=DH), :],
                                wof[j, pl.ds(d + DH * (H // 2), H // 2, stride=DH), :])
                    wop[d * 16:(d + 1) * 16, j * 128:(j + 1) * 128] = blk
                    if dl and d % 4 == 3:
                        emit_token(blk[8:16], dl)
            return [functools.partial(piece, j) for j in range(NJ)]

        def ln_stats(x):
            m = jnp.sum(x, axis=-1, keepdims=True) * (1.0 / D)
            v = jnp.maximum(jnp.sum(x * x, axis=-1, keepdims=True) * (1.0 / D) - m * m, 0.0)
            return m, rsqrt(v + EPS)

        def a_pieces(i, dst, d=0):
            r = row0(i)

            def piece(b):
                if ilv_a:
                    xu = xs[xrows(r + b * LNB, LNB), :]
                    ys = []
                    for half in range(2):
                        x = pltpu.unpack_elementwise(xu, index=half, packed_dtype=bf16, unpacked_dtype=f32)
                        m, rs = ln_stats(x)
                        ys.append(x * rs - m * rs)
                    yu = pack2(ys[0], ys[1])
                else:
                    x = pltpu.bitcast(xs[xrows(r + b * LNB, LNB), :], bf16).astype(f32)
                    m, rs = ln_stats(x)
                    yu = pltpu.bitcast((x * rs - m * rs).astype(bf16), u32)
                dst[dyn('xn', b * LNB // 2, LNB // 2), :] = yu
                if d:
                    for r8 in range(LNB // 16):
                        emit_token(yu[r8 * 8:r8 * 8 + 8, D - 128:D], d)
            return [functools.partial(piece, b) for b in range(T // LNB)]

        def b_slots(p, src, dst, halo=None):
            def slot(j):
                lhs = pltpu.bitcast(src[...], bf16)
                c = p * D + j * 128
                w = pltpu.bitcast(gated(wp[:, c:c + 128]), bf16)
                res = jnp.dot(lhs, w, preferred_element_type=f32)
                hist.append(res[0:8])
                if p == 0:
                    dst[j, dyn('q', 0, T), :] = res
                else:
                    if halo is None:
                        dst[j, 0:HALO, :] = jnp.zeros((HALO, 128), f32)
                    else:
                        dst[j, 0:HALO, :] = halo[j, T:T + HALO, :]
                    dst[j, dyn('kv', HALO, T), :] = res
            return [functools.partial(slot, j) for j in range(NJ)]

        def ldw(ref, j, start, n):
            if not ilv_pv:
                return ref[j, start:start + n, :]
            parts = []
            for g0 in range(start, start + n, 16):
                parts += [ref[j, pl.ds(g0, 8, stride=2), :], ref[j, pl.ds(g0 + 1, 8, stride=2), :]]
            return jnp.concatenate(parts, axis=0)

        def qk_pieces(qr, kr, lr, first=False):
            def piece(rb):
                r0 = rb * QB
                sv = jnp.full((8, 128), QSCALE, f32)
                g = gate_after(0)
                if g is not None:
                    sv = pltpu.bitcast(pltpu.bitcast(sv, u32) | g, f32)
                lw = []
                q = [(ldw(qr, j, r0, QB).reshape(QB // 8, 8, 128) * sv[None]).reshape(QB, 128) for j in range(NJ)]
                for w in range(NW):
                    lo = HALO + r0 - DIL * w
                    a = None
                    for j in range(NJ):
                        t = q[j] * ldw(kr, j, lo, QB)
                        a = t if a is None else a + t
                    a = a + pltpu.roll(a, 64, 1)
                    a = a + pltpu.roll(a, 32, 1)
                    if first and r0 < DIL * w:
                        rows = jax.lax.broadcasted_iota(i32, (QB, 128), 0)
                        if ilv_pv:
                            rows = (rows // 16) * 16 + (rows % 8) * 2 + (rows % 16) // 8
                        rows = rows + r0
                        a = jnp.where(rows >= DIL * w, a, -1e9)
                    if smqk:
                        lw.append(a)
                    else:
                        lr[w, dyn('ls', r0, QB), :] = a
                if smqk:
                    m = lw[0]
                    for w in range(1, NW):
                        m = jnp.maximum(m, lw[w])
                    es = [jnp.exp2(l - m) for l in lw]
                    s = es[0]
                    for w in range(1, NW):
                        s = s + es[w]
                    inv = pl.reciprocal(s, approx=True)
                    if smqk == 1:
                        for w in range(NW):
                            lr[w, dyn('ls', r0, QB), :] = es[w] * inv
                    else:
                        for w in range(NW):
                            lr[w, dyn('ls', r0, QB), :] = es[w]
                        lr[NW, dyn('ls', r0, QB), :] = inv
            return [functools.partial(piece, rb) for rb in range(T // QB)]

        def pv_pieces(lr, vr, orf, tok=True):
            def piece(rb):
                r0 = rb * RB
                lw = [lr[w, r0:r0 + RB, :] for w in range(NW)]
                g = gate_after(pv_lag) if tok else None

                def gt(m):
                    if g is None:
                        return m
                    return pltpu.bitcast((pltpu.bitcast(m, u32).reshape(RB // 8, 8, 128) | g[None]).reshape(RB, 128), f32)
                if smqk:
                    es = [gt(l) if w < pv_ng else l for w, l in enumerate(lw)]
                    inv = None if smqk == 1 else lr[NW, r0:r0 + RB, :]
                else:
                    m = lw[0]
                    for w in range(1, NW):
                        m = jnp.maximum(m, lw[w])
                    m = gt(m)
                    es = [jnp.exp2(l - m) for l in lw]
                    s = es[0]
                    for w in range(1, NW):
                        s = s + es[w]
                    inv = pl.reciprocal(s, approx=True)
                for j in range(NJ):
                    o = None
                    for w in range(NW):
                        lo = HALO + r0 - DIL * w
                        t = es[w] * ldw(vr, j, lo, RB)
                        o = t if o is None else o + t
                    o = o if inv is None else o * inv
                    if ilv_pv:
                        ob = jnp.concatenate([pack2(o[g0:g0 + 8], o[g0 + 8:g0 + 16]) for g0 in range(0, RB, 16)], axis=0)
                    else:
                        ob = pltpu.bitcast(o.astype(bf16), u32)
                    orf[dyn('os', r0 // 2, RB // 2), j * 128:(j + 1) * 128] = ob
                    if tok:
                        emit_token(ob[0:8])
            return [functools.partial(piece, rb) for rb in range(T // RB)]

        def d_slots(i, orf):
            r = row0(i)

            def slot(j):
                lhs = pltpu.bitcast(orf[...], bf16)
                w = pltpu.bitcast(gated(wop[:, j * 128:(j + 1) * 128]), bf16)
                res = jnp.dot(lhs, w, preferred_element_type=f32)
                hist.append(res[0:8])
                hs[pl.ds(r, T), j * 128:(j + 1) * 128] = res + pltpu.bitcast(xs[xrows(r, T), j * 128:(j + 1) * 128], bf16).astype(f32)
            return [functools.partial(slot, j) for j in range(NJ)]

        def e_pieces(i, par, d=0):
            r = row0(i)

            def piece(b):
                rr = r + b * LNB
                h = hs[pl.ds(pl.multiple_of(rr + zz[0], 8) if 'hs' in opaque else rr, LNB), :]
                m, rs = ln_stats(h)
                hw = (h.reshape(LNB // 8, 8, D) * wrf[0:8, :][None]).reshape(LNB, D)
                rv_all = (jnp.sum(hw, axis=-1, keepdims=True) - m * wrf[8:9, 0:1]) * rs
                ov = h * (1.0 + rs) - m * rs
                outs[pl.ds(rr, LNB), :] = ov.astype(bf16)
                bv = best[2 * par]
                bi = best[2 * par + 1]
                rows = (jax.lax.broadcasted_iota(i32, (8, 128), 0) + rr).astype(f32)
                for rb in range(LNB // 8):
                    rv = jnp.broadcast_to(rv_all[rb * 8:(rb + 1) * 8, :], (8, 128))
                    upd = rv > bv
                    bv = jnp.where(upd, rv, bv)
                    bi = jnp.where(upd, rows + float(rb * 8), bi)
                if d:
                    for r8 in range(LNB // 8):
                        emit_token(pltpu.bitcast(ov[r8 * 8:r8 * 8 + 8, D - 128:D], u32), d)
                    emit_token(pltpu.bitcast(bv, u32), d)
                best[2 * par] = bv
                best[2 * par + 1] = bi
                late = isinstance(i, int) and i >= NT - NLAST
                if isinstance(i, int) and i == NT - 1:
                    o_copy(rr, LNB, late).start()
                elif b == T // LNB - 1:
                    o_copy(r, T, late).start()
            return [functools.partial(piece, b) for b in range(T // LNB)]

        K4 = 512

        def g_dot(src, wref, c0, n, slot0, add_x=None, tok=True):
            wu = wref[K4 // 2:, c0 * 128:(c0 + n) * 128]
            if tok:
                t = take_due(len(hist))
                if t is not None:
                    top = jnp.concatenate([wu[0:8, 0:128] | t, wu[0:8, 128:]], axis=1) if n > 1 else wu[0:8] | t
                    wu = jnp.concatenate([top, wu[8:]], axis=0)
            lhs = pltpu.bitcast(src[:, K4:], bf16)
            res = jnp.dot(lhs, pltpu.bitcast(wu, bf16), preferred_element_type=f32)
            for u in range(n):
                r = res[:, u * 128:(u + 1) * 128]
                if add_x is not None:
                    r = r + pltpu.bitcast(xs[xrows(add_x, T), (c0 + u) * 128:(c0 + u + 1) * 128], bf16).astype(f32)
                pk[slot0 + u, dyn('pk', 0, T), :] = r
            return res[0:8, 0:128]

        def gb_slot(src, c0):
            def slot():
                hist.append(g_dot(src, wp, c0, 4, c0))
            return slot

        def gd_slots(i, src, orf):
            r = row0(i)

            def s0():
                hist.append(g_dot(orf, wop, 0, 4, 15, r))

            def s1():
                hist.append(g_dot(orf, wop, 4, 1, 19, r))
                g_dot(src, wp, 12, 3, 12, tok=False)
            return [s0, s1]

        def b4_slots(p, src, dst, halo):
            def slot(j):
                c = p * D + j * 128
                w = pltpu.bitcast(gated(wp[0:K4 // 2, c:c + 128]), bf16)
                lhs = pltpu.bitcast(src[:, 0:K4], bf16)
                res = jnp.dot(lhs, w, preferred_element_type=f32)
                hist.append(res[0:8])
                res = res + pk[p * NJ + j, 0:T, :]
                if p == 0:
                    dst[j, dyn('q', 0, T), :] = res
                else:
                    dst[j, 0:HALO, :] = halo[j, T:T + HALO, :]
                    dst[j, dyn('kv', HALO, T), :] = res
            return [functools.partial(slot, j) for j in range(NJ)]

        def d4_slots(i, orf):
            r = row0(i)

            def slot(j):
                w = pltpu.bitcast(gated(wop[0:K4 // 2, j * 128:(j + 1) * 128]), bf16)
                lhs = pltpu.bitcast(orf[:, 0:K4], bf16)
                res = jnp.dot(lhs, w, preferred_element_type=f32)
                hist.append(res[0:8])
                hs[pl.ds(r, T), j * 128:(j + 1) * 128] = res + pk[15 + j, 0:T, :]
            return [functools.partial(slot, j) for j in range(NJ)]

        def step(i, par, has_a=True):
            pieces = []
            src = xn[1 - par]
            qn, kn, kp = (qq[1 - par], kk[1 - par], kk[par]) if qkpar else (qs, ks, ks)
            if ksplit:
                slots = ([gb_slot(src, 0), gb_slot(src, 4), gb_slot(src, 8)]
                         + b4_slots(0, src, qn, None) + b4_slots(1, src, kn, kp)
                         + gd_slots(i, src, os_) + d4_slots(i, os_) + b4_slots(2, src, vs, vs))
            else:
                slots = b_slots(0, src, qn) + b_slots(1, src, kn, kp) + d_slots(i, os_) + b_slots(2, src, vs, vs)
            pieces += at(e_sched, e_pieces(i - 1, par, e_d))
            pieces += at(pv_sched, pv_pieces(ls, vs, os_))
            pieces += at(qk_sched, qk_pieces(qn, kn, ls))
            if has_a:
                pieces += at(a_sched, a_pieces(i + 2, xn[par], a_d))
            interleave(slots, pieces)

        def blk(name, f):
            return f if only is None or name in only else (lambda *a, **k: None)

        cur = [None]

        def mark(name):
            if not scopes:
                return
            if cur[0] is not None:
                cur[0].__exit__(None, None, None)
                cur[0] = None
            if name:
                cur[0] = jax.named_scope(name)
                cur[0].__enter__()

        mark("s0_start")
        x0_copy.start()
        for c in range(NWQ):
            wq_copy(c).start()
        x12_copy.start()
        wk_copy.start()
        zv[...] = jnp.zeros((8, 128), u32)
        zs[0] = 0
        for par in range(2):
            best[2 * par] = jnp.full((8, 128), -jnp.inf, f32)
            best[2 * par + 1] = jnp.zeros((8, 128), f32)
        x0_copy.wait()
        for p in a_pieces(0, xna):
            p()
        for c in range(NWQ):
            wq_copy(c).wait()
            for p in prep_w_pieces(0, c * WQR, (c + 1) * WQR, WQR // 2 if WQR % 32 == 0 else WQR):
                p()
        x12_copy.wait()
        mark('s1_X')
        wv_copy.start()
        new_block()
        blk('X', interleave)(b_slots(0, xna, qa) + b_slots(0, xn[1], qb),
                   spread(a_pieces(1, xn[1]), 0, 2) + spread(a_pieces(2, xn[0], 2), 5, 8))
        mark('s2_waitWk')
        wk_copy.wait()
        mark('s3_X2')
        for c in grp_wo:
            c.start()
        new_block()
        blk('X2', interleave)(b_slots(0, xn[0], qs) + b_slots(1, xna, ka), prep_sched(1))
        mark('s4_waitWv')
        wv_copy.wait()
        mark('s5_Y')
        xr_copy.start()
        new_block()
        blk('Y', interleave)(b_slots(1, xn[1], ks, ka) + b_slots(2, xna, va) + b_slots(2, xn[1], vs, va),
                   prep_sched(2)
                   + at(y_qk0, qk_pieces(qa, ka, lsa, True))
                   + at(y_qk1, qk_pieces(qb, ks, ls))
                   + at(y_pv, pv_pieces(lsa, va, osa, y_pvtok)))
        mark('s6_waitWo')
        for c in grp_wo:
            c.wait()
        mark('s7_Z')
        for c in grp_ffn:
            c.start()
        new_block()
        wrv = jnp.broadcast_to(wr[...].astype(f32).reshape(1, D), (8, D))
        wrf[0:8, :] = wrv
        wrf[8:16, :] = jnp.broadcast_to(jnp.sum(wrv, axis=-1, keepdims=True), (8, D))
        blk('Z', interleave)(b_slots(1, xn[0], ks, ks) + d_slots(0, osa) + d_slots(1, os_) + b_slots(2, xn[0], vs, vs),
                   at(z_wo, prep_wo_pieces(z_wod))
                   + at(z_pv, pv_pieces(ls, vs, os_))
                   + at(z_qk, qk_pieces(qs, ks, ls))
                   + at(z_e, e_pieces(0, 0, z_ed))
                   + at(z_a, a_pieces(3, xn[1], z_ad)))

        first = 2
        nloop = (NT - 2 - first) // unroll

        def body(k, c):
            i0 = first + k * unroll
            new_block()
            for u in range(unroll):
                blk('loop', step)(i0 + u, (first + u) % 2)
            return c

        xr_copy.wait()
        mark('s8_loop')
        jax.lax.fori_loop(0, nloop, body, 0)
        mark('s9_tail')
        rest = list(range(first + nloop * unroll, NT - 2))
        new_block()
        for i in rest:
            step(i, i % 2)
        def pick():
            bv = jnp.concatenate([best[0], best[2]], axis=0)
            bi = jnp.concatenate([best[1], best[3]], axis=0)
            mx = jnp.max(bv, axis=0, keepdims=True)
            cand = jnp.where(bv == mx, bi, float(S))
            idx_v = jnp.min(cand, axis=0, keepdims=True)
            return jnp.clip(jnp.min(idx_v).astype(i32), 0, S - 1), mx

        def ffn_in(idx):
            base = pl.multiple_of(jnp.clip(idx >> 4, 0, S // 16 - 1) * 16, 16)
            h16 = hs[pl.ds(base, 16), :]
            m16, rs16 = ln_stats(h16)
            hn16 = (h16 - m16) * rs16
            return base, h16 + hn16, hn16.astype(bf16)

        def ffn_act(xb, c0, n):
            g = jnp.dot(xb, pltpu.bitcast(wg[:, c0:c0 + n], bf16), preferred_element_type=f32)
            u = jnp.dot(xb, pltpu.bitcast(wu[:, c0:c0 + n], bf16), preferred_element_type=f32)
            return (g * jax.nn.sigmoid(g) * u).astype(bf16)

        def ffn_out(act, idx, base, mx, o16, y=None):
            if y is None:
                y = jnp.dot(act, pltpu.bitcast(wd[...], bf16), preferred_element_type=f32)
            gate = jax.nn.sigmoid(mx[:, 0:1])
            rows16 = jax.lax.broadcasted_iota(i32, (16, D), 0)
            fixbuf[...] = (o16 + jnp.where(rows16 == idx - base, y * gate, 0.0)).astype(bf16)

        def fix_copy(base):
            return pltpu.make_async_copy(fixbuf, out_hbm.at[pl.ds(base, 16)], sems.at[S_A])

        for c in grp_ffn:
            c.wait()
        new_block()
        L = NT - 1
        src = xn[L % 2]
        qn, kn, kp = (qq[L % 2], kk[L % 2], kk[1 - L % 2]) if qkpar else (qs, ks, ks)
        sp = {}

        def sp_in():
            sp['idx'], sp['mx'] = pick()
            sp['base'], sp['o16'], sp['xb'] = ffn_in(sp['idx'])
            sp['act'] = []

        def sp_act(c0, n):
            sp['act'].append(ffn_act(sp['xb'], c0, n))

        def sp_half(k):
            c0 = (k // 2) * 128
            r = jnp.dot(sp['xb'], pltpu.bitcast((wu if k % 2 else wg)[:, c0:c0 + 128], bf16),
                        preferred_element_type=f32)
            if k % 2:
                g = sp['g']
                sp['act'].append((g * jax.nn.sigmoid(g) * r).astype(bf16))
            else:
                sp['g'] = r

        def sp_down(n):
            r = jnp.dot(sp['act'][n], pltpu.bitcast(wd[n * 64:(n + 1) * 64, :], bf16), preferred_element_type=f32)
            sp['y'] = r if n == 0 else sp['y'] + r

        def sp_out():
            if len(t_act) == 36:
                ffn_out(None, sp['idx'], sp['base'], sp['mx'], sp['o16'], sp['y'])
            else:
                ffn_out(jnp.concatenate(sp['act'], axis=1), sp['idx'], sp['base'], sp['mx'], sp['o16'])

        FC = F // len(t_act)
        seq36 = []
        for n in range(12 + dlag):
            if n < 12:
                seq36 += [functools.partial(sp_half, 2 * n), functools.partial(sp_half, 2 * n + 1)]
            if n >= dlag:
                seq36.append(functools.partial(sp_down, n - dlag))
        act_pieces = (seq36 if len(t_act) == 36 else [functools.partial(sp_half, k) for k in range(24)] if len(t_act) == 24 else
                      [functools.partial(sp_act, c0, FC) for c0 in range(0, F, FC)])
        blk('tail', interleave)(b_slots(0, src, qn) + b_slots(1, src, kn, kp) + b_slots(2, src, va, vs)
                   + d_slots(L - 1, os_) + d_slots(L, osa),
                   at(t_e0, e_pieces(L - 2, L % 2, t_ed0))
                   + [(t_in, sp_in)]
                   + at(t_pv0, pv_pieces(ls, vs, os_))
                   + at(t_qk, qk_pieces(qn, kn, lsa))
                   + at(t_pv, pv_pieces(lsa, va, osa, t_pvtok))
                   + at(t_act, act_pieces)
                   + at(t_e, e_pieces(L - 1, (L - 1) % 2, t_ed))
                   + [(25, sp_out)]
                   + spread(e_pieces(L, L % 2), 25, 26))

        mark('sa_final')
        idx, mx = pick()
        o_copy(0, S - NLAST * T, False).wait()
        late_copies = o_copy(S - NLAST * T, NLAST * T, True)
        hit = idx == sp['idx'] if sp else idx < 0

        @pl.when(hit)
        def _():
            fix_copy(sp['base'] if sp else 0).start()
            late_copies.wait()
            fix_copy(sp['base'] if sp else 0).wait()

        @pl.when(jnp.logical_not(hit))
        def _():
            base, o16, xb = ffn_in(idx)
            ffn_out(ffn_act(xb, 0, F), idx, base, mx, o16)
            late_copies.wait()
            fix_copy(base).start()
            fix_copy(base).wait()
        mark(None)

    lhs_buf = pltpu.VMEM((T // 2, D), u32)
    q_buf = pltpu.VMEM((NJ, T + padq, 128), f32)
    kv_buf = pltpu.VMEM((NJ, T + HALO + padk, 128), f32)
    l_buf = pltpu.VMEM((NW + 1, T + padl, 128), f32)
    scratch = [
        pltpu.VMEM((S // 2, D), u32),
        pltpu.VMEM((D // 2, 3 * D), u32),
        pltpu.VMEM((D // 2, D), u32),
        pltpu.VMEM((D // 2, 3 * D), u32),
        pltpu.VMEM((D // 2, D), u32),
        pltpu.VMEM((NJ, D, 128), f32),
        pltpu.VMEM((D // 2, D), u32),
        pltpu.VMEM((D,), bf16),
        pltpu.VMEM((16, D), f32),
        pltpu.VMEM((D // 2, F), u32),
        pltpu.VMEM((D // 2, F), u32),
        pltpu.VMEM((F // 2, D), u32),
        lhs_buf, lhs_buf, lhs_buf,
        q_buf, q_buf, q_buf,
        kv_buf, kv_buf, kv_buf, kv_buf,
        l_buf, l_buf,
        lhs_buf, lhs_buf,
        pltpu.VMEM((S, D), f32),
        pltpu.VMEM((S, D), bf16),
        pltpu.VMEM((4, 8, 128), f32),
        pltpu.VMEM((8, 128), u32),
        pltpu.VMEM((20, T + padp, 128), f32),
        pltpu.SMEM((1,), i32),
        pltpu.VMEM((16, D), bf16),
        pltpu.SemaphoreType.DMA((3 + NWQ,)),
    ]
    return kernel, scratch


def build(**kw):
    nobc = kw.get('nobc', True)
    kernel, scratch = make_kernel(**kw)

    def fn(A_x, A_wqkv, A_wo, B_x, B_w_r, B_w_gate, B_w_up, B_w_down):
        x2 = A_x.reshape(S, D)
        out = pl.pallas_call(
            kernel,
            in_specs=[pl.BlockSpec(memory_space=pl.ANY)] * 7,
            out_specs=pl.BlockSpec(memory_space=pl.ANY),
            out_shape=jax.ShapeDtypeStruct((S, D), bf16),
            scratch_shapes=scratch,
            name="fused",
            compiler_params=pltpu.CompilerParams(vmem_limit_bytes=100 * 2**20, disable_bounds_checks=nobc),
        )(x2, A_wqkv, A_wo, B_w_r, B_w_gate, B_w_up, B_w_down)
        return out.reshape(1, S, D)
    return fn


_fn = build()


@jax.jit
def pallas_sequential_preLN__sliding_local_dilated__moe_arch_mod__prompt_kernel(
    A_x: jax.Array,
    A_wqkv: jax.Array,
    A_wo: jax.Array,
    B_x: jax.Array,
    B_w_r: jax.Array,
    B_w_gate: jax.Array,
    B_w_up: jax.Array,
    B_w_down: jax.Array,
):
    return _fn(A_x, A_wqkv, A_wo, B_x, B_w_r, B_w_gate, B_w_up, B_w_down)
```

```python
import functools
import math
import jax
import jax.numpy as jnp
from jax.experimental import pallas as pl
from jax.experimental.pallas import tpu as pltpu

S, D, H, DH, F = 2048, 640, 32, 20, 1536
NW, DIL = 8, 2
HALO = 16
NJ = D // 128
EPS = 1e-5
QSCALE = (DH ** -0.5) * math.log2(math.e)
f32, bf16, u32, i32 = jnp.float32, jnp.bfloat16, jnp.uint32, jnp.int32


def interleave(slots, pieces):
    pieces = sorted(pieces, key=lambda kp: kp[0])
    for k, p in pieces:
        if k < 0:
            p()
    for c, s in enumerate(slots):
        s()
        for k, p in pieces:
            if k == c:
                p()
    for k, p in pieces:
        if k >= len(slots):
            p()


def spread(pieces, lo, hi):
    n = len(pieces)
    return [(lo + (k * (hi - lo)) // n, p) for k, p in enumerate(pieces)]


def at(sched, pieces):
    k = len(pieces) // len(sched)
    sched = [c for c in sched for _ in range(k)]
    return list(zip(sched, pieces, strict=True))


def pack2(even, odd):
    p = pltpu.pack_elementwise([even, odd], packed_dtype=bf16)
    return p if p.dtype == u32 else pltpu.bitcast(p, u32)


def as_bf16(x_u32):
    return pltpu.bitcast(x_u32, bf16)


def or_bits(x, g):
    return pltpu.bitcast(pltpu.bitcast(x, u32) | g, f32)


def rsqrt(v):
    return jnp.exp2(jnp.log2(v) * -0.5)


def make_kernel(T=128, LNB=64, unroll=4, NWQ=4, only=None, scopes=False,
                pv_sched=(2, 3, 4, 5, 6, 7, 8, 9), pv_lag=2, a_sched=(16, 17), a_d=2,
                e_sched=(0, 3), e_d=4, qk_sched=(9, 10, 11, 11, 12, 13, 13, 14),
                qkpar=True,
                sel_pb=64, perm_sched=(2, 2, 3, 3, 4),
                y_qk0=(1, 2, 3, 4, 5, 5, 5, 8), y_qk1=(6, 7, 7, 8, 10, 11, 12, 12),
                y_pv=(10, 10, 11, 11, 12, 12, 13, 13), y_pvtok=False,
                z_wo=(-1, 0, 1, 2, 3), z_pv=(2, 3, 4, 5, 6, 7, 8, 9), z_qk=(10, 11, 12, 13, 14, 15, 16, 16),
                z_e=(13, 16), z_ed=1, z_a=(16, 17), z_ad=2,
                t_e0=(-1, 0), t_ed0=4, t_pv0=(3, 4, 5, 6, 7, 8, 9, 10), t_qk=(9, 10, 11, 11, 11, 11, 12, 13),
                t_pv=(16, 17, 18, 19, 19, 19, 19, 19), t_pvtok=False, t_e=(21, 22), t_ed=2, t_in=6,
                t_act=(8, 9, 10, 11, 12, 13, 14, 15, 16, 17, 18, 19, 20, 21, 22, 23, 23, 24, 24, 24, 24, 24, 24, 24),
                padq=8, padl=8, padk=24, ):
    NT = S // T
    NG = T // 16

    def kernel(x_hbm, wqkv_hbm, wo_hbm, wr_hbm, wg_hbm, wu_hbm, wd_hbm, out_hbm,
               xs, wraw, wt, wp, woraw, wof, wop, wr, filler, wrf, wg, wu, wd,
               xn0, xn1, xna, qs, qa, qb, zv_, ks, ka, best, vs, va, ls, lsa, os_, osa, hs, outs, fixbuf,
               sems):
        x_u, wqkv_u, wo_u, wg_u, wu_u, wd_u = [r.bitcast(u32) for r in
                                               (x_hbm, wqkv_hbm, wo_hbm, wg_hbm, wu_hbm, wd_hbm)]
        xn, qq, kk = (xn0, xn1), (qs, qa), (ks, ka)

        zv = zv_.at[pl.ds(0, 8)]
        pending = []
        hist = []

        def new_block():
            hist.clear()
            pending.clear()

        def emit_token(val_u32, d=1):
            pending.append((len(hist) + d - 1, val_u32))

        def gated(w_u32):
            due = [v for (c, v) in pending if c <= len(hist)]
            pending[:] = [(c, v) for (c, v) in pending if c > len(hist)]
            if not due:
                return w_u32
            t = due.pop()
            while due:
                t = t | due.pop()
            return jnp.concatenate([w_u32[0:8] | (t & zv[...]), w_u32[8:]], axis=0)

        def zero_of(v):
            return pltpu.bitcast(v, u32) & zv[...]

        def gate_after(lag):
            return zero_of(hist[-1 - lag]) if len(hist) > lag else None

        def row0(i):
            return i * T if isinstance(i, int) else pl.multiple_of(i * T, T)

        def xrows(r, n):
            return pl.ds(r // 2 if isinstance(r, int) else pl.multiple_of(r // 2, 8), n // 2)

        S_A, S_B, S_C = 0, 1, 2
        S_Q = [3 + c for c in range(NWQ)]
        WQR = D // NWQ
        NLAST = 2

        def x_copy(t0, t1, sem):
            rows = pl.ds(t0 * T // 2, (t1 - t0) * T // 2)
            return pltpu.make_async_copy(x_u.at[rows], xs.at[rows], sems.at[sem])

        def w_copy(p, sem):
            return pltpu.make_async_copy(wqkv_u.at[:, pl.ds(p * D, D)], wraw.at[:, pl.ds(p * D, D)], sems.at[sem])

        def wq_copy(c):
            rows = pl.ds(c * WQR // 2, WQR // 2)
            return pltpu.make_async_copy(wqkv_u.at[rows, pl.ds(0, D)], wraw.at[rows, pl.ds(0, D)], sems.at[S_Q[c]])

        x0_copy = x_copy(0, 1, S_A)
        x12_copy = x_copy(1, 3, S_B)
        wk_copy = w_copy(1, S_C)
        wv_copy = w_copy(2, S_A)
        grp_wo = [pltpu.make_async_copy(wr_hbm, wr, sems.at[S_Q[0]]),
                  pltpu.make_async_copy(wo_u, woraw, sems.at[S_Q[0]]),
                  x_copy(3, 4, S_Q[0])]
        xr_copy = x_copy(4, NT, S_Q[1])
        grp_ffn = [pltpu.make_async_copy(wg_u, wg, sems.at[S_B]),
                   pltpu.make_async_copy(wu_u, wu, sems.at[S_B]),
                   pltpu.make_async_copy(wd_u, wd, sems.at[S_B])]

        def o_copy(r, n, late):
            return pltpu.make_async_copy(outs.at[pl.ds(r, n)], out_hbm.at[pl.ds(r, n)],
                                         sems.at[S_B if late else S_C])

        def fix_copy(base):
            return pltpu.make_async_copy(fixbuf.at[pl.ds(0, 16)], out_hbm.at[pl.ds(base, 16)], sems.at[S_A])

        def prep_w_pieces(p, lo=0, hi=D, PB=128):
            def sel(r0):
                r5 = (jax.lax.broadcasted_iota(i32, (PB // 2, 128), 1) // 4) % 5
                src = [wraw[r0 // 2:(r0 + PB) // 2, p * D + jj * 128: p * D + (jj + 1) * 128] for jj in range(NJ)]
                for j in range(NJ):
                    t = src[4]
                    for jj in range(4):
                        t = jnp.where(r5 == (j - 2 * jj) % 5, src[jj], t)
                    wt[r0 // 2:(r0 + PB) // 2, j * 128:(j + 1) * 128] = t

            def perm(j):
                lane = jax.lax.broadcasted_iota(i32, ((hi - lo) // 2, 128), 1)
                head = (lane % 32) // 2 + 16 * (lane % 2)
                idx = (20 * head + 4 * j + lane // 32) % 128
                wp[lo // 2:hi // 2, p * D + j * 128: p * D + (j + 1) * 128] = jnp.take_along_axis(
                    wt[lo // 2:hi // 2, j * 128:(j + 1) * 128], idx, axis=1)
            return ([functools.partial(sel, r0) for r0 in range(lo, hi, PB)]
                    + [functools.partial(perm, j) for j in range(NJ)])

        def prep_sched(p):
            ps = prep_w_pieces(p, 0, D, sel_pb)
            return spread(ps[:-NJ], -1, 2) + at(perm_sched, ps[-NJ:])

        def prep_wo_pieces():
            def piece(j):
                wof[j] = as_bf16(woraw[:, j * 128:(j + 1) * 128]).astype(f32)
                for d in range(DH):
                    wop[d * 16:(d + 1) * 16, j * 128:(j + 1) * 128] = pack2(
                        wof[j, pl.ds(d, H // 2, stride=DH), :],
                        wof[j, pl.ds(d + DH * (H // 2), H // 2, stride=DH), :])
            return [functools.partial(piece, j) for j in range(NJ)]

        def ln_stats(x):
            m = jnp.sum(x, axis=-1, keepdims=True) * (1.0 / D)
            v = jnp.maximum(jnp.sum(x * x, axis=-1, keepdims=True) * (1.0 / D) - m * m, 0.0)
            return m, rsqrt(v + EPS)

        def a_pieces(i, dst, d=0):
            r = row0(i)

            def piece(b):
                xu = xs[xrows(r + b * LNB, LNB), :]
                ys = []
                for half in range(2):
                    x = pltpu.unpack_elementwise(xu, index=half, packed_dtype=bf16, unpacked_dtype=f32)
                    m, rs = ln_stats(x)
                    ys.append(x * rs - m * rs)
                yu = pack2(ys[0], ys[1])
                dst[b * LNB // 2:(b + 1) * LNB // 2, :] = yu
                if d:
                    for r8 in range(LNB // 16):
                        emit_token(yu[r8 * 8:r8 * 8 + 8, D - 128:D], d)
            return [functools.partial(piece, b) for b in range(T // LNB)]

        def b_slots(p, src, dst, halo=None):
            def slot(j):
                c = p * D + j * 128
                res = jnp.dot(as_bf16(src[...]), as_bf16(gated(wp[:, c:c + 128])), preferred_element_type=f32)
                hist.append(res[0:8])
                if p == 0:
                    dst[j, 0:T, :] = res
                else:
                    dst[j, 0:HALO, :] = jnp.zeros((HALO, 128), f32) if halo is None else halo[j, T:T + HALO, :]
                    dst[j, HALO:HALO + T, :] = res
            return [functools.partial(slot, j) for j in range(NJ)]

        def ld16(ref, j, start):
            return jnp.concatenate([ref[j, pl.ds(start, 8, stride=2), :],
                                    ref[j, pl.ds(start + 1, 8, stride=2), :]], axis=0)

        def times8(x, v8):
            return (x.reshape(2, 8, 128) * v8[None]).reshape(16, 128)

        def qk_pieces(qr, kr, lr, first=False):
            def piece(g16):
                r0 = g16 * 16
                sv = jnp.full((8, 128), QSCALE, f32)
                gate = gate_after(0)
                if gate is not None:
                    sv = or_bits(sv, gate)
                q = [times8(ld16(qr, j, r0), sv) for j in range(NJ)]
                for w in range(NW):
                    a = None
                    for j in range(NJ):
                        t = q[j] * ld16(kr, j, HALO + r0 - DIL * w)
                        a = t if a is None else a + t
                    a = a + pltpu.roll(a, 64, 1)
                    a = a + pltpu.roll(a, 32, 1)
                    if first and r0 < DIL * w:
                        rows = jax.lax.broadcasted_iota(i32, (16, 128), 0)
                        rows = (rows % 8) * 2 + rows // 8 + r0
                        a = jnp.where(rows >= DIL * w, a, -1e9)
                    lr[w, r0:r0 + 16, :] = a
            return [functools.partial(piece, g) for g in range(NG)]

        def pv_pieces(lr, vr, orf, tok=True):
            def piece(g16):
                r0 = g16 * 16
                lw = [lr[w, r0:r0 + 16, :] for w in range(NW)]
                gate = gate_after(pv_lag) if tok else None
                m = lw[0]
                for w in range(1, NW):
                    m = jnp.maximum(m, lw[w])
                if gate is not None:
                    m = pltpu.bitcast((pltpu.bitcast(m, u32).reshape(2, 8, 128) | gate[None]).reshape(16, 128), f32)
                es = [jnp.exp2(l - m) for l in lw]
                s = es[0]
                for w in range(1, NW):
                    s = s + es[w]
                inv = pl.reciprocal(s, approx=True)
                for j in range(NJ):
                    o = None
                    for w in range(NW):
                        t = es[w] * ld16(vr, j, HALO + r0 - DIL * w)
                        o = t if o is None else o + t
                    o = o * inv
                    ob = pack2(o[0:8], o[8:16])
                    orf[r0 // 2:r0 // 2 + 8, j * 128:(j + 1) * 128] = ob
                    if tok:
                        emit_token(ob)
            return [functools.partial(piece, g) for g in range(NG)]

        def d_slots(i, orf):
            r = row0(i)

            def slot(j):
                cols = slice(j * 128, (j + 1) * 128)
                res = jnp.dot(as_bf16(orf[...]), as_bf16(gated(wop[:, cols])), preferred_element_type=f32)
                hist.append(res[0:8])
                hs[pl.ds(r, T), cols] = res + as_bf16(xs[xrows(r, T), cols]).astype(f32)
            return [functools.partial(slot, j) for j in range(NJ)]

        def e_pieces(i, par, d=0):
            r = row0(i)

            def piece(b):
                rr = r + b * LNB
                h = hs[pl.ds(rr, LNB), :]
                m, rs = ln_stats(h)
                hw = (h.reshape(LNB // 8, 8, D) * wrf[0:8, :][None]).reshape(LNB, D)
                rv_all = (jnp.sum(hw, axis=-1, keepdims=True) - m * wrf[8:9, 0:1]) * rs
                ov = h * (1.0 + rs) - m * rs
                outs[pl.ds(rr, LNB), :] = ov.astype(bf16)
                bv = best[2 * par]
                bi = best[2 * par + 1]
                rows = (jax.lax.broadcasted_iota(i32, (8, 128), 0) + rr).astype(f32)
                for rb in range(LNB // 8):
                    rv = jnp.broadcast_to(rv_all[rb * 8:(rb + 1) * 8, :], (8, 128))
                    upd = rv > bv
                    bv = jnp.where(upd, rv, bv)
                    bi = jnp.where(upd, rows + float(rb * 8), bi)
                if d:
                    for r8 in range(LNB // 8):
                        emit_token(pltpu.bitcast(ov[r8 * 8:r8 * 8 + 8, D - 128:D], u32), d)
                    emit_token(pltpu.bitcast(bv, u32), d)
                best[2 * par] = bv
                best[2 * par + 1] = bi
                late = isinstance(i, int) and i >= NT - NLAST
                if isinstance(i, int) and i == NT - 1:
                    o_copy(rr, LNB, late).start()
                elif b == T // LNB - 1:
                    o_copy(r, T, late).start()
            return [functools.partial(piece, b) for b in range(T // LNB)]

        def step(i, par):
            src = xn[1 - par]
            qn, kn, kp = (qq[1 - par], kk[1 - par], kk[par]) if qkpar else (qs, ks, ks)
            interleave(b_slots(0, src, qn) + b_slots(1, src, kn, kp) + d_slots(i, os_) + b_slots(2, src, vs, vs),
                       at(e_sched, e_pieces(i - 1, par, e_d))
                       + at(pv_sched, pv_pieces(ls, vs, os_))
                       + at(qk_sched, qk_pieces(qn, kn, ls))
                       + at(a_sched, a_pieces(i + 2, xn[par], a_d)))

        def pick():
            bv = jnp.concatenate([best[0], best[2]], axis=0)
            bi = jnp.concatenate([best[1], best[3]], axis=0)
            mx = jnp.max(bv, axis=0, keepdims=True)
            cand = jnp.where(bv == mx, bi, float(S))
            idx_v = jnp.min(cand, axis=0, keepdims=True)
            return jnp.clip(jnp.min(idx_v).astype(i32), 0, S - 1), mx

        def ffn_in(idx):
            base = pl.multiple_of(jnp.clip(idx >> 4, 0, S // 16 - 1) * 16, 16)
            h16 = hs[pl.ds(base, 16), :]
            m16, rs16 = ln_stats(h16)
            hn16 = (h16 - m16) * rs16
            return base, h16 + hn16, hn16.astype(bf16)

        def swiglu(g, u):
            return (g * jax.nn.sigmoid(g) * u).astype(bf16)

        def ffn_out(act, idx, base, mx, o16):
            y = jnp.dot(act, as_bf16(wd[...]), preferred_element_type=f32)
            gate = jax.nn.sigmoid(mx[:, 0:1])
            rows16 = jax.lax.broadcasted_iota(i32, (16, D), 0)
            fixbuf[0:16, :] = (o16 + jnp.where(rows16 == idx - base, y * gate, 0.0)).astype(bf16)

        def blk(name, f):
            return f if only is None or name in only else (lambda *a, **k: None)

        cur = [None]

        def mark(name):
            if not scopes:
                return
            if cur[0] is not None:
                cur[0].__exit__(None, None, None)
                cur[0] = None
            if name:
                cur[0] = jax.named_scope(name)
                cur[0].__enter__()

        mark("s0_start")
        x0_copy.start()
        for c in range(NWQ):
            wq_copy(c).start()
        x12_copy.start()
        wk_copy.start()
        zv[...] = jnp.zeros((8, 128), u32)
        filler[pl.ds(0, 1280)] = jnp.zeros((1280,), bf16)
        for par in range(2):
            best[2 * par] = jnp.full((8, 128), -jnp.inf, f32)
            best[2 * par + 1] = jnp.zeros((8, 128), f32)
        x0_copy.wait()
        for p in a_pieces(0, xna):
            p()
        for c in range(NWQ):
            wq_copy(c).wait()
            for p in prep_w_pieces(0, c * WQR, (c + 1) * WQR, WQR // 2 if WQR % 32 == 0 else WQR):
                p()
        wv_copy.start()
        x12_copy.wait()
        mark('s1_X')
        new_block()
        blk('X', interleave)(b_slots(0, xna, qa) + b_slots(0, xn[1], qb),
                             spread(a_pieces(1, xn[1]), 0, 2) + spread(a_pieces(2, xn[0], 2), 5, 8))
        for c in grp_wo:
            c.start()
        mark('s2_waitWk')
        wk_copy.wait()
        mark('s3_X2')
        new_block()
        blk('X2', interleave)(b_slots(0, xn[0], qs) + b_slots(1, xna, ka), prep_sched(1))
        xr_copy.start()
        mark('s4_waitWv')
        wv_copy.wait()
        mark('s5_Y')
        new_block()
        blk('Y', interleave)(b_slots(1, xn[1], ks, ka) + b_slots(2, xna, va) + b_slots(2, xn[1], vs, va),
                             prep_sched(2)
                             + at(y_qk0, qk_pieces(qa, ka, lsa, True))
                             + at(y_qk1, qk_pieces(qb, ks, ls))
                             + at(y_pv, pv_pieces(lsa, va, osa, y_pvtok)))
        for c in grp_ffn:
            c.start()
        mark('s6_waitWo')
        for c in grp_wo:
            c.wait()
        mark('s7_Z')
        new_block()
        wrv = jnp.broadcast_to((wr[...].astype(f32) + filler[pl.ds(0, D)].astype(f32)).reshape(1, D), (8, D))
        wrf[0:8, :] = wrv
        wrf[8:16, :] = jnp.broadcast_to(jnp.sum(wrv, axis=-1, keepdims=True), (8, D))
        blk('Z', interleave)(b_slots(1, xn[0], ks, ks) + d_slots(0, osa) + d_slots(1, os_)
                             + b_slots(2, xn[0], vs, vs),
                             at(z_wo, prep_wo_pieces())
                             + at(z_pv, pv_pieces(ls, vs, os_))
                             + at(z_qk, qk_pieces(qs, ks, ls))
                             + at(z_e, e_pieces(0, 0, z_ed))
                             + at(z_a, a_pieces(3, xn[1], z_ad)))

        first = 2
        assert (NT - 2 - first) % unroll == 0 and unroll % 2 == 0

        def body(k, c):
            new_block()
            for u in range(unroll):
                blk('loop', step)(first + k * unroll + u, (first + u) % 2)
            return c

        xr_copy.wait()
        mark('s8_loop')
        jax.lax.fori_loop(0, (NT - 2 - first) // unroll, body, 0)
        mark('s9_tail')

        for c in grp_ffn:
            c.wait()
        new_block()
        L = NT - 1
        src = xn[L % 2]
        qn, kn, kp = (qq[L % 2], kk[L % 2], kk[1 - L % 2]) if qkpar else (qs, ks, ks)
        sp = {}

        def sp_in():
            sp['idx'], sp['mx'] = pick()
            sp['base'], sp['o16'], sp['xb'] = ffn_in(sp['idx'])
            sp['act'] = []

        def sp_half(k):
            c0 = (k // 2) * 128
            r = jnp.dot(sp['xb'], as_bf16((wu if k % 2 else wg)[:, c0:c0 + 128]), preferred_element_type=f32)
            if k % 2:
                sp['act'].append(swiglu(sp['g'], r))
            else:
                sp['g'] = r

        def sp_out():
            ffn_out(jnp.concatenate(sp['act'], axis=1), sp['idx'], sp['base'], sp['mx'], sp['o16'])

        blk('tail', interleave)(b_slots(0, src, qn) + b_slots(1, src, kn, kp) + b_slots(2, src, va, vs)
                                + d_slots(L - 1, os_) + d_slots(L, osa),
                                at(t_e0, e_pieces(L - 2, L % 2, t_ed0))
                                + [(t_in, sp_in)]
                                + at(t_pv0, pv_pieces(ls, vs, os_))
                                + at(t_qk, qk_pieces(qn, kn, lsa))
                                + at(t_pv, pv_pieces(lsa, va, osa, t_pvtok))
                                + at(t_act, [functools.partial(sp_half, k) for k in range(2 * F // 128)])
                                + at(t_e, e_pieces(L - 1, (L - 1) % 2, t_ed))
                                + [(25, sp_out)]
                                + spread(e_pieces(L, L % 2), 25, 26))

        mark('sa_final')
        idx, mx = pick()
        o_copy(0, S - NLAST * T, False).wait()
        late_copies = o_copy(S - NLAST * T, NLAST * T, True)
        hit = idx == sp['idx'] if sp else idx < 0

        @pl.when(hit)
        def _():
            fix_copy(sp['base'] if sp else 0).start()
            late_copies.wait()
            fix_copy(sp['base'] if sp else 0).wait()

        @pl.when(jnp.logical_not(hit))
        def _():
            base, o16, xb = ffn_in(idx)
            act = swiglu(jnp.dot(xb, as_bf16(wg[...]), preferred_element_type=f32),
                         jnp.dot(xb, as_bf16(wu[...]), preferred_element_type=f32))
            ffn_out(act, idx, base, mx, o16)
            late_copies.wait()
            fix_copy(base).start()
            fix_copy(base).wait()
        mark(None)

    lhs_buf = pltpu.VMEM((T // 2, D), u32)
    q_buf = pltpu.VMEM((8, T + padq, 128), f32)
    kv_buf = pltpu.VMEM((8, T + HALO + padk, 128), f32)
    l_buf = pltpu.VMEM((NW, T + padl, 128), f32)
    scratch = [
        pltpu.VMEM((S // 2, D), u32),
        pltpu.VMEM((D // 2, 3 * D), u32),
        pltpu.VMEM((D // 2, D), u32),
        pltpu.VMEM((D // 2, 3 * D), u32),
        pltpu.VMEM((D // 2, D), u32),
        pltpu.VMEM((NJ, D, 128), f32),
        pltpu.VMEM((D // 2, D), u32),
        pltpu.VMEM((D,), bf16),
        pltpu.VMEM((1280 + 2048 * 7,), bf16),
        pltpu.VMEM((64, D), f32),
        pltpu.VMEM((D // 2, F), u32),
        pltpu.VMEM((D // 2, F), u32),
        pltpu.VMEM((F // 2, D), u32),
        lhs_buf, lhs_buf, lhs_buf,
        q_buf, q_buf, q_buf,
        pltpu.VMEM((64, 128), u32),
        kv_buf, kv_buf,
        pltpu.VMEM((8, 8, 128), f32),
        kv_buf, kv_buf,
        l_buf, l_buf,
        lhs_buf, lhs_buf,
        pltpu.VMEM((S, D), f32),
        pltpu.VMEM((S, D), bf16),
        pltpu.VMEM((128, D), bf16),
        pltpu.SemaphoreType.DMA((3 + NWQ,)),
    ]
    return kernel, scratch


def build(**kw):
    kernel, scratch = make_kernel(**kw)

    def fn(A_x, A_wqkv, A_wo, B_x, B_w_r, B_w_gate, B_w_up, B_w_down):
        x2 = A_x.reshape(S, D)
        out = pl.pallas_call(
            kernel,
            in_specs=[pl.BlockSpec(memory_space=pl.ANY)] * 7,
            out_specs=pl.BlockSpec(memory_space=pl.ANY),
            out_shape=jax.ShapeDtypeStruct((S, D), bf16),
            scratch_shapes=scratch,
            name="fused",
            compiler_params=pltpu.CompilerParams(vmem_limit_bytes=100 * 2**20, disable_bounds_checks=True),
        )(x2, A_wqkv, A_wo, B_w_r, B_w_gate, B_w_up, B_w_down)
        return out.reshape(1, S, D)
    return fn


_fn = build()


@jax.jit
def pallas_sequential_preLN__sliding_local_dilated__moe_arch_mod__prompt_kernel(
    A_x: jax.Array,
    A_wqkv: jax.Array,
    A_wo: jax.Array,
    B_x: jax.Array,
    B_w_r: jax.Array,
    B_w_gate: jax.Array,
    B_w_up: jax.Array,
    B_w_down: jax.Array,
):
    return _fn(A_x, A_wqkv, A_wo, B_x, B_w_r, B_w_gate, B_w_up, B_w_down)
```

```python
import functools
import math
import jax
import jax.numpy as jnp
from jax.experimental import pallas as pl
from jax.experimental.pallas import tpu as pltpu

S, D, H, DH, F = 2048, 640, 32, 20, 1536
NW, DIL = 8, 2
HALO = 16
NJ = D // 128
EPS = 1e-5
QSCALE = (DH ** -0.5) * math.log2(math.e)
f32, bf16, u32, i32 = jnp.float32, jnp.bfloat16, jnp.uint32, jnp.int32


def interleave(slots, pieces):
    pieces = sorted(pieces, key=lambda kp: kp[0])
    for k, p in pieces:
        if k < 0:
            p()
    for c, s in enumerate(slots):
        s()
        for k, p in pieces:
            if k == c:
                p()
    for k, p in pieces:
        if k >= len(slots):
            p()


def spread(pieces, lo, hi):
    n = len(pieces)
    return [(lo + (k * (hi - lo)) // n, p) for k, p in enumerate(pieces)]


def at(sched, pieces):
    k = len(pieces) // len(sched)
    sched = [c for c in sched for _ in range(k)]
    return list(zip(sched, pieces, strict=True))


def pack2(even, odd):
    p = pltpu.pack_elementwise([even, odd], packed_dtype=bf16)
    return p if p.dtype == u32 else pltpu.bitcast(p, u32)


def as_bf16(x_u32):
    return pltpu.bitcast(x_u32, bf16)


def or_bits(x, g):
    return pltpu.bitcast(pltpu.bitcast(x, u32) | g, f32)


def fold(op, xs, tree):
    xs = list(xs)
    if not tree:
        return functools.reduce(op, xs)
    while len(xs) > 1:
        xs = [op(xs[i], xs[i + 1]) if i + 1 < len(xs) else xs[i] for i in range(0, len(xs), 2)]
    return xs[0]


def rsqrt(v):
    return jnp.exp2(jnp.log2(v) * -0.5)


def make_kernel(T=128, LNB=64, unroll=4, NWQ=4, only=None, scopes=False,
                pv_sched=(2, 3, 4, 5, 6, 7, 8, 9), pv_lag=2, a_sched=(16, 17), a_d=2,
                e_sched=(0, 3), e_d=4, qk_sched=(9, 10, 11, 11, 12, 13, 13, 14),
                qkpar=True, qk_tree=False, sm_tree=False, pv_order='w',
                sel_pb=64, perm_sched=(2, 2, 3, 3, 4),
                y_qk0=(1, 1, 2, 4, 4, 5, 5, 8), y_qk1=(6, 7, 7, 7, 10, 10, 12, 12),
                y_pv=(9, 10, 11, 11, 12, 13, 13, 14), y_pvtok=False,
                z_wo=(-1, 1, 2, 2, 3), z_pv=(0, 1, 2, 4, 5, 6, 7, 8), z_qk=(10, 11, 12, 13, 14, 15, 16, 16),
                z_e=(13, 16), z_ed=1, z_a=(16, 17), z_ad=2,
                t_e0=(-1, 2), t_ed0=5, t_pv0=(3, 4, 5, 6, 7, 8, 9, 10), t_qk=(9, 10, 11, 11, 11, 11, 12, 14),
                t_pv=(16, 17, 18, 19, 19, 19, 19, 19), t_pvtok=False, t_e=(21, 22), t_ed=2, t_in=6,
                t_act=(8, 9, 10, 11, 12, 13, 14, 15, 16, 17, 18, 19, 20, 21, 22, 23, 23, 24, 24, 24, 24, 24, 24, 24),
                t_down=(24,),
                padq=8, padl=8, padk=24, ):
    NT = S // T
    NG = T // 16

    def kernel(x_hbm, wqkv_hbm, wo_hbm, wr_hbm, wg_hbm, wu_hbm, wd_hbm, out_hbm,
               xs, wraw, wt, wp, woraw, wof, wop, wr, filler, wrf, wg, wu, wd,
               xn0, xn1, xna, qs, qa, qb, zv_, ks, ka, best, vs, va, ls, lsa, os_, osa, hs, outs, fixbuf,
               sems):
        x_u, wqkv_u, wo_u, wg_u, wu_u, wd_u = [r.bitcast(u32) for r in
                                               (x_hbm, wqkv_hbm, wo_hbm, wg_hbm, wu_hbm, wd_hbm)]
        xn, qq, kk = (xn0, xn1), (qs, qa), (ks, ka)

        zv = zv_.at[pl.ds(0, 8)]
        pending = []
        hist = []

        def new_block():
            hist.clear()
            pending.clear()

        def emit_token(val_u32, d=1):
            pending.append((len(hist) + d - 1, val_u32))

        def gated(w_u32):
            due = [v for (c, v) in pending if c <= len(hist)]
            pending[:] = [(c, v) for (c, v) in pending if c > len(hist)]
            if not due:
                return w_u32
            t = due.pop()
            while due:
                t = t | due.pop()
            return jnp.concatenate([w_u32[0:8] | (t & zv[...]), w_u32[8:]], axis=0)

        def zero_of(v):
            return pltpu.bitcast(v, u32) & zv[...]

        def gate_after(lag):
            return zero_of(hist[-1 - lag]) if len(hist) > lag else None

        def row0(i):
            return i * T if isinstance(i, int) else pl.multiple_of(i * T, T)

        def xrows(r, n):
            return pl.ds(r // 2 if isinstance(r, int) else pl.multiple_of(r // 2, 8), n // 2)

        S_A, S_B, S_C = 0, 1, 2
        S_Q = [3 + c for c in range(NWQ)]
        WQR = D // NWQ
        NLAST = 2

        def x_copy(t0, t1, sem):
            rows = pl.ds(t0 * T // 2, (t1 - t0) * T // 2)
            return pltpu.make_async_copy(x_u.at[rows], xs.at[rows], sems.at[sem])

        def w_copy(p, sem):
            return pltpu.make_async_copy(wqkv_u.at[:, pl.ds(p * D, D)], wraw.at[:, pl.ds(p * D, D)], sems.at[sem])

        def wq_copy(c):
            rows = pl.ds(c * WQR // 2, WQR // 2)
            return pltpu.make_async_copy(wqkv_u.at[rows, pl.ds(0, D)], wraw.at[rows, pl.ds(0, D)], sems.at[S_Q[c]])

        x0_copy = x_copy(0, 1, S_A)
        x12_copy = x_copy(1, 3, S_B)
        wk_copy = w_copy(1, S_C)
        wv_copy = w_copy(2, S_A)
        grp_wo = [pltpu.make_async_copy(wr_hbm, wr, sems.at[S_Q[0]]),
                  pltpu.make_async_copy(wo_u, woraw, sems.at[S_Q[0]]),
                  x_copy(3, 4, S_Q[0])]
        xr_copy = x_copy(4, NT, S_Q[1])
        grp_ffn = [pltpu.make_async_copy(wg_u, wg, sems.at[S_B]),
                   pltpu.make_async_copy(wu_u, wu, sems.at[S_B]),
                   pltpu.make_async_copy(wd_u, wd, sems.at[S_B])]

        def o_copy(r, n, late):
            return pltpu.make_async_copy(outs.at[pl.ds(r, n)], out_hbm.at[pl.ds(r, n)],
                                         sems.at[S_B if late else S_C])

        def fix_copy(base):
            return pltpu.make_async_copy(fixbuf.at[pl.ds(0, 16)], out_hbm.at[pl.ds(base, 16)], sems.at[S_A])

        def prep_w_pieces(p, lo=0, hi=D, PB=128):
            def sel(r0):
                r5 = (jax.lax.broadcasted_iota(i32, (PB // 2, 128), 1) // 4) % 5
                src = [wraw[r0 // 2:(r0 + PB) // 2, p * D + jj * 128: p * D + (jj + 1) * 128] for jj in range(NJ)]
                for j in range(NJ):
                    t = src[4]
                    for jj in range(4):
                        t = jnp.where(r5 == (j - 2 * jj) % 5, src[jj], t)
                    wt[r0 // 2:(r0 + PB) // 2, j * 128:(j + 1) * 128] = t

            def perm(j):
                lane = jax.lax.broadcasted_iota(i32, ((hi - lo) // 2, 128), 1)
                head = (lane % 32) // 2 + 16 * (lane % 2)
                idx = (20 * head + 4 * j + lane // 32) % 128
                wp[lo // 2:hi // 2, p * D + j * 128: p * D + (j + 1) * 128] = jnp.take_along_axis(
                    wt[lo // 2:hi // 2, j * 128:(j + 1) * 128], idx, axis=1)
            return ([functools.partial(sel, r0) for r0 in range(lo, hi, PB)]
                    + [functools.partial(perm, j) for j in range(NJ)])

        def prep_sched(p):
            ps = prep_w_pieces(p, 0, D, sel_pb)
            return spread(ps[:-NJ], -1, 2) + at(perm_sched, ps[-NJ:])

        def prep_wo_pieces():
            def piece(j):
                wof[j] = as_bf16(woraw[:, j * 128:(j + 1) * 128]).astype(f32)
                for d in range(DH):
                    wop[d * 16:(d + 1) * 16, j * 128:(j + 1) * 128] = pack2(
                        wof[j, pl.ds(d, H // 2, stride=DH), :],
                        wof[j, pl.ds(d + DH * (H // 2), H // 2, stride=DH), :])
            return [functools.partial(piece, j) for j in range(NJ)]

        def ln_stats(x):
            m = jnp.sum(x, axis=-1, keepdims=True) * (1.0 / D)
            v = jnp.maximum(jnp.sum(x * x, axis=-1, keepdims=True) * (1.0 / D) - m * m, 0.0)
            return m, rsqrt(v + EPS)

        def a_pieces(i, dst, d=0):
            r = row0(i)

            def piece(b):
                xu = xs[xrows(r + b * LNB, LNB), :]
                ys = []
                for half in range(2):
                    x = pltpu.unpack_elementwise(xu, index=half, packed_dtype=bf16, unpacked_dtype=f32)
                    m, rs = ln_stats(x)
                    ys.append(x * rs - m * rs)
                yu = pack2(ys[0], ys[1])
                dst[b * LNB // 2:(b + 1) * LNB // 2, :] = yu
                if d:
                    for r8 in range(LNB // 16):
                        emit_token(yu[r8 * 8:r8 * 8 + 8, D - 128:D], d)
            return [functools.partial(piece, b) for b in range(T // LNB)]

        def b_slots(p, src, dst, halo=None):
            def slot(j):
                c = p * D + j * 128
                res = jnp.dot(as_bf16(src[...]), as_bf16(gated(wp[:, c:c + 128])), preferred_element_type=f32)
                hist.append(res[0:8])
                if p == 0:
                    dst[j, 0:T, :] = res
                else:
                    dst[j, 0:HALO, :] = jnp.zeros((HALO, 128), f32) if halo is None else halo[j, T:T + HALO, :]
                    dst[j, HALO:HALO + T, :] = res
            return [functools.partial(slot, j) for j in range(NJ)]

        def ld16(ref, j, start):
            return jnp.concatenate([ref[j, pl.ds(start, 8, stride=2), :],
                                    ref[j, pl.ds(start + 1, 8, stride=2), :]], axis=0)

        def times8(x, v8):
            return (x.reshape(2, 8, 128) * v8[None]).reshape(16, 128)

        def qk_pieces(qr, kr, lr, first=False):
            def piece(g16):
                r0 = g16 * 16
                sv = jnp.full((8, 128), QSCALE, f32)
                gate = gate_after(0)
                if gate is not None:
                    sv = or_bits(sv, gate)
                q = [times8(ld16(qr, j, r0), sv) for j in range(NJ)]
                for w in range(NW):
                    if qk_tree:
                        a = fold(jnp.add, [q[j] * ld16(kr, j, HALO + r0 - DIL * w) for j in range(NJ)], True)
                    else:
                        a = None
                        for j in range(NJ):
                            t = q[j] * ld16(kr, j, HALO + r0 - DIL * w)
                            a = t if a is None else a + t
                    a = a + pltpu.roll(a, 64, 1)
                    a = a + pltpu.roll(a, 32, 1)
                    if first and r0 < DIL * w:
                        rows = jax.lax.broadcasted_iota(i32, (16, 128), 0)
                        rows = (rows % 8) * 2 + rows // 8 + r0
                        a = jnp.where(rows >= DIL * w, a, -1e9)
                    lr[w, r0:r0 + 16, :] = a
            return [functools.partial(piece, g) for g in range(NG)]

        def pv_pieces(lr, vr, orf, tok=True):
            def piece(g16):
                r0 = g16 * 16
                lw = [lr[w, r0:r0 + 16, :] for w in range(NW)]
                gate = gate_after(pv_lag) if tok else None
                m = fold(jnp.maximum, lw, sm_tree)
                if gate is not None:
                    m = pltpu.bitcast((pltpu.bitcast(m, u32).reshape(2, 8, 128) | gate[None]).reshape(16, 128), f32)
                es = [jnp.exp2(l - m) for l in lw]
                inv = pl.reciprocal(fold(jnp.add, es, sm_tree), approx=True)
                if pv_order == 'w':
                    acc = [None] * NJ
                    for w in range(NW):
                        for j in range(NJ):
                            t = es[w] * ld16(vr, j, HALO + r0 - DIL * w)
                            acc[j] = t if acc[j] is None else acc[j] + t
                for j in range(NJ):
                    if pv_order == 'w':
                        o = acc[j]
                    elif pv_order == 't':
                        o = fold(jnp.add, [es[w] * ld16(vr, j, HALO + r0 - DIL * w) for w in range(NW)], True)
                    else:
                        o = None
                        for w in range(NW):
                            t = es[w] * ld16(vr, j, HALO + r0 - DIL * w)
                            o = t if o is None else o + t
                    o = o * inv
                    ob = pack2(o[0:8], o[8:16])
                    orf[r0 // 2:r0 // 2 + 8, j * 128:(j + 1) * 128] = ob
                    if tok:
                        emit_token(ob)
            return [functools.partial(piece, g) for g in range(NG)]

        def d_slots(i, orf):
            r = row0(i)

            def slot(j):
                cols = slice(j * 128, (j + 1) * 128)
                res = jnp.dot(as_bf16(orf[...]), as_bf16(gated(wop[:, cols])), preferred_element_type=f32)
                hist.append(res[0:8])
                hs[pl.ds(r, T), cols] = res + as_bf16(xs[xrows(r, T), cols]).astype(f32)
            return [functools.partial(slot, j) for j in range(NJ)]

        def e_pieces(i, par, d=0):
            r = row0(i)

            def piece(b):
                rr = r + b * LNB
                h = hs[pl.ds(rr, LNB), :]
                m, rs = ln_stats(h)
                hw = (h.reshape(LNB // 8, 8, D) * wrf[0:8, :][None]).reshape(LNB, D)
                rv_all = (jnp.sum(hw, axis=-1, keepdims=True) - m * wrf[8:9, 0:1]) * rs
                ov = h * (1.0 + rs) - m * rs
                outs[pl.ds(rr, LNB), :] = ov.astype(bf16)
                bv = best[2 * par]
                bi = best[2 * par + 1]
                rows = (jax.lax.broadcasted_iota(i32, (8, 128), 0) + rr).astype(f32)
                for rb in range(LNB // 8):
                    rv = jnp.broadcast_to(rv_all[rb * 8:(rb + 1) * 8, :], (8, 128))
                    upd = rv > bv
                    bv = jnp.where(upd, rv, bv)
                    bi = jnp.where(upd, rows + float(rb * 8), bi)
                if d:
                    for r8 in range(LNB // 8):
                        emit_token(pltpu.bitcast(ov[r8 * 8:r8 * 8 + 8, D - 128:D], u32), d)
                    emit_token(pltpu.bitcast(bv, u32), d)
                best[2 * par] = bv
                best[2 * par + 1] = bi
                late = isinstance(i, int) and i >= NT - NLAST
                if isinstance(i, int) and i == NT - 1:
                    o_copy(rr, LNB, late).start()
                elif b == T // LNB - 1:
                    o_copy(r, T, late).start()
            return [functools.partial(piece, b) for b in range(T // LNB)]

        def step(i, par):
            src = xn[1 - par]
            qn, kn, kp = (qq[1 - par], kk[1 - par], kk[par]) if qkpar else (qs, ks, ks)
            interleave(b_slots(0, src, qn) + b_slots(1, src, kn, kp) + d_slots(i, os_) + b_slots(2, src, vs, vs),
                       at(e_sched, e_pieces(i - 1, par, e_d))
                       + at(pv_sched, pv_pieces(ls, vs, os_))
                       + at(qk_sched, qk_pieces(qn, kn, ls))
                       + at(a_sched, a_pieces(i + 2, xn[par], a_d)))

        def pick():
            bv = jnp.concatenate([best[0], best[2]], axis=0)
            bi = jnp.concatenate([best[1], best[3]], axis=0)
            mx = jnp.max(bv, axis=0, keepdims=True)
            cand = jnp.where(bv == mx, bi, float(S))
            idx_v = jnp.min(cand, axis=0, keepdims=True)
            return jnp.clip(idx_v.astype(i32)[0, 0], 0, S - 1), mx

        def ffn_in(idx):
            base = pl.multiple_of(jnp.clip(idx >> 4, 0, S // 16 - 1) * 16, 16)
            h16 = hs[pl.ds(base, 16), :]
            m16, rs16 = ln_stats(h16)
            hn16 = (h16 - m16) * rs16
            return base, h16 + hn16, hn16.astype(bf16)

        def swiglu(g, u):
            return (g * jax.nn.sigmoid(g) * u).astype(bf16)

        def ffn_out(act, idx, base, mx, o16, y=None):
            if y is None:
                y = jnp.dot(act, as_bf16(wd[...]), preferred_element_type=f32)
            gate = jax.nn.sigmoid(mx[:, 0:1])
            rows16 = jax.lax.broadcasted_iota(i32, (16, D), 0)
            fixbuf[0:16, :] = (o16 + jnp.where(rows16 == idx - base, y * gate, 0.0)).astype(bf16)

        def blk(name, f):
            return f if only is None or name in only else (lambda *a, **k: None)

        cur = [None]

        def mark(name):
            if not scopes:
                return
            if cur[0] is not None:
                cur[0].__exit__(None, None, None)
                cur[0] = None
            if name:
                cur[0] = jax.named_scope(name)
                cur[0].__enter__()

        mark("s0_start")
        x0_copy.start()
        for c in range(NWQ):
            wq_copy(c).start()
        x12_copy.start()
        wk_copy.start()
        zv[...] = jnp.zeros((8, 128), u32)
        filler[pl.ds(0, 1280)] = jnp.zeros((1280,), bf16)
        for par in range(2):
            best[2 * par] = jnp.full((8, 128), -jnp.inf, f32)
            best[2 * par + 1] = jnp.zeros((8, 128), f32)
        x0_copy.wait()
        for p in a_pieces(0, xna):
            p()
        for c in range(NWQ):
            wq_copy(c).wait()
            for p in prep_w_pieces(0, c * WQR, (c + 1) * WQR, WQR // 2 if WQR % 32 == 0 else WQR):
                p()
        wv_copy.start()
        x12_copy.wait()
        mark('s1_X')
        new_block()
        blk('X', interleave)(b_slots(0, xna, qa) + b_slots(0, xn[1], qb),
                             spread(a_pieces(1, xn[1]), 0, 2) + spread(a_pieces(2, xn[0], 2), 5, 8))
        for c in grp_wo:
            c.start()
        mark('s2_waitWk')
        wk_copy.wait()
        mark('s3_X2')
        new_block()
        blk('X2', interleave)(b_slots(0, xn[0], qs) + b_slots(1, xna, ka), prep_sched(1))
        xr_copy.start()
        mark('s4_waitWv')
        wv_copy.wait()
        mark('s5_Y')
        new_block()
        blk('Y', interleave)(b_slots(1, xn[1], ks, ka) + b_slots(2, xna, va) + b_slots(2, xn[1], vs, va),
                             prep_sched(2)
                             + at(y_qk0, qk_pieces(qa, ka, lsa, True))
                             + at(y_qk1, qk_pieces(qb, ks, ls))
                             + at(y_pv, pv_pieces(lsa, va, osa, y_pvtok)))
        for c in grp_ffn:
            c.start()
        mark('s6_waitWo')
        for c in grp_wo:
            c.wait()
        mark('s7_Z')
        new_block()
        wrv = jnp.broadcast_to((wr[...].astype(f32) + filler[pl.ds(0, D)].astype(f32)).reshape(1, D), (8, D))
        wrf[0:8, :] = wrv
        wrf[8:16, :] = jnp.broadcast_to(jnp.sum(wrv, axis=-1, keepdims=True), (8, D))
        blk('Z', interleave)(b_slots(1, xn[0], ks, ks) + d_slots(0, osa) + d_slots(1, os_)
                             + b_slots(2, xn[0], vs, vs),
                             at(z_wo, prep_wo_pieces())
                             + at(z_pv, pv_pieces(ls, vs, os_))
                             + at(z_qk, qk_pieces(qs, ks, ls))
                             + at(z_e, e_pieces(0, 0, z_ed))
                             + at(z_a, a_pieces(3, xn[1], z_ad)))

        first = 2
        assert (NT - 2 - first) % unroll == 0 and unroll % 2 == 0

        def body(k, c):
            new_block()
            for u in range(unroll):
                blk('loop', step)(first + k * unroll + u, (first + u) % 2)
            return c

        xr_copy.wait()
        mark('s8_loop')
        jax.lax.fori_loop(0, (NT - 2 - first) // unroll, body, 0)
        mark('s9_tail')

        for c in grp_ffn:
            c.wait()
        new_block()
        L = NT - 1
        src = xn[L % 2]
        qn, kn, kp = (qq[L % 2], kk[L % 2], kk[1 - L % 2]) if qkpar else (qs, ks, ks)
        sp = {}

        def sp_in():
            sp['idx'], sp['mx'] = pick()
            sp['base'], sp['o16'], sp['xb'] = ffn_in(sp['idx'])
            sp['act'] = []

        def sp_half(k):
            c0 = (k // 2) * 128
            r = jnp.dot(sp['xb'], as_bf16((wu if k % 2 else wg)[:, c0:c0 + 128]), preferred_element_type=f32)
            if k % 2:
                sp['act'].append(swiglu(sp['g'], r))
            else:
                sp['g'] = r

        def sp_down(kg, j):
            a = jnp.concatenate(sp['act'][4 * kg:4 * kg + 4], axis=1)
            r = jnp.dot(a, as_bf16(wd[kg * 256:(kg + 1) * 256, j * 128:(j + 1) * 128]), preferred_element_type=f32)
            sp['y', j] = r if kg == 0 else sp['y', j] + r

        def sp_out():
            if t_down:
                y = jnp.concatenate([sp['y', j] for j in range(NJ)], axis=1)
                ffn_out(None, sp['idx'], sp['base'], sp['mx'], sp['o16'], y)
            else:
                ffn_out(jnp.concatenate(sp['act'], axis=1), sp['idx'], sp['base'], sp['mx'], sp['o16'])

        blk('tail', interleave)(b_slots(0, src, qn) + b_slots(1, src, kn, kp) + b_slots(2, src, va, vs)
                                + d_slots(L - 1, os_) + d_slots(L, osa),
                                at(t_e0, e_pieces(L - 2, L % 2, t_ed0))
                                + [(t_in, sp_in)]
                                + at(t_pv0, pv_pieces(ls, vs, os_))
                                + at(t_qk, qk_pieces(qn, kn, lsa))
                                + at(t_pv, pv_pieces(lsa, va, osa, t_pvtok))
                                + at(t_act, [functools.partial(sp_half, k) for k in range(2 * F // 128)])
                                + (at(t_down, [functools.partial(sp_down, kg, j) for kg in range(3) for j in range(NJ)])
                                   if t_down else [])
                                + at(t_e, e_pieces(L - 1, (L - 1) % 2, t_ed))
                                + [(25, sp_out)]
                                + spread(e_pieces(L, L % 2), 25, 26))

        mark('sa_final')
        idx, mx = pick()
        o_copy(0, S - NLAST * T, False).wait()
        late_copies = o_copy(S - NLAST * T, NLAST * T, True)
        hit = idx == sp['idx'] if sp else idx < 0

        @pl.when(hit)
        def _():
            fix_copy(sp['base'] if sp else 0).start()
            late_copies.wait()
            fix_copy(sp['base'] if sp else 0).wait()

        @pl.when(jnp.logical_not(hit))
        def _():
            base, o16, xb = ffn_in(idx)
            act = swiglu(jnp.dot(xb, as_bf16(wg[...]), preferred_element_type=f32),
                         jnp.dot(xb, as_bf16(wu[...]), preferred_element_type=f32))
            ffn_out(act, idx, base, mx, o16)
            late_copies.wait()
            fix_copy(base).start()
            fix_copy(base).wait()
        mark(None)

    lhs_buf = pltpu.VMEM((T // 2, D), u32)
    q_buf = pltpu.VMEM((8, T + padq, 128), f32)
    kv_buf = pltpu.VMEM((8, T + HALO + padk, 128), f32)
    l_buf = pltpu.VMEM((NW, T + padl, 128), f32)
    scratch = [
        pltpu.VMEM((S // 2, D), u32),
        pltpu.VMEM((D // 2, 3 * D), u32),
        pltpu.VMEM((D // 2, D), u32),
        pltpu.VMEM((D // 2, 3 * D), u32),
        pltpu.VMEM((D // 2, D), u32),
        pltpu.VMEM((NJ, D, 128), f32),
        pltpu.VMEM((D // 2, D), u32),
        pltpu.VMEM((D,), bf16),
        pltpu.VMEM((1280 + 2048 * 7,), bf16),
        pltpu.VMEM((64, D), f32),
        pltpu.VMEM((D // 2, F), u32),
        pltpu.VMEM((D // 2, F), u32),
        pltpu.VMEM((F // 2, D), u32),
        lhs_buf, lhs_buf, lhs_buf,
        q_buf, q_buf, q_buf,
        pltpu.VMEM((64, 128), u32),
        kv_buf, kv_buf,
        pltpu.VMEM((8, 8, 128), f32),
        kv_buf, kv_buf,
        l_buf, l_buf,
        lhs_buf, lhs_buf,
        pltpu.VMEM((S, D), f32),
        pltpu.VMEM((S, D), bf16),
        pltpu.VMEM((128, D), bf16),
        pltpu.SemaphoreType.DMA((3 + NWQ,)),
    ]
    return kernel, scratch


def build(**kw):
    kernel, scratch = make_kernel(**kw)

    def fn(A_x, A_wqkv, A_wo, B_x, B_w_r, B_w_gate, B_w_up, B_w_down):
        x2 = A_x.reshape(S, D)
        out = pl.pallas_call(
            kernel,
            in_specs=[pl.BlockSpec(memory_space=pl.ANY)] * 7,
            out_specs=pl.BlockSpec(memory_space=pl.ANY),
            out_shape=jax.ShapeDtypeStruct((S, D), bf16),
            scratch_shapes=scratch,
            name="fused",
            compiler_params=pltpu.CompilerParams(vmem_limit_bytes=100 * 2**20, disable_bounds_checks=True),
        )(x2, A_wqkv, A_wo, B_w_r, B_w_gate, B_w_up, B_w_down)
        return out.reshape(1, S, D)
    return fn


_fn = build()


@jax.jit
def pallas_sequential_preLN__sliding_local_dilated__moe_arch_mod__prompt_kernel(
    A_x: jax.Array,
    A_wqkv: jax.Array,
    A_wo: jax.Array,
    B_x: jax.Array,
    B_w_r: jax.Array,
    B_w_gate: jax.Array,
    B_w_up: jax.Array,
    B_w_down: jax.Array,
):
    return _fn(A_x, A_wqkv, A_wo, B_x, B_w_r, B_w_gate, B_w_up, B_w_down)
```

```python
import functools
import math
import jax
import jax.numpy as jnp
from jax.experimental import pallas as pl
from jax.experimental.pallas import tpu as pltpu

S, D, H, DH, F = 2048, 640, 32, 20, 1536
NW, DIL = 8, 2
HALO = 16
NJ = D // 128
EPS = 1e-5
QSCALE = (DH ** -0.5) * math.log2(math.e)
f32, bf16, u32, i32 = jnp.float32, jnp.bfloat16, jnp.uint32, jnp.int32


def interleave(slots, pieces):
    pieces = sorted(pieces, key=lambda kp: kp[0])
    for k, p in pieces:
        if k < 0:
            p()
    for c, s in enumerate(slots):
        s()
        for k, p in pieces:
            if k == c:
                p()
    for k, p in pieces:
        if k >= len(slots):
            p()


def spread(pieces, lo, hi):
    n = len(pieces)
    return [(lo + (k * (hi - lo)) // n, p) for k, p in enumerate(pieces)]


def at(sched, pieces):
    k = len(pieces) // len(sched)
    sched = [c for c in sched for _ in range(k)]
    return list(zip(sched, pieces, strict=True))


def pack2(even, odd):
    p = pltpu.pack_elementwise([even, odd], packed_dtype=bf16)
    return p if p.dtype == u32 else pltpu.bitcast(p, u32)


def as_bf16(x_u32):
    return pltpu.bitcast(x_u32, bf16)


def or_bits(x, g):
    return pltpu.bitcast(pltpu.bitcast(x, u32) | g, f32)


def fold(op, xs, tree):
    xs = list(xs)
    if not tree:
        return functools.reduce(op, xs)
    while len(xs) > 1:
        xs = [op(xs[i], xs[i + 1]) if i + 1 < len(xs) else xs[i] for i in range(0, len(xs), 2)]
    return xs[0]


def rsqrt(v):
    return jnp.exp2(jnp.log2(v) * -0.5)


def make_kernel(T=128, LNB=64, unroll=4, NWQ=4, only=None, scopes=False,
                pv_sched=(2, 3, 4, 5, 6, 7, 8, 9), pv_lag=2, a_sched=(16, 17), a_d=2,
                e_sched=(0, 3), e_d=4, qk_sched=(9, 10, 11, 11, 12, 13, 13, 14),
                qk_tree=False, sm_tree=False, pv_order='w',
                x_qk=(4, 4, 5, 5, 6, 6, 7, 7),
                y_qk1=(0, 2, 3, 3, 4, 4, 6, 7), y_a=(4, 4), y_ad=1, y_pv0=(5, 6, 7, 8, 9, 10, 11, 12),
                y_pv1=(12, 13, 14, 15, 16, 17, 18, 19), y_pvtok=True,
                z_qk=(0, 1, 1, 2, 4, 4, 6, 7), z_e=(6, 9), z_ed=0, z_a=(10, 11), z_ad=3,
                t_e0=(-1, 2), t_ed0=5, t_pv0=(3, 4, 5, 6, 7, 8, 9, 10), t_qk=(9, 10, 11, 11, 11, 11, 12, 14),
                t_pv=(16, 17, 18, 19, 19, 19, 19, 19), t_pvtok=False, t_e=(21, 22), t_ed=2, t_in=6,
                t_act=(8, 9, 10, 11, 12, 13, 14, 15, 16, 17, 18, 19, 20, 21, 22, 23, 23, 24, 24, 24, 24, 24, 24, 24),
                t_down=(24,),
                padq=8, padl=8, padk=24, ):
    NT = S // T
    NG = T // 16

    def kernel(x_hbm, wqkv_hbm, wo_hbm, wr_hbm, wg_hbm, wu_hbm, wd_hbm, out_hbm,
               xs, wraw, wp, woraw, wop, wr, filler, wrf, wg, wu, wd,
               xn0, xn1, qs, qa, zv_, ks, ka, best, vs, va, ls, lsa, os_, osa, hs, outs, fixbuf,
               sems):
        x_u, wqkv_u, wo_u, wg_u, wu_u, wd_u = [r.bitcast(u32) for r in
                                               (x_hbm, wqkv_hbm, wo_hbm, wg_hbm, wu_hbm, wd_hbm)]
        xn, qq, kk = (xn0, xn1), (qs, qa), (ks, ka)

        zv = zv_.at[pl.ds(0, 8)]
        pending = []
        hist = []

        def new_block():
            hist.clear()
            pending.clear()

        def emit_token(val_u32, d=1):
            pending.append((len(hist) + d - 1, val_u32))

        def gated(w_u32):
            due = [v for (c, v) in pending if c <= len(hist)]
            pending[:] = [(c, v) for (c, v) in pending if c > len(hist)]
            if not due:
                return w_u32
            t = due.pop()
            while due:
                t = t | due.pop()
            return jnp.concatenate([w_u32[0:8] | (t & zv[...]), w_u32[8:]], axis=0)

        def zero_of(v):
            return pltpu.bitcast(v, u32) & zv[...]

        def gate_after(lag):
            return zero_of(hist[-1 - lag]) if len(hist) > lag else None

        def row0(i):
            return i * T if isinstance(i, int) else pl.multiple_of(i * T, T)

        def xrows(r, n):
            return pl.ds(r // 2 if isinstance(r, int) else pl.multiple_of(r // 2, 8), n // 2)

        S_A, S_B, S_C = 0, 1, 2
        S_Q = [3 + c for c in range(NWQ)]
        WQR = D // NWQ
        NLAST = 2

        def x_copy(t0, t1, sem):
            rows = pl.ds(t0 * T // 2, (t1 - t0) * T // 2)
            return pltpu.make_async_copy(x_u.at[rows], xs.at[rows], sems.at[sem])

        def w_copy(p, sem):
            return pltpu.make_async_copy(wqkv_u.at[:, pl.ds(p * D, D)], wraw.at[:, pl.ds(p * D, D)], sems.at[sem])

        def wq_copy(c):
            rows = pl.ds(c * WQR // 2, WQR // 2)
            return pltpu.make_async_copy(wqkv_u.at[rows, pl.ds(0, D)], wraw.at[rows, pl.ds(0, D)], sems.at[S_Q[c]])

        x0_copy = x_copy(0, 1, S_A)
        x1_copy = x_copy(1, 2, S_B)
        wk_copy = w_copy(1, S_C)
        grp_wv = [x_copy(2, 3, S_A), w_copy(2, S_A)]
        grp_wo = [pltpu.make_async_copy(wr_hbm, wr, sems.at[S_Q[0]]),
                  x_copy(3, 4, S_Q[0])]
        grp_wo += [pltpu.make_async_copy(wo_u.at[:, pl.ds(j * 128, 128)], woraw.at[j], sems.at[S_Q[0]])
                   for j in range(NJ)]
        xr_copy = x_copy(4, NT, S_Q[1])
        grp_ffn = [pltpu.make_async_copy(wg_u, wg, sems.at[S_B]),
                   pltpu.make_async_copy(wu_u, wu, sems.at[S_B]),
                   pltpu.make_async_copy(wd_u, wd, sems.at[S_B])]

        def o_copy(r, n, late):
            return pltpu.make_async_copy(outs.at[pl.ds(r, n)], out_hbm.at[pl.ds(r, n)],
                                         sems.at[S_B if late else S_C])

        def fix_copy(base):
            return pltpu.make_async_copy(fixbuf.at[pl.ds(0, 16)], out_hbm.at[pl.ds(base, 16)], sems.at[S_A])

        def prep_j(p, j, lo=0, hi=D):
            rows = slice(lo // 2, hi // 2)
            lane = jax.lax.broadcasted_iota(i32, ((hi - lo) // 2, 128), 1)
            r5 = (lane // 4) % 5
            t = wraw[rows, p * D + 4 * 128: p * D + 5 * 128]
            for jj in range(4):
                t = jnp.where(r5 == (j - 2 * jj) % 5, wraw[rows, p * D + jj * 128: p * D + (jj + 1) * 128], t)
            head = (lane % 32) // 2 + 16 * (lane % 2)
            idx = (20 * head + 4 * j + lane // 32) % 128
            wp[rows, p * D + j * 128: p * D + (j + 1) * 128] = jnp.take_along_axis(t, idx, axis=1)

        def with_prep(preps, slots):
            return [lambda f=f, g=g: (f(), g()) for f, g in zip(preps, slots, strict=True)]

        def prep_w(p):
            return [functools.partial(prep_j, p, j) for j in range(NJ)]

        def prep_wo_pieces():
            def piece(j):
                for d in range(0, DH, 2):
                    lo = woraw[j, pl.ds(d // 2, H // 2, stride=DH // 2), :]
                    hi = woraw[j, pl.ds(d // 2 + (DH // 2) * (H // 2), H // 2, stride=DH // 2), :]
                    cols = slice(j * 128, (j + 1) * 128)
                    wop[d * 16:(d + 1) * 16, cols] = (lo & jnp.uint32(0xFFFF)) | (hi << 16)
                    wop[(d + 1) * 16:(d + 2) * 16, cols] = (lo >> 16) | (hi & jnp.uint32(0xFFFF0000))
            return [functools.partial(piece, j) for j in range(NJ)]

        def ln_stats(x):
            m = jnp.sum(x, axis=-1, keepdims=True) * (1.0 / D)
            v = jnp.maximum(jnp.sum(x * x, axis=-1, keepdims=True) * (1.0 / D) - m * m, 0.0)
            return m, rsqrt(v + EPS)

        def a_pieces(i, dst, d=0):
            r = row0(i)

            def piece(b):
                xu = xs[xrows(r + b * LNB, LNB), :]
                ys = []
                for half in range(2):
                    x = pltpu.unpack_elementwise(xu, index=half, packed_dtype=bf16, unpacked_dtype=f32)
                    m, rs = ln_stats(x)
                    ys.append(x * rs - m * rs)
                yu = pack2(ys[0], ys[1])
                dst[b * LNB // 2:(b + 1) * LNB // 2, :] = yu
                if d:
                    for r8 in range(LNB // 16):
                        emit_token(yu[r8 * 8:r8 * 8 + 8, D - 128:D], d)
            return [functools.partial(piece, b) for b in range(T // LNB)]

        def b_slots(p, src, dst, halo=None):
            def slot(j):
                c = p * D + j * 128
                res = jnp.dot(as_bf16(src[...]), as_bf16(gated(wp[:, c:c + 128])), preferred_element_type=f32)
                hist.append(res[0:8])
                if p == 0:
                    dst[j, 0:T, :] = res
                else:
                    dst[j, 0:HALO, :] = jnp.zeros((HALO, 128), f32) if halo is None else halo[j, T:T + HALO, :]
                    dst[j, HALO:HALO + T, :] = res
            return [functools.partial(slot, j) for j in range(NJ)]

        def ld16(ref, j, start):
            return jnp.concatenate([ref[j, pl.ds(start, 8, stride=2), :],
                                    ref[j, pl.ds(start + 1, 8, stride=2), :]], axis=0)

        def times8(x, v8):
            return (x.reshape(2, 8, 128) * v8[None]).reshape(16, 128)

        def qk_pieces(qr, kr, lr, first=False):
            def piece(g16):
                r0 = g16 * 16
                sv = jnp.full((8, 128), QSCALE, f32)
                gate = gate_after(0)
                if gate is not None:
                    sv = or_bits(sv, gate)
                q = [times8(ld16(qr, j, r0), sv) for j in range(NJ)]
                for w in range(NW):
                    if qk_tree:
                        a = fold(jnp.add, [q[j] * ld16(kr, j, HALO + r0 - DIL * w) for j in range(NJ)], True)
                    else:
                        a = None
                        for j in range(NJ):
                            t = q[j] * ld16(kr, j, HALO + r0 - DIL * w)
                            a = t if a is None else a + t
                    a = a + pltpu.roll(a, 64, 1)
                    a = a + pltpu.roll(a, 32, 1)
                    if first and r0 < DIL * w:
                        rows = jax.lax.broadcasted_iota(i32, (16, 128), 0)
                        rows = (rows % 8) * 2 + rows // 8 + r0
                        a = jnp.where(rows >= DIL * w, a, -1e9)
                    lr[w, r0:r0 + 16, :] = a
            return [functools.partial(piece, g) for g in range(NG)]

        def pv_pieces(lr, vr, orf, tok=True):
            def piece(g16):
                r0 = g16 * 16
                lw = [lr[w, r0:r0 + 16, :] for w in range(NW)]
                gate = gate_after(pv_lag) if tok else None
                m = fold(jnp.maximum, lw, sm_tree)
                if gate is not None:
                    m = pltpu.bitcast((pltpu.bitcast(m, u32).reshape(2, 8, 128) | gate[None]).reshape(16, 128), f32)
                es = [jnp.exp2(l - m) for l in lw]
                inv = pl.reciprocal(fold(jnp.add, es, sm_tree), approx=True)
                if pv_order == 'w':
                    acc = [None] * NJ
                    for w in range(NW):
                        for j in range(NJ):
                            t = es[w] * ld16(vr, j, HALO + r0 - DIL * w)
                            acc[j] = t if acc[j] is None else acc[j] + t
                for j in range(NJ):
                    if pv_order == 'w':
                        o = acc[j]
                    elif pv_order == 't':
                        o = fold(jnp.add, [es[w] * ld16(vr, j, HALO + r0 - DIL * w) for w in range(NW)], True)
                    else:
                        o = None
                        for w in range(NW):
                            t = es[w] * ld16(vr, j, HALO + r0 - DIL * w)
                            o = t if o is None else o + t
                    o = o * inv
                    ob = pack2(o[0:8], o[8:16])
                    orf[r0 // 2:r0 // 2 + 8, j * 128:(j + 1) * 128] = ob
                    if tok:
                        emit_token(ob)
            return [functools.partial(piece, g) for g in range(NG)]

        def d_slots(i, orf):
            r = row0(i)

            def slot(j):
                cols = slice(j * 128, (j + 1) * 128)
                res = jnp.dot(as_bf16(orf[...]), as_bf16(gated(wop[:, cols])), preferred_element_type=f32)
                hist.append(res[0:8])
                hs[pl.ds(r, T), cols] = res + as_bf16(xs[xrows(r, T), cols]).astype(f32)
            return [functools.partial(slot, j) for j in range(NJ)]

        def e_pieces(i, par, d=0):
            r = row0(i)

            def piece(b):
                rr = r + b * LNB
                h = hs[pl.ds(rr, LNB), :]
                m, rs = ln_stats(h)
                hw = (h.reshape(LNB // 8, 8, D) * wrf[0:8, :][None]).reshape(LNB, D)
                rv_all = (jnp.sum(hw, axis=-1, keepdims=True) - m * wrf[8:9, 0:1]) * rs
                ov = h * (1.0 + rs) - m * rs
                outs[pl.ds(rr, LNB), :] = ov.astype(bf16)
                bv = best[2 * par]
                bi = best[2 * par + 1]
                rows = (jax.lax.broadcasted_iota(i32, (8, 128), 0) + rr).astype(f32)
                for rb in range(LNB // 8):
                    rv = jnp.broadcast_to(rv_all[rb * 8:(rb + 1) * 8, :], (8, 128))
                    upd = rv > bv
                    bv = jnp.where(upd, rv, bv)
                    bi = jnp.where(upd, rows + float(rb * 8), bi)
                if d:
                    for r8 in range(LNB // 8):
                        emit_token(pltpu.bitcast(ov[r8 * 8:r8 * 8 + 8, D - 128:D], u32), d)
                    emit_token(pltpu.bitcast(bv, u32), d)
                best[2 * par] = bv
                best[2 * par + 1] = bi
                late = isinstance(i, int) and i >= NT - NLAST
                if isinstance(i, int) and i == NT - 1:
                    o_copy(rr, LNB, late).start()
                elif b == T // LNB - 1:
                    o_copy(r, T, late).start()
            return [functools.partial(piece, b) for b in range(T // LNB)]

        def step(i, par):
            src = xn[1 - par]
            qn, kn, kp = qq[1 - par], kk[1 - par], kk[par]
            interleave(b_slots(0, src, qn) + b_slots(1, src, kn, kp) + d_slots(i, os_) + b_slots(2, src, vs, vs),
                       at(e_sched, e_pieces(i - 1, par, e_d))
                       + at(pv_sched, pv_pieces(ls, vs, os_))
                       + at(qk_sched, qk_pieces(qn, kn, ls))
                       + at(a_sched, a_pieces(i + 2, xn[par], a_d)))

        def pick():
            bv = jnp.concatenate([best[0], best[2]], axis=0)
            bi = jnp.concatenate([best[1], best[3]], axis=0)
            mx = jnp.max(bv, axis=0, keepdims=True)
            cand = jnp.where(bv == mx, bi, float(S))
            idx_v = jnp.min(cand, axis=0, keepdims=True)
            return jnp.clip(idx_v.astype(i32)[0, 0], 0, S - 1), mx

        def ffn_in(idx):
            base = pl.multiple_of(jnp.clip(idx >> 4, 0, S // 16 - 1) * 16, 16)
            h16 = hs[pl.ds(base, 16), :]
            m16, rs16 = ln_stats(h16)
            hn16 = (h16 - m16) * rs16
            return base, h16 + hn16, hn16.astype(bf16)

        def swiglu(g, u):
            return (g * jax.nn.sigmoid(g) * u).astype(bf16)

        def ffn_out(act, idx, base, mx, o16, y=None):
            if y is None:
                y = jnp.dot(act, as_bf16(wd[...]), preferred_element_type=f32)
            gate = jax.nn.sigmoid(mx[:, 0:1])
            rows16 = jax.lax.broadcasted_iota(i32, (16, D), 0)
            fixbuf[0:16, :] = (o16 + jnp.where(rows16 == idx - base, y * gate, 0.0)).astype(bf16)

        def blk(name, f):
            return f if only is None or name in only else (lambda *a, **k: None)

        cur = [None]

        def mark(name):
            if not scopes:
                return
            if cur[0] is not None:
                cur[0].__exit__(None, None, None)
                cur[0] = None
            if name:
                cur[0] = jax.named_scope(name)
                cur[0].__enter__()

        mark("s0_start")
        x0_copy.start()
        for c in range(NWQ):
            wq_copy(c).start()
        x1_copy.start()
        wk_copy.start()
        zv[...] = jnp.zeros((8, 128), u32)
        filler[pl.ds(0, 1280)] = jnp.zeros((1280,), bf16)
        for par in range(2):
            best[2 * par] = jnp.full((8, 128), -jnp.inf, f32)
            best[2 * par + 1] = jnp.zeros((8, 128), f32)
        x0_copy.wait()
        for p in a_pieces(0, xn[0]):
            p()
        for c in range(NWQ):
            wq_copy(c).wait()
            if c == NWQ - 1:
                for cp in grp_wv:
                    cp.start()
                x1_copy.wait()
                mark('s1_X')
                new_block()
            for j in range(NJ):
                prep_j(0, j, c * WQR, (c + 1) * WQR)
        blk('X', interleave)(b_slots(0, xn[0], qq[0]) + b_slots(0, xn[1], qq[1]),
                             spread(a_pieces(1, xn[1]), 0, 2))
        for c in grp_wo:
            c.start()
        mark('s2_waitWk')
        wk_copy.wait()
        mark('s3_X2')
        new_block()
        blk('X2', interleave)(with_prep(prep_w(1), b_slots(1, xn[0], kk[0])) + b_slots(1, xn[1], kk[1], kk[0]),
                              at(x_qk, qk_pieces(qq[0], kk[0], lsa, True)))
        xr_copy.start()
        mark('s4_waitWv')
        for c in grp_wv:
            c.wait()
        mark('s5_Y')
        new_block()
        blk('Y', interleave)(with_prep(prep_w(2), b_slots(2, xn[0], va)) + b_slots(2, xn[1], vs, va)
                             + b_slots(0, xn[0], qq[0]) + b_slots(1, xn[0], kk[0], kk[1]),
                             at(y_qk1, qk_pieces(qq[1], kk[1], ls))
                             + at(y_a, a_pieces(2, xn[0], y_ad))
                             + at(y_pv0, pv_pieces(lsa, va, osa, y_pvtok))
                             + at(y_pv1, pv_pieces(ls, vs, os_, y_pvtok)))
        for c in grp_ffn:
            c.start()
        mark('s6_waitWo')
        for c in grp_wo:
            c.wait()
        mark('s7_Z')
        new_block()
        wrv = jnp.broadcast_to((wr[...].astype(f32) + filler[pl.ds(0, D)].astype(f32)).reshape(1, D), (8, D))
        wrf[0:8, :] = wrv
        wrf[8:16, :] = jnp.broadcast_to(jnp.sum(wrv, axis=-1, keepdims=True), (8, D))
        blk('Z', interleave)(with_prep(prep_wo_pieces(), d_slots(0, osa)) + d_slots(1, os_)
                             + b_slots(2, xn[0], vs, vs),
                             at(z_qk, qk_pieces(qq[0], kk[0], ls))
                             + at(z_e, e_pieces(0, 0, z_ed))
                             + at(z_a, a_pieces(3, xn[1], z_ad)))

        first = 2
        assert (NT - 2 - first) % unroll == 0 and unroll % 2 == 0

        def body(k, c):
            new_block()
            for u in range(unroll):
                blk('loop', step)(first + k * unroll + u, (first + u) % 2)
            return c

        xr_copy.wait()
        mark('s8_loop')
        jax.lax.fori_loop(0, (NT - 2 - first) // unroll, body, 0)
        mark('s9_tail')

        for c in grp_ffn:
            c.wait()
        new_block()
        L = NT - 1
        src = xn[L % 2]
        qn, kn, kp = qq[L % 2], kk[L % 2], kk[1 - L % 2]
        sp = {}

        def sp_in():
            sp['idx'], sp['mx'] = pick()
            sp['base'], sp['o16'], sp['xb'] = ffn_in(sp['idx'])
            sp['act'] = []

        def sp_half(k):
            c0 = (k // 2) * 128
            r = jnp.dot(sp['xb'], as_bf16((wu if k % 2 else wg)[:, c0:c0 + 128]), preferred_element_type=f32)
            if k % 2:
                sp['act'].append(swiglu(sp['g'], r))
            else:
                sp['g'] = r

        def sp_down(kg, j):
            a = jnp.concatenate(sp['act'][4 * kg:4 * kg + 4], axis=1)
            r = jnp.dot(a, as_bf16(wd[kg * 256:(kg + 1) * 256, j * 128:(j + 1) * 128]), preferred_element_type=f32)
            sp['y', j] = r if kg == 0 else sp['y', j] + r

        def sp_out():
            if t_down:
                y = jnp.concatenate([sp['y', j] for j in range(NJ)], axis=1)
                ffn_out(None, sp['idx'], sp['base'], sp['mx'], sp['o16'], y)
            else:
                ffn_out(jnp.concatenate(sp['act'], axis=1), sp['idx'], sp['base'], sp['mx'], sp['o16'])

        blk('tail', interleave)(b_slots(0, src, qn) + b_slots(1, src, kn, kp) + b_slots(2, src, va, vs)
                                + d_slots(L - 1, os_) + d_slots(L, osa),
                                at(t_e0, e_pieces(L - 2, L % 2, t_ed0))
                                + [(t_in, sp_in)]
                                + at(t_pv0, pv_pieces(ls, vs, os_))
                                + at(t_qk, qk_pieces(qn, kn, lsa))
                                + at(t_pv, pv_pieces(lsa, va, osa, t_pvtok))
                                + at(t_act, [functools.partial(sp_half, k) for k in range(2 * F // 128)])
                                + (at(t_down, [functools.partial(sp_down, kg, j) for kg in range(3) for j in range(NJ)])
                                   if t_down else [])
                                + at(t_e, e_pieces(L - 1, (L - 1) % 2, t_ed))
                                + [(25, sp_out)]
                                + spread(e_pieces(L, L % 2), 25, 26))

        mark('sa_final')
        idx, mx = pick()
        o_copy(0, S - NLAST * T, False).wait()
        late_copies = o_copy(S - NLAST * T, NLAST * T, True)
        hit = idx == sp['idx'] if sp else idx < 0

        @pl.when(hit)
        def _():
            fix_copy(sp['base'] if sp else 0).start()
            late_copies.wait()
            fix_copy(sp['base'] if sp else 0).wait()

        @pl.when(jnp.logical_not(hit))
        def _():
            base, o16, xb = ffn_in(idx)
            act = swiglu(jnp.dot(xb, as_bf16(wg[...]), preferred_element_type=f32),
                         jnp.dot(xb, as_bf16(wu[...]), preferred_element_type=f32))
            ffn_out(act, idx, base, mx, o16)
            late_copies.wait()
            fix_copy(base).start()
            fix_copy(base).wait()
        mark(None)

    lhs_buf = pltpu.VMEM((T // 2, D), u32)
    q_buf = pltpu.VMEM((8, T + padq, 128), f32)
    kv_buf = pltpu.VMEM((8, T + HALO + padk, 128), f32)
    l_buf = pltpu.VMEM((NW, T + padl, 128), f32)
    scratch = [
        pltpu.VMEM((S // 2, D), u32),
        pltpu.VMEM((D // 2, 3 * D), u32),
        pltpu.VMEM((D // 2, 3 * D), u32),
        pltpu.VMEM((NJ, D // 2, 128), u32),
        pltpu.VMEM((D // 2, D), u32),
        pltpu.VMEM((D,), bf16),
        pltpu.VMEM((1280 + 2048 * 7,), bf16),
        pltpu.VMEM((64, D), f32),
        pltpu.VMEM((D // 2, F), u32),
        pltpu.VMEM((D // 2, F), u32),
        pltpu.VMEM((F // 2, D), u32),
        lhs_buf, lhs_buf,
        q_buf, q_buf,
        pltpu.VMEM((64, 128), u32),
        kv_buf, kv_buf,
        pltpu.VMEM((8, 8, 128), f32),
        kv_buf, kv_buf,
        l_buf, l_buf,
        lhs_buf, lhs_buf,
        pltpu.VMEM((S, D), f32),
        pltpu.VMEM((S, D), bf16),
        pltpu.VMEM((128, D), bf16),
        pltpu.SemaphoreType.DMA((3 + NWQ,)),
    ]
    return kernel, scratch


def build(**kw):
    kernel, scratch = make_kernel(**kw)

    def fn(A_x, A_wqkv, A_wo, B_x, B_w_r, B_w_gate, B_w_up, B_w_down):
        x2 = A_x.reshape(S, D)
        out = pl.pallas_call(
            kernel,
            in_specs=[pl.BlockSpec(memory_space=pl.ANY)] * 7,
            out_specs=pl.BlockSpec(memory_space=pl.ANY),
            out_shape=jax.ShapeDtypeStruct((S, D), bf16),
            scratch_shapes=scratch,
            name="fused",
            compiler_params=pltpu.CompilerParams(vmem_limit_bytes=100 * 2**20, disable_bounds_checks=True),
        )(x2, A_wqkv, A_wo, B_w_r, B_w_gate, B_w_up, B_w_down)
        return out.reshape(1, S, D)
    return fn


_fn = build()


@jax.jit
def pallas_sequential_preLN__sliding_local_dilated__moe_arch_mod__prompt_kernel(
    A_x: jax.Array,
    A_wqkv: jax.Array,
    A_wo: jax.Array,
    B_x: jax.Array,
    B_w_r: jax.Array,
    B_w_gate: jax.Array,
    B_w_up: jax.Array,
    B_w_down: jax.Array,
):
    return _fn(A_x, A_wqkv, A_wo, B_x, B_w_r, B_w_gate, B_w_up, B_w_down)
```

```python
import functools
import math
import jax
import jax.numpy as jnp
from jax.experimental import pallas as pl
from jax.experimental.pallas import tpu as pltpu

S, D, H, DH, F = 2048, 640, 32, 20, 1536
NW, DIL = 8, 2
HALO = 16
NJ = D // 128
EPS = 1e-5
QSCALE = (DH ** -0.5) * math.log2(math.e)
f32, bf16, u32, i32 = jnp.float32, jnp.bfloat16, jnp.uint32, jnp.int32


_PV, _QK = (0, 3, 4, 5, 6, 7, 8, 9), (9, 10, 11, 11, 12, 13, 13, 14)
STEP = [
    dict(e=(-1, 1), ed=4, pv=_PV, lag=2, qk=_QK, a=(16, 17), ad=2),
    dict(e=(1, 3), ed=5, pv=_PV, lag=2, qk=_QK, a=(16, 17), ad=2),
    dict(e=(1, 3), ed=5, pv=_PV, lag=2, qk=_QK, a=(16, 17), ad=2),
    dict(e=(1, 3), ed=5, pv=_PV, lag=2, qk=(9, 10, 11, 11, 13, 13, 14, 16), a=(17, 17), ad=2),
]


def interleave(slots, pieces):
    pieces = sorted(pieces, key=lambda kp: kp[0])
    for k, p in pieces:
        if k < 0:
            p()
    for c, s in enumerate(slots):
        s()
        for k, p in pieces:
            if k == c:
                p()
    for k, p in pieces:
        if k >= len(slots):
            p()


def spread(pieces, lo, hi):
    n = len(pieces)
    return [(lo + (k * (hi - lo)) // n, p) for k, p in enumerate(pieces)]


def at(sched, pieces):
    k = len(pieces) // len(sched)
    sched = [c for c in sched for _ in range(k)]
    return list(zip(sched, pieces, strict=True))


def pack2(even, odd):
    p = pltpu.pack_elementwise([even, odd], packed_dtype=bf16)
    return p if p.dtype == u32 else pltpu.bitcast(p, u32)


def as_bf16(x_u32):
    return pltpu.bitcast(x_u32, bf16)


def or_bits(x, g):
    return pltpu.bitcast(pltpu.bitcast(x, u32) | g, f32)


def fold(op, xs, tree):
    xs = list(xs)
    if not tree:
        return functools.reduce(op, xs)
    while len(xs) > 1:
        xs = [op(xs[i], xs[i + 1]) if i + 1 < len(xs) else xs[i] for i in range(0, len(xs), 2)]
    return xs[0]


def rsqrt(v):
    return jnp.exp2(jnp.log(v) * (-0.5 * math.log2(math.e)))


def make_kernel(T=128, LNB=64, unroll=4, NWQ=4, only=None, scopes=False,
                qk_tree=True, sm_tree=False, pv_order='w',
                x_qk=(4, 4, 5, 5, 6, 6, 7, 7),
                y_qk1=(0, 2, 3, 3, 4, 4, 6, 7), y_a=(4, 4), y_ad=1, y_pv0=(5, 6, 7, 8, 9, 10, 11, 12),
                y_pv1=(12, 13, 14, 15, 16, 17, 18, 19), y_pvtok=True,
                z_qk=(0, 1, 1, 2, 4, 4, 6, 7), z_e=(6, 9), z_ed=0, z_a=(10, 11), z_ad=3,
                t_e0=(-1, 2), t_ed0=5, t_pv0=(3, 4, 5, 6, 7, 8, 9, 10), t_qk=(9, 10, 11, 11, 11, 11, 12, 14),
                t_pv=(16, 17, 18, 19, 19, 19, 19, 19), t_pvtok=False, t_e=(21, 22), t_ed=2, t_in=6,
                t_act=(8, 9, 10, 11, 12, 13, 14, 15, 16, 17, 18, 19, 20, 21, 22, 23, 23, 24, 24, 24, 24, 24, 24, 24),
                t_down=(24,),
                padq=8, padl=8, padk=24, **ov):
    NT = S // T
    NG = T // 16

    def kernel(x_hbm, wqkv_hbm, wo_hbm, wr_hbm, wg_hbm, wu_hbm, wd_hbm, out_hbm,
               xs, wraw, wp, woraw, wop, wr, filler, wrf, wg, wu, wd,
               xn0, xn1, qs, qa, zv_, ks, ka, best, vs, va, ls, lsa, os_, osa, hs, outs, fixbuf,
               sems):
        x_u, wqkv_u, wo_u, wg_u, wu_u, wd_u = [r.bitcast(u32) for r in
                                               (x_hbm, wqkv_hbm, wo_hbm, wg_hbm, wu_hbm, wd_hbm)]
        xn, qq, kk = (xn0, xn1), (qs, qa), (ks, ka)

        zv = zv_.at[pl.ds(0, 8)]
        pending = []
        hist = []

        def new_block():
            hist.clear()
            pending.clear()

        def emit_token(val_u32, d=1):
            pending.append((len(hist) + d - 1, val_u32))

        def gated(w_u32):
            due = [v for (c, v) in pending if c <= len(hist)]
            pending[:] = [(c, v) for (c, v) in pending if c > len(hist)]
            if not due:
                return w_u32
            t = due.pop()
            while due:
                t = t | due.pop()
            return jnp.concatenate([w_u32[0:8] | (t & zv[...]), w_u32[8:]], axis=0)

        def zero_of(v):
            return pltpu.bitcast(v, u32) & zv[...]

        def gate_after(lag):
            return zero_of(hist[-1 - lag]) if len(hist) > lag else None

        def row0(i):
            return i * T if isinstance(i, int) else pl.multiple_of(i * T, T)

        def xrows(r, n):
            return pl.ds(r // 2 if isinstance(r, int) else pl.multiple_of(r // 2, 8), n // 2)

        S_A, S_B, S_C = 0, 1, 2
        S_Q = [3 + c for c in range(NWQ)]
        WQR = D // NWQ
        NLAST = 2

        def x_copy(t0, t1, sem):
            rows = pl.ds(t0 * T // 2, (t1 - t0) * T // 2)
            return pltpu.make_async_copy(x_u.at[rows], xs.at[rows], sems.at[sem])

        def w_copy(p, sem):
            return pltpu.make_async_copy(wqkv_u.at[:, pl.ds(p * D, D)], wraw.at[:, pl.ds(p * D, D)], sems.at[sem])

        def wq_copy(c):
            rows = pl.ds(c * WQR // 2, WQR // 2)
            return pltpu.make_async_copy(wqkv_u.at[rows, pl.ds(0, D)], wraw.at[rows, pl.ds(0, D)], sems.at[S_Q[c]])

        x0_copy = x_copy(0, 1, S_A)
        x1_copy = x_copy(1, 2, S_B)
        wk_copy = w_copy(1, S_C)
        grp_wv = [x_copy(2, 3, S_A), w_copy(2, S_A)]
        grp_wo = [pltpu.make_async_copy(wr_hbm, wr, sems.at[S_Q[0]]),
                  x_copy(3, 4, S_Q[0])]
        grp_wo += [pltpu.make_async_copy(wo_u.at[:, pl.ds(j * 128, 128)], woraw.at[j], sems.at[S_Q[0]])
                   for j in range(NJ)]
        xr_copy = x_copy(4, NT, S_Q[1])
        grp_ffn = [pltpu.make_async_copy(wg_u, wg, sems.at[S_B]),
                   pltpu.make_async_copy(wu_u, wu, sems.at[S_B]),
                   pltpu.make_async_copy(wd_u, wd, sems.at[S_B])]

        def o_copy(r, n, late):
            return pltpu.make_async_copy(outs.at[pl.ds(r, n)], out_hbm.at[pl.ds(r, n)],
                                         sems.at[S_B if late else S_C])

        def fix_copy(base):
            return pltpu.make_async_copy(fixbuf.at[pl.ds(0, 16)], out_hbm.at[pl.ds(base, 16)], sems.at[S_A])

        def prep_j(p, j, lo=0, hi=D):
            rows = slice(lo // 2, hi // 2)
            lane = jax.lax.broadcasted_iota(i32, ((hi - lo) // 2, 128), 1)
            r5 = (lane // 4) % 5
            t = wraw[rows, p * D + 4 * 128: p * D + 5 * 128]
            for jj in range(4):
                t = jnp.where(r5 == (j - 2 * jj) % 5, wraw[rows, p * D + jj * 128: p * D + (jj + 1) * 128], t)
            head = (lane % 32) // 2 + 16 * (lane % 2)
            idx = (20 * head + 4 * j + lane // 32) % 128
            wp[rows, p * D + j * 128: p * D + (j + 1) * 128] = jnp.take_along_axis(t, idx, axis=1)

        def with_prep(preps, slots):
            return [lambda f=f, g=g: (f(), g()) for f, g in zip(preps, slots, strict=True)]

        def prep_w(p):
            return [functools.partial(prep_j, p, j) for j in range(NJ)]

        def prep_wo_pieces():
            def piece(j):
                for d in range(0, DH, 2):
                    lo = woraw[j, pl.ds(d // 2, H // 2, stride=DH // 2), :]
                    hi = woraw[j, pl.ds(d // 2 + (DH // 2) * (H // 2), H // 2, stride=DH // 2), :]
                    cols = slice(j * 128, (j + 1) * 128)
                    wop[d * 16:(d + 1) * 16, cols] = (lo & jnp.uint32(0xFFFF)) | (hi << 16)
                    wop[(d + 1) * 16:(d + 2) * 16, cols] = (lo >> 16) | (hi & jnp.uint32(0xFFFF0000))
            return [functools.partial(piece, j) for j in range(NJ)]

        def ln_stats(x):
            m = jnp.sum(x, axis=-1, keepdims=True) * (1.0 / D)
            v = jnp.maximum(jnp.sum(x * x, axis=-1, keepdims=True) * (1.0 / D) - m * m, 0.0)
            return m, rsqrt(v + EPS)

        def a_pieces(i, dst, d=0):
            r = row0(i)

            def piece(b):
                xu = xs[xrows(r + b * LNB, LNB), :]
                ys = []
                for half in range(2):
                    x = pltpu.bitcast((xu & jnp.uint32(0xFFFF0000)) if half else (xu << 16), f32)
                    m, rs = ln_stats(x)
                    ys.append(x * rs - m * rs)
                yu = pack2(ys[0], ys[1])
                dst[b * LNB // 2:(b + 1) * LNB // 2, :] = yu
                if d:
                    for r8 in range(LNB // 16):
                        emit_token(yu[r8 * 8:r8 * 8 + 8, D - 128:D], d)
            return [functools.partial(piece, b) for b in range(T // LNB)]

        def b_slots(p, src, dst, halo=None):
            def slot(j):
                c = p * D + j * 128
                res = jnp.dot(as_bf16(src[...]), as_bf16(gated(wp[:, c:c + 128])), preferred_element_type=f32)
                hist.append(res[0:8])
                if p == 0:
                    dst[j, 0:T, :] = res
                else:
                    dst[j, 0:HALO, :] = jnp.zeros((HALO, 128), f32) if halo is None else halo[j, T:T + HALO, :]
                    dst[j, HALO:HALO + T, :] = res
            return [functools.partial(slot, j) for j in range(NJ)]

        def ld16(ref, j, start):
            return jnp.concatenate([ref[j, pl.ds(start, 8, stride=2), :],
                                    ref[j, pl.ds(start + 1, 8, stride=2), :]], axis=0)

        def times8(x, v8):
            return (x.reshape(2, 8, 128) * v8[None]).reshape(16, 128)

        def qk_pieces(qr, kr, lr, first=False):
            def piece(g16):
                r0 = g16 * 16
                sv = jnp.full((8, 128), QSCALE, f32)
                gate = gate_after(0)
                if gate is not None:
                    sv = or_bits(sv, gate)
                q = [times8(ld16(qr, j, r0), sv) for j in range(NJ)]
                for w in range(NW):
                    if qk_tree:
                        a = fold(jnp.add, [q[j] * ld16(kr, j, HALO + r0 - DIL * w) for j in range(NJ)], True)
                    else:
                        a = None
                        for j in range(NJ):
                            t = q[j] * ld16(kr, j, HALO + r0 - DIL * w)
                            a = t if a is None else a + t
                    a = a + pltpu.roll(a, 64, 1)
                    a = a + pltpu.roll(a, 32, 1)
                    if first and r0 < DIL * w:
                        rows = jax.lax.broadcasted_iota(i32, (16, 128), 0)
                        rows = (rows % 8) * 2 + rows // 8 + r0
                        a = jnp.where(rows >= DIL * w, a, -1e9)
                    lr[w, r0:r0 + 16, :] = a
            return [functools.partial(piece, g) for g in range(NG)]

        def pv_pieces(lr, vr, orf, tok=True, lag=2):
            def piece(g16):
                r0 = g16 * 16
                lw = [lr[w, r0:r0 + 16, :] for w in range(NW)]
                gate = gate_after(lag) if tok else None
                m = fold(jnp.maximum, lw, sm_tree)
                if gate is not None:
                    m = pltpu.bitcast((pltpu.bitcast(m, u32).reshape(2, 8, 128) | gate[None]).reshape(16, 128), f32)
                es = [jnp.exp2(l - m) for l in lw]
                inv = pl.reciprocal(fold(jnp.add, es, sm_tree), approx=True)
                if pv_order == 'w':
                    acc = [None] * NJ
                    for w in range(NW):
                        for j in range(NJ):
                            t = es[w] * ld16(vr, j, HALO + r0 - DIL * w)
                            acc[j] = t if acc[j] is None else acc[j] + t
                for j in range(NJ):
                    if pv_order == 'w':
                        o = acc[j]
                    elif pv_order == 't':
                        o = fold(jnp.add, [es[w] * ld16(vr, j, HALO + r0 - DIL * w) for w in range(NW)], True)
                    else:
                        o = None
                        for w in range(NW):
                            t = es[w] * ld16(vr, j, HALO + r0 - DIL * w)
                            o = t if o is None else o + t
                    o = o * inv
                    ob = pack2(o[0:8], o[8:16])
                    orf[r0 // 2:r0 // 2 + 8, j * 128:(j + 1) * 128] = ob
                    if tok:
                        emit_token(ob)
            return [functools.partial(piece, g) for g in range(NG)]

        def d_slots(i, orf):
            r = row0(i)

            def slot(j):
                cols = slice(j * 128, (j + 1) * 128)
                res = jnp.dot(as_bf16(orf[...]), as_bf16(gated(wop[:, cols])), preferred_element_type=f32)
                hist.append(res[0:8])
                hs[pl.ds(r, T), cols] = res + as_bf16(xs[xrows(r, T), cols]).astype(f32)
            return [functools.partial(slot, j) for j in range(NJ)]

        def e_pieces(i, par, d=0):
            r = row0(i)

            def piece(b):
                rr = r + b * LNB
                h = hs[pl.ds(rr, LNB), :]
                m, rs = ln_stats(h)
                hw = (h.reshape(LNB // 8, 8, D) * wrf[0:8, :][None]).reshape(LNB, D)
                rv_all = (jnp.sum(hw, axis=-1, keepdims=True) - m * wrf[8:9, 0:1]) * rs
                ov = h * (1.0 + rs) - m * rs
                outs[pl.ds(rr, LNB), :] = ov.astype(bf16)
                bv = best[2 * par]
                bi = best[2 * par + 1]
                rows = (jax.lax.broadcasted_iota(i32, (8, 128), 0) + rr).astype(f32)
                for rb in range(LNB // 8):
                    rv = jnp.broadcast_to(rv_all[rb * 8:(rb + 1) * 8, :], (8, 128))
                    upd = rv > bv
                    bv = jnp.where(upd, rv, bv)
                    bi = jnp.where(upd, rows + float(rb * 8), bi)
                if d:
                    for r8 in range(LNB // 8):
                        emit_token(pltpu.bitcast(ov[r8 * 8:r8 * 8 + 8, D - 128:D], u32), d)
                    emit_token(pltpu.bitcast(bv, u32), d)
                best[2 * par] = bv
                best[2 * par + 1] = bi
                late = isinstance(i, int) and i >= NT - NLAST
                if isinstance(i, int) and i == NT - 1:
                    o_copy(rr, LNB, late).start()
                elif b == T // LNB - 1:
                    o_copy(r, T, late).start()
            return [functools.partial(piece, b) for b in range(T // LNB)]

        def step(i, par, pos):
            sc = {k: ov.get(f'{k}{pos}', v) for k, v in STEP[pos % len(STEP)].items()}
            src = xn[1 - par]
            qn, kn, kp = qq[1 - par], kk[1 - par], kk[par]
            interleave(b_slots(0, src, qn) + b_slots(1, src, kn, kp) + d_slots(i, os_) + b_slots(2, src, vs, vs),
                       at(sc['e'], e_pieces(i - 1, par, sc['ed']))
                       + at(sc['pv'], pv_pieces(ls, vs, os_, True, sc['lag']))
                       + at(sc['qk'], qk_pieces(qn, kn, ls))
                       + at(sc['a'], a_pieces(i + 2, xn[par], sc['ad'])))

        def pick():
            bv = jnp.concatenate([best[0], best[2]], axis=0)
            bi = jnp.concatenate([best[1], best[3]], axis=0)
            mx = jnp.max(bv, axis=0, keepdims=True)
            cand = jnp.where(bv == mx, bi, float(S))
            idx_v = jnp.min(cand, axis=0, keepdims=True)
            return jnp.clip(idx_v.astype(i32)[0, 0], 0, S - 1), mx

        def ffn_in(idx, nrows):
            base = pl.multiple_of(jnp.clip(idx >> 4, 0, nrows // 16 - 1) * 16, 16)
            h16 = hs[pl.ds(base, 16), :]
            m16, rs16 = ln_stats(h16)
            hn16 = (h16 - m16) * rs16
            return base, h16 + hn16, hn16.astype(bf16)

        def swiglu(g, u):
            return (g * jax.nn.sigmoid(g) * u).astype(bf16)

        def ffn_out(act, idx, base, mx, o16, y=None):
            if y is None:
                y = jnp.dot(act, as_bf16(wd[...]), preferred_element_type=f32)
            gate = jax.nn.sigmoid(mx[:, 0:1])
            rows16 = jax.lax.broadcasted_iota(i32, (16, D), 0)
            fixbuf[0:16, :] = (o16 + jnp.where(rows16 == idx - base, y * gate, 0.0)).astype(bf16)

        def blk(name, f):
            return f if only is None or name in only else (lambda *a, **k: None)

        cur = [None]

        def mark(name):
            if not scopes:
                return
            if cur[0] is not None:
                cur[0].__exit__(None, None, None)
                cur[0] = None
            if name:
                cur[0] = jax.named_scope(name)
                cur[0].__enter__()

        mark("s0_start")
        x0_copy.start()
        for c in range(NWQ):
            wq_copy(c).start()
        x1_copy.start()
        wk_copy.start()
        zv[...] = jnp.zeros((8, 128), u32)
        filler[pl.ds(0, 1280)] = jnp.zeros((1280,), bf16)
        for par in range(2):
            best[2 * par] = jnp.full((8, 128), -jnp.inf, f32)
            best[2 * par + 1] = jnp.zeros((8, 128), f32)
        x0_copy.wait()
        for p in a_pieces(0, xn[0]):
            p()
        for c in range(NWQ):
            wq_copy(c).wait()
            if c == NWQ - 1:
                for cp in grp_wv:
                    cp.start()
                x1_copy.wait()
                mark('s1_X')
                new_block()
            for j in range(NJ):
                prep_j(0, j, c * WQR, (c + 1) * WQR)
        blk('X', interleave)(b_slots(0, xn[0], qq[0]) + b_slots(0, xn[1], qq[1]),
                             spread(a_pieces(1, xn[1]), 0, 2))
        for c in grp_wo:
            c.start()
        mark('s2_waitWk')
        wk_copy.wait()
        mark('s3_X2')
        new_block()
        blk('X2', interleave)(with_prep(prep_w(1), b_slots(1, xn[0], kk[0])) + b_slots(1, xn[1], kk[1], kk[0]),
                              at(x_qk, qk_pieces(qq[0], kk[0], lsa, True)))
        xr_copy.start()
        mark('s4_waitWv')
        for c in grp_wv:
            c.wait()
        mark('s5_Y')
        new_block()
        blk('Y', interleave)(with_prep(prep_w(2), b_slots(2, xn[0], va)) + b_slots(2, xn[1], vs, va)
                             + b_slots(0, xn[0], qq[0]) + b_slots(1, xn[0], kk[0], kk[1]),
                             at(y_qk1, qk_pieces(qq[1], kk[1], ls))
                             + at(y_a, a_pieces(2, xn[0], y_ad))
                             + at(y_pv0, pv_pieces(lsa, va, osa, y_pvtok))
                             + at(y_pv1, pv_pieces(ls, vs, os_, y_pvtok)))
        for c in grp_ffn:
            c.start()
        mark('s6_waitWo')
        for c in grp_wo:
            c.wait()
        mark('s7_Z')
        new_block()
        wrv = jnp.broadcast_to((wr[...].astype(f32) + filler[pl.ds(0, D)].astype(f32)).reshape(1, D), (8, D))
        wrf[0:8, :] = wrv
        wrf[8:16, :] = jnp.broadcast_to(jnp.sum(wrv, axis=-1, keepdims=True), (8, D))
        blk('Z', interleave)(with_prep(prep_wo_pieces(), d_slots(0, osa)) + d_slots(1, os_)
                             + b_slots(2, xn[0], vs, vs),
                             at(z_qk, qk_pieces(qq[0], kk[0], ls))
                             + at(z_e, e_pieces(0, 0, z_ed))
                             + at(z_a, a_pieces(3, xn[1], z_ad)))

        first = 2
        assert (NT - 2 - first) % unroll == 0 and unroll % 2 == 0

        def body(k, c):
            new_block()
            for u in range(unroll):
                blk('loop', step)(first + k * unroll + u, (first + u) % 2, u)
            return c

        xr_copy.wait()
        mark('s8_loop')
        jax.lax.fori_loop(0, (NT - 2 - first) // unroll, body, 0)
        mark('s9_tail')

        for c in grp_ffn:
            c.wait()
        new_block()
        L = NT - 1
        src = xn[L % 2]
        qn, kn, kp = qq[L % 2], kk[L % 2], kk[1 - L % 2]
        sp = {}

        def sp_in():
            sp['idx'], sp['mx'] = pick()
            sp['base'], sp['o16'], sp['xb'] = ffn_in(sp['idx'], S - NLAST * T)
            sp['act'] = []

        def sp_half(k):
            c0 = (k // 2) * 128
            r = jnp.dot(sp['xb'], as_bf16((wu if k % 2 else wg)[:, c0:c0 + 128]), preferred_element_type=f32)
            if k % 2:
                sp['act'].append(swiglu(sp['g'], r))
            else:
                sp['g'] = r

        def sp_down(kg, j):
            a = jnp.concatenate(sp['act'][4 * kg:4 * kg + 4], axis=1)
            r = jnp.dot(a, as_bf16(wd[kg * 256:(kg + 1) * 256, j * 128:(j + 1) * 128]), preferred_element_type=f32)
            sp['y', j] = r if kg == 0 else sp['y', j] + r

        def sp_out():
            if t_down:
                y = jnp.concatenate([sp['y', j] for j in range(NJ)], axis=1)
                ffn_out(None, sp['idx'], sp['base'], sp['mx'], sp['o16'], y)
            else:
                ffn_out(jnp.concatenate(sp['act'], axis=1), sp['idx'], sp['base'], sp['mx'], sp['o16'])

        blk('tail', interleave)(b_slots(0, src, qn) + b_slots(1, src, kn, kp) + b_slots(2, src, va, vs)
                                + d_slots(L - 1, os_) + d_slots(L, osa),
                                at(t_e0, e_pieces(L - 2, L % 2, t_ed0))
                                + [(t_in, sp_in)]
                                + at(t_pv0, pv_pieces(ls, vs, os_))
                                + at(t_qk, qk_pieces(qn, kn, lsa))
                                + at(t_pv, pv_pieces(lsa, va, osa, t_pvtok))
                                + at(t_act, [functools.partial(sp_half, k) for k in range(2 * F // 128)])
                                + (at(t_down, [functools.partial(sp_down, kg, j) for kg in range(3) for j in range(NJ)])
                                   if t_down else [])
                                + at(t_e, e_pieces(L - 1, (L - 1) % 2, t_ed))
                                + [(25, sp_out)]
                                + spread(e_pieces(L, L % 2), 25, 26))

        mark('sa_final')
        idx, mx = pick()
        o_copy(0, S - NLAST * T, False).wait()
        late_copies = o_copy(S - NLAST * T, NLAST * T, True)
        hit = idx == sp['idx'] if sp else idx < 0

        @pl.when(hit)
        def _():
            fix_copy(sp['base'] if sp else 0).start()
            late_copies.wait()
            fix_copy(sp['base'] if sp else 0).wait()

        @pl.when(jnp.logical_not(hit))
        def _():
            base, o16, xb = ffn_in(idx, S)
            act = swiglu(jnp.dot(xb, as_bf16(wg[...]), preferred_element_type=f32),
                         jnp.dot(xb, as_bf16(wu[...]), preferred_element_type=f32))
            ffn_out(act, idx, base, mx, o16)
            late_copies.wait()
            fix_copy(base).start()
            fix_copy(base).wait()
        mark(None)

    lhs_buf = pltpu.VMEM((T // 2, D), u32)
    q_buf = pltpu.VMEM((8, T + padq, 128), f32)
    kv_buf = pltpu.VMEM((8, T + HALO + padk, 128), f32)
    l_buf = pltpu.VMEM((NW, T + padl, 128), f32)
    scratch = [
        pltpu.VMEM((S // 2, D), u32),
        pltpu.VMEM((D // 2, 3 * D), u32),
        pltpu.VMEM((D // 2, 3 * D), u32),
        pltpu.VMEM((NJ, D // 2, 128), u32),
        pltpu.VMEM((D // 2, D), u32),
        pltpu.VMEM((D,), bf16),
        pltpu.VMEM((1280 + 2048 * 7,), bf16),
        pltpu.VMEM((64, D), f32),
        pltpu.VMEM((D // 2, F), u32),
        pltpu.VMEM((D // 2, F), u32),
        pltpu.VMEM((F // 2, D), u32),
        lhs_buf, lhs_buf,
        q_buf, q_buf,
        pltpu.VMEM((64, 128), u32),
        kv_buf, kv_buf,
        pltpu.VMEM((8, 8, 128), f32),
        kv_buf, kv_buf,
        l_buf, l_buf,
        lhs_buf, lhs_buf,
        pltpu.VMEM((S, D), f32),
        pltpu.VMEM((S, D), bf16),
        pltpu.VMEM((128, D), bf16),
        pltpu.SemaphoreType.DMA((3 + NWQ,)),
    ]
    return kernel, scratch


def build(**kw):
    kernel, scratch = make_kernel(**kw)

    def fn(A_x, A_wqkv, A_wo, B_x, B_w_r, B_w_gate, B_w_up, B_w_down):
        x2 = A_x.reshape(S, D)
        out = pl.pallas_call(
            kernel,
            in_specs=[pl.BlockSpec(memory_space=pl.ANY)] * 7,
            out_specs=pl.BlockSpec(memory_space=pl.ANY),
            out_shape=jax.ShapeDtypeStruct((S, D), bf16),
            scratch_shapes=scratch,
            name="fused",
            compiler_params=pltpu.CompilerParams(vmem_limit_bytes=100 * 2**20, disable_bounds_checks=True),
        )(x2, A_wqkv, A_wo, B_w_r, B_w_gate, B_w_up, B_w_down)
        return out.reshape(1, S, D)
    return fn


_fn = build()


@jax.jit
def pallas_sequential_preLN__sliding_local_dilated__moe_arch_mod__prompt_kernel(
    A_x: jax.Array,
    A_wqkv: jax.Array,
    A_wo: jax.Array,
    B_x: jax.Array,
    B_w_r: jax.Array,
    B_w_gate: jax.Array,
    B_w_up: jax.Array,
    B_w_down: jax.Array,
):
    return _fn(A_x, A_wqkv, A_wo, B_x, B_w_r, B_w_gate, B_w_up, B_w_down)
```

```python
import functools
import math
import jax
import jax.numpy as jnp
from jax.experimental import pallas as pl
from jax.experimental.pallas import tpu as pltpu

S, D, H, DH, F = 2048, 640, 32, 20, 1536
NW, DIL = 8, 2
HALO = 16
NJ = D // 128
EPS = 1e-5
QSCALE = (DH ** -0.5) * math.log2(math.e)
f32, bf16, u32, i32 = jnp.float32, jnp.bfloat16, jnp.uint32, jnp.int32


_PV, _QK = (0, 3, 4, 5, 6, 7, 8, 9), (9, 10, 11, 11, 12, 13, 13, 14)
STEP = [
    dict(e=(-1, 0), ed=4, pv=_PV, lag=2, qk=_QK, a=(16, 17), ad=2),
    dict(e=(1, 3), ed=5, pv=_PV, lag=2, qk=_QK, a=(16, 17), ad=2),
    dict(e=(1, 3), ed=5, pv=_PV, lag=2, qk=(9, 10, 11, 12, 13, 13, 13, 16), a=(16, 17), ad=2),
    dict(e=(1, 3), ed=5, pv=_PV, lag=2, qk=(9, 10, 11, 12, 13, 13, 14, 16), a=(17, 17), ad=2),
]


def interleave(slots, pieces):
    pieces = sorted(pieces, key=lambda kp: kp[0])
    for k, p in pieces:
        if k < 0:
            p()
    for c, s in enumerate(slots):
        s()
        for k, p in pieces:
            if k == c:
                p()
    for k, p in pieces:
        if k >= len(slots):
            p()


def spread(pieces, lo, hi):
    n = len(pieces)
    return [(lo + (k * (hi - lo)) // n, p) for k, p in enumerate(pieces)]


def at(sched, pieces):
    k = len(pieces) // len(sched)
    sched = [c for c in sched for _ in range(k)]
    return list(zip(sched, pieces, strict=True))


def pack2(even, odd):
    p = pltpu.pack_elementwise([even, odd], packed_dtype=bf16)
    return p if p.dtype == u32 else pltpu.bitcast(p, u32)


def as_bf16(x_u32):
    return pltpu.bitcast(x_u32, bf16)


def or_bits(x, g):
    return pltpu.bitcast(pltpu.bitcast(x, u32) | g, f32)


def fold(op, xs, tree):
    xs = list(xs)
    if not tree:
        return functools.reduce(op, xs)
    while len(xs) > 1:
        xs = [op(xs[i], xs[i + 1]) if i + 1 < len(xs) else xs[i] for i in range(0, len(xs), 2)]
    return xs[0]


def rsqrt(v):
    return jnp.exp2(jnp.log(v) * (-0.5 * math.log2(math.e)))


def make_kernel(T=128, LNB=64, unroll=4, WQB=(0, 256, 512, 640), only=None, scopes=False,
                qk_tree=True, sm_tree=False, pv_order='w',
                x_qk=(4, 4, 5, 5, 6, 6, 7, 7),
                y_qk1=(1, 2, 4, 5, 6, 7, 7, 7), y_a=(7, 8), y_ad=1, t_lag=2,
                z_pv0=(0, 1, 2, 3, 4, 5, 6, 6), z_lag0=3, z_pv1=(4, 6, 7, 8, 9, 10, 11, 12), z_lag1=2,
                z_qk=(14, 16, 16, 17, 17, 18, 19, 20), z_e=(17, 18), z_ed=0, z_a=(21, 22), z_ad=2,
                t_e0=(-1, 2), t_ed0=5, t_pv0=(3, 4, 5, 6, 7, 8, 9, 10), t_qk=(9, 10, 10, 11, 11, 11, 12, 14),
                t_pv=(16, 17, 18, 19, 19, 19, 19, 19), t_pvtok=False, t_e=(21, 22), t_ed=2, t_in=6,
                t_act=(8, 9, 10, 11, 12, 13, 14, 15, 16, 17, 18, 19, 20, 21, 22, 23, 23, 24, 24, 24, 24, 24, 24, 24),
                t_down=(24,),
                padq=8, padl=8, padk=24, **ov):
    NT = S // T
    NWQ = len(WQB) - 1
    NG = T // 16

    def kernel(x_hbm, wqkv_hbm, wo_hbm, wr_hbm, wg_hbm, wu_hbm, wd_hbm, out_hbm,
               xs, wraw, wp, woraw, wop, wr, filler, wrf, wg, wu, wd,
               xn0, xn1, qs, qa, zv_, ks, ka, best, vs, va, ls, lsa, os_, osa, hs, outs, fixbuf,
               sems):
        x_u, wqkv_u, wo_u, wg_u, wu_u, wd_u = [r.bitcast(u32) for r in
                                               (x_hbm, wqkv_hbm, wo_hbm, wg_hbm, wu_hbm, wd_hbm)]
        xn, qq, kk = (xn0, xn1), (qs, qa), (ks, ka)

        zv = zv_.at[pl.ds(0, 8)]
        pending = []
        hist = []

        def new_block():
            hist.clear()
            pending.clear()

        def emit_token(val_u32, d=1):
            pending.append((len(hist) + d - 1, val_u32))

        def gated(w_u32):
            due = [v for (c, v) in pending if c <= len(hist)]
            pending[:] = [(c, v) for (c, v) in pending if c > len(hist)]
            if not due:
                return w_u32
            t = due.pop()
            while due:
                t = t | due.pop()
            return jnp.concatenate([w_u32[0:8] | (t & zv[...]), w_u32[8:]], axis=0)

        def zero_of(v):
            return pltpu.bitcast(v, u32) & zv[...]

        def gate_after(lag):
            return zero_of(hist[-1 - lag]) if len(hist) > lag else None

        def row0(i):
            return i * T if isinstance(i, int) else pl.multiple_of(i * T, T)

        def xrows(r, n):
            return pl.ds(r // 2 if isinstance(r, int) else pl.multiple_of(r // 2, 8), n // 2)

        S_A, S_B, S_C = 0, 1, 2
        S_Q = [3 + c for c in range(NWQ)]
        NLAST = 2

        def x_copy(t0, t1, sem):
            rows = pl.ds(t0 * T // 2, (t1 - t0) * T // 2)
            return pltpu.make_async_copy(x_u.at[rows], xs.at[rows], sems.at[sem])

        def w_copy(p, sem):
            return pltpu.make_async_copy(wqkv_u.at[:, pl.ds(p * D, D)], wraw.at[:, pl.ds(p * D, D)], sems.at[sem])

        def wq_copy(c):
            rows = pl.ds(WQB[c] // 2, (WQB[c + 1] - WQB[c]) // 2)
            return pltpu.make_async_copy(wqkv_u.at[rows, pl.ds(0, D)], wraw.at[rows, pl.ds(0, D)], sems.at[S_Q[c]])

        x0_copy = x_copy(0, 1, S_A)
        x1_copy = x_copy(1, 2, S_B)
        wk_copy = w_copy(1, S_C)
        grp_wv = [x_copy(2, 3, S_A), w_copy(2, S_A)]
        grp_wo = [pltpu.make_async_copy(wr_hbm, wr, sems.at[S_Q[0]]),
                  x_copy(3, 4, S_Q[0])]
        grp_wo += [pltpu.make_async_copy(wo_u.at[:, pl.ds(j * 128, 128)], woraw.at[j], sems.at[S_Q[0]])
                   for j in range(NJ)]
        xr_copy = x_copy(4, NT, S_Q[1])
        grp_ffn = [pltpu.make_async_copy(wg_u, wg, sems.at[S_B]),
                   pltpu.make_async_copy(wu_u, wu, sems.at[S_B]),
                   pltpu.make_async_copy(wd_u, wd, sems.at[S_B])]

        def o_copy(r, n, late):
            return pltpu.make_async_copy(outs.at[pl.ds(r, n)], out_hbm.at[pl.ds(r, n)],
                                         sems.at[S_B if late else S_C])

        def fix_copy(base):
            return pltpu.make_async_copy(fixbuf.at[pl.ds(0, 16)], out_hbm.at[pl.ds(base, 16)], sems.at[S_A])

        def prep_j(p, j, lo=0, hi=D):
            rows = slice(lo // 2, hi // 2)
            lane = jax.lax.broadcasted_iota(i32, ((hi - lo) // 2, 128), 1)
            r5 = (lane // 4) % 5
            t = wraw[rows, p * D + 4 * 128: p * D + 5 * 128]
            for jj in range(4):
                t = jnp.where(r5 == (j - 2 * jj) % 5, wraw[rows, p * D + jj * 128: p * D + (jj + 1) * 128], t)
            head = (lane % 32) // 2 + 16 * (lane % 2)
            idx = (20 * head + 4 * j + lane // 32) % 128
            wp[rows, p * D + j * 128: p * D + (j + 1) * 128] = jnp.take_along_axis(t, idx, axis=1)

        def with_prep(preps, slots):
            return [lambda f=f, g=g: (f(), g()) for f, g in zip(preps, slots, strict=True)]

        def prep_w(p):
            return [functools.partial(prep_j, p, j) for j in range(NJ)]

        def prep_wo_pieces():
            def piece(j):
                for d in range(0, DH, 2):
                    lo = woraw[j, pl.ds(d // 2, H // 2, stride=DH // 2), :]
                    hi = woraw[j, pl.ds(d // 2 + (DH // 2) * (H // 2), H // 2, stride=DH // 2), :]
                    cols = slice(j * 128, (j + 1) * 128)
                    wop[d * 16:(d + 1) * 16, cols] = (lo & jnp.uint32(0xFFFF)) | (hi << 16)
                    wop[(d + 1) * 16:(d + 2) * 16, cols] = (lo >> 16) | (hi & jnp.uint32(0xFFFF0000))
            return [functools.partial(piece, j) for j in range(NJ)]

        def ln_stats(x):
            m = jnp.sum(x, axis=-1, keepdims=True) * (1.0 / D)
            v = jnp.maximum(jnp.sum(x * x, axis=-1, keepdims=True) * (1.0 / D) - m * m, 0.0)
            return m, rsqrt(v + EPS)

        def a_pieces(i, dst, d=0):
            r = row0(i)

            def piece(b):
                xu = xs[xrows(r + b * LNB, LNB), :]
                ys = []
                for half in range(2):
                    x = pltpu.bitcast((xu & jnp.uint32(0xFFFF0000)) if half else (xu << 16), f32)
                    m, rs = ln_stats(x)
                    ys.append(x * rs - m * rs)
                yu = pack2(ys[0], ys[1])
                dst[b * LNB // 2:(b + 1) * LNB // 2, :] = yu
                if d:
                    for r8 in range(LNB // 16):
                        emit_token(yu[r8 * 8:r8 * 8 + 8, D - 128:D], d)
            return [functools.partial(piece, b) for b in range(T // LNB)]

        def b_slots(p, src, dst, halo=None):
            def slot(j):
                c = p * D + j * 128
                res = jnp.dot(as_bf16(src[...]), as_bf16(gated(wp[:, c:c + 128])), preferred_element_type=f32)
                hist.append(res[0:8])
                if p == 0:
                    dst[j, 0:T, :] = res
                else:
                    dst[j, 0:HALO, :] = jnp.zeros((HALO, 128), f32) if halo is None else halo[j, T:T + HALO, :]
                    dst[j, HALO:HALO + T, :] = res
            return [functools.partial(slot, j) for j in range(NJ)]

        def ld16(ref, j, start):
            return jnp.concatenate([ref[j, pl.ds(start, 8, stride=2), :],
                                    ref[j, pl.ds(start + 1, 8, stride=2), :]], axis=0)

        def times8(x, v8):
            return (x.reshape(2, 8, 128) * v8[None]).reshape(16, 128)

        def qk_pieces(qr, kr, lr, first=False):
            def piece(g16):
                r0 = g16 * 16
                sv = jnp.full((8, 128), QSCALE, f32)
                gate = gate_after(0)
                if gate is not None:
                    sv = or_bits(sv, gate)
                q = [times8(ld16(qr, j, r0), sv) for j in range(NJ)]
                for w in range(NW):
                    if qk_tree:
                        a = fold(jnp.add, [q[j] * ld16(kr, j, HALO + r0 - DIL * w) for j in range(NJ)], True)
                    else:
                        a = None
                        for j in range(NJ):
                            t = q[j] * ld16(kr, j, HALO + r0 - DIL * w)
                            a = t if a is None else a + t
                    a = a + pltpu.roll(a, 64, 1)
                    a = a + pltpu.roll(a, 32, 1)
                    if first and r0 < DIL * w:
                        rows = jax.lax.broadcasted_iota(i32, (16, 128), 0)
                        rows = (rows % 8) * 2 + rows // 8 + r0
                        a = jnp.where(rows >= DIL * w, a, -1e9)
                    lr[w, r0:r0 + 16, :] = a
            return [functools.partial(piece, g) for g in range(NG)]

        def pv_pieces(lr, vr, orf, tok=True, lag=2):
            def piece(g16):
                r0 = g16 * 16
                lw = [lr[w, r0:r0 + 16, :] for w in range(NW)]
                gate = gate_after(lag) if tok else None
                m = fold(jnp.maximum, lw, sm_tree)
                if gate is not None:
                    m = pltpu.bitcast((pltpu.bitcast(m, u32).reshape(2, 8, 128) | gate[None]).reshape(16, 128), f32)
                es = [jnp.exp2(l - m) for l in lw]
                inv = pl.reciprocal(fold(jnp.add, es, sm_tree), approx=True)
                if pv_order == 'w':
                    acc = [None] * NJ
                    for w in range(NW):
                        for j in range(NJ):
                            t = es[w] * ld16(vr, j, HALO + r0 - DIL * w)
                            acc[j] = t if acc[j] is None else acc[j] + t
                for j in range(NJ):
                    if pv_order == 'w':
                        o = acc[j]
                    elif pv_order == 't':
                        o = fold(jnp.add, [es[w] * ld16(vr, j, HALO + r0 - DIL * w) for w in range(NW)], True)
                    else:
                        o = None
                        for w in range(NW):
                            t = es[w] * ld16(vr, j, HALO + r0 - DIL * w)
                            o = t if o is None else o + t
                    o = o * inv
                    ob = pack2(o[0:8], o[8:16])
                    orf[r0 // 2:r0 // 2 + 8, j * 128:(j + 1) * 128] = ob
                    if tok:
                        emit_token(ob)
            return [functools.partial(piece, g) for g in range(NG)]

        def d_slots(i, orf):
            r = row0(i)

            def slot(j):
                cols = slice(j * 128, (j + 1) * 128)
                res = jnp.dot(as_bf16(orf[...]), as_bf16(gated(wop[:, cols])), preferred_element_type=f32)
                hist.append(res[0:8])
                hs[pl.ds(r, T), cols] = res + as_bf16(xs[xrows(r, T), cols]).astype(f32)
            return [functools.partial(slot, j) for j in range(NJ)]

        def e_pieces(i, par, d=0):
            r = row0(i)

            def piece(b):
                rr = r + b * LNB
                h = hs[pl.ds(rr, LNB), :]
                m, rs = ln_stats(h)
                hw = (h.reshape(LNB // 8, 8, D) * wrf[0:8, :][None]).reshape(LNB, D)
                rv_all = (jnp.sum(hw, axis=-1, keepdims=True) - m * wrf[8:9, 0:1]) * rs
                ov = h * (1.0 + rs) - m * rs
                outs[pl.ds(rr, LNB), :] = ov.astype(bf16)
                bv = best[2 * par]
                bi = best[2 * par + 1]
                rows = (jax.lax.broadcasted_iota(i32, (8, 128), 0) + rr).astype(f32)
                for rb in range(LNB // 8):
                    rv = jnp.broadcast_to(rv_all[rb * 8:(rb + 1) * 8, :], (8, 128))
                    upd = rv > bv
                    bv = jnp.where(upd, rv, bv)
                    bi = jnp.where(upd, rows + float(rb * 8), bi)
                if d:
                    for r8 in range(LNB // 8):
                        emit_token(pltpu.bitcast(ov[r8 * 8:r8 * 8 + 8, D - 128:D], u32), d)
                    emit_token(pltpu.bitcast(bv, u32), d)
                best[2 * par] = bv
                best[2 * par + 1] = bi
                late = isinstance(i, int) and i >= NT - NLAST
                if isinstance(i, int) and i == NT - 1:
                    o_copy(rr, LNB, late).start()
                elif b == T // LNB - 1:
                    o_copy(r, T, late).start()
            return [functools.partial(piece, b) for b in range(T // LNB)]

        def step(i, par, pos):
            sc = {k: ov.get(f'{k}{pos}', v) for k, v in STEP[pos % len(STEP)].items()}
            src = xn[1 - par]
            qn, kn, kp = qq[1 - par], kk[1 - par], kk[par]
            interleave(b_slots(0, src, qn) + b_slots(1, src, kn, kp) + d_slots(i, os_) + b_slots(2, src, vs, vs),
                       at(sc['e'], e_pieces(i - 1, par, sc['ed']))
                       + at(sc['pv'], pv_pieces(ls, vs, os_, True, sc['lag']))
                       + at(sc['qk'], qk_pieces(qn, kn, ls))
                       + at(sc['a'], a_pieces(i + 2, xn[par], sc['ad'])))

        def pick():
            bv = jnp.concatenate([best[0], best[2]], axis=0)
            bi = jnp.concatenate([best[1], best[3]], axis=0)
            mx = jnp.max(bv, axis=0, keepdims=True)
            cand = jnp.where(bv == mx, bi, float(S))
            idx_v = jnp.min(cand, axis=0, keepdims=True)
            return jnp.clip(idx_v.astype(i32)[0, 0], 0, S - 1), mx

        def ffn_in(idx, nrows):
            base = pl.multiple_of(jnp.clip(idx >> 4, 0, nrows // 16 - 1) * 16, 16)
            h16 = hs[pl.ds(base, 16), :]
            m16, rs16 = ln_stats(h16)
            hn16 = (h16 - m16) * rs16
            return base, h16 + hn16, hn16.astype(bf16)

        def swiglu(g, u):
            return (g * jax.nn.sigmoid(g) * u).astype(bf16)

        def ffn_out(act, idx, base, mx, o16, y=None):
            if y is None:
                y = jnp.dot(act, as_bf16(wd[...]), preferred_element_type=f32)
            gate = jax.nn.sigmoid(mx[:, 0:1])
            rows16 = jax.lax.broadcasted_iota(i32, (16, D), 0)
            fixbuf[0:16, :] = (o16 + jnp.where(rows16 == idx - base, y * gate, 0.0)).astype(bf16)

        def blk(name, f):
            return f if only is None or name in only else (lambda *a, **k: None)

        cur = [None]

        def mark(name):
            if not scopes:
                return
            if cur[0] is not None:
                cur[0].__exit__(None, None, None)
                cur[0] = None
            if name:
                cur[0] = jax.named_scope(name)
                cur[0].__enter__()

        mark("s0_start")
        x0_copy.start()
        for c in range(NWQ):
            wq_copy(c).start()
        x1_copy.start()
        wk_copy.start()
        zv[...] = jnp.zeros((8, 128), u32)
        filler[pl.ds(0, 1280)] = jnp.zeros((1280,), bf16)
        for par in range(2):
            best[2 * par] = jnp.full((8, 128), -jnp.inf, f32)
            best[2 * par + 1] = jnp.zeros((8, 128), f32)
        x0_copy.wait()
        for p in a_pieces(0, xn[0]):
            p()
        for c in range(NWQ):
            wq_copy(c).wait()
            if c == NWQ - 1:
                for cp in grp_wv:
                    cp.start()
                x1_copy.wait()
                mark('s1_X')
                new_block()
            for j in range(NJ):
                prep_j(0, j, WQB[c], WQB[c + 1])
        blk('X', interleave)(b_slots(0, xn[0], qq[0]) + b_slots(0, xn[1], qq[1]),
                             spread(a_pieces(1, xn[1]), 0, 2))
        for c in grp_wo:
            c.start()
        mark('s2_waitWk')
        wk_copy.wait()
        mark('s3_X2')
        new_block()
        blk('X2', interleave)(with_prep(prep_w(1), b_slots(1, xn[0], kk[0])) + b_slots(1, xn[1], kk[1], kk[0]),
                              at(x_qk, qk_pieces(qq[0], kk[0], lsa, True)))
        xr_copy.start()
        mark('s4_waitWv')
        for c in grp_wv:
            c.wait()
        mark('s5_Y')
        new_block()
        blk('Y', interleave)(with_prep(prep_w(2), b_slots(2, xn[0], va)) + b_slots(2, xn[1], vs, va),
                             at(y_qk1, qk_pieces(qq[1], kk[1], ls))
                             + at(y_a, a_pieces(2, xn[0], y_ad)))
        for c in grp_ffn:
            c.start()
        mark('s6_waitWo')
        for c in grp_wo:
            c.wait()
        mark('s7_Z')
        new_block()
        wrv = jnp.broadcast_to((wr[...].astype(f32) + filler[pl.ds(0, D)].astype(f32)).reshape(1, D), (8, D))
        wrf[0:8, :] = wrv
        wrf[8:16, :] = jnp.broadcast_to(jnp.sum(wrv, axis=-1, keepdims=True), (8, D))
        blk('Z', interleave)(b_slots(0, xn[0], qq[0]) + b_slots(1, xn[0], kk[0], kk[1])
                             + with_prep(prep_wo_pieces(), d_slots(0, osa)) + d_slots(1, os_)
                             + b_slots(2, xn[0], vs, vs),
                             at(z_pv0, pv_pieces(lsa, va, osa, True, z_lag0))
                             + at(z_pv1, pv_pieces(ls, vs, os_, True, z_lag1))
                             + at(z_qk, qk_pieces(qq[0], kk[0], ls))
                             + at(z_e, e_pieces(0, 0, z_ed))
                             + at(z_a, a_pieces(3, xn[1], z_ad)))

        first = 2
        assert (NT - 2 - first) % unroll == 0 and unroll % 2 == 0

        def body(k, c):
            new_block()
            for u in range(unroll):
                blk('loop', step)(first + k * unroll + u, (first + u) % 2, u)
            return c

        xr_copy.wait()
        mark('s8_loop')
        jax.lax.fori_loop(0, (NT - 2 - first) // unroll, body, 0)
        mark('s9_tail')

        for c in grp_ffn:
            c.wait()
        new_block()
        L = NT - 1
        src = xn[L % 2]
        qn, kn, kp = qq[L % 2], kk[L % 2], kk[1 - L % 2]
        sp = {}

        def sp_in():
            sp['idx'], sp['mx'] = pick()
            sp['base'], sp['o16'], sp['xb'] = ffn_in(sp['idx'], S - NLAST * T)
            sp['act'] = []

        def sp_half(k):
            c0 = (k // 2) * 128
            r = jnp.dot(sp['xb'], as_bf16((wu if k % 2 else wg)[:, c0:c0 + 128]), preferred_element_type=f32)
            if k % 2:
                sp['act'].append(swiglu(sp['g'], r))
            else:
                sp['g'] = r

        def sp_down(kg, j):
            a = jnp.concatenate(sp['act'][4 * kg:4 * kg + 4], axis=1)
            r = jnp.dot(a, as_bf16(wd[kg * 256:(kg + 1) * 256, j * 128:(j + 1) * 128]), preferred_element_type=f32)
            sp['y', j] = r if kg == 0 else sp['y', j] + r

        def sp_out():
            if t_down:
                y = jnp.concatenate([sp['y', j] for j in range(NJ)], axis=1)
                ffn_out(None, sp['idx'], sp['base'], sp['mx'], sp['o16'], y)
            else:
                ffn_out(jnp.concatenate(sp['act'], axis=1), sp['idx'], sp['base'], sp['mx'], sp['o16'])

        blk('tail', interleave)(b_slots(0, src, qn) + b_slots(1, src, kn, kp) + b_slots(2, src, va, vs)
                                + d_slots(L - 1, os_) + d_slots(L, osa),
                                at(t_e0, e_pieces(L - 2, L % 2, t_ed0))
                                + [(t_in, sp_in)]
                                + at(t_pv0, pv_pieces(ls, vs, os_, True, t_lag))
                                + at(t_qk, qk_pieces(qn, kn, lsa))
                                + at(t_pv, pv_pieces(lsa, va, osa, t_pvtok))
                                + at(t_act, [functools.partial(sp_half, k) for k in range(2 * F // 128)])
                                + (at(t_down, [functools.partial(sp_down, kg, j) for kg in range(3) for j in range(NJ)])
                                   if t_down else [])
                                + at(t_e, e_pieces(L - 1, (L - 1) % 2, t_ed))
                                + [(25, sp_out)]
                                + spread(e_pieces(L, L % 2), 25, 26))

        mark('sa_final')
        idx, mx = pick()
        o_copy(0, S - NLAST * T, False).wait()
        late_copies = o_copy(S - NLAST * T, NLAST * T, True)
        hit = idx == sp['idx'] if sp else idx < 0

        @pl.when(hit)
        def _():
            fix_copy(sp['base'] if sp else 0).start()
            late_copies.wait()
            fix_copy(sp['base'] if sp else 0).wait()

        @pl.when(jnp.logical_not(hit))
        def _():
            base, o16, xb = ffn_in(idx, S)
            act = swiglu(jnp.dot(xb, as_bf16(wg[...]), preferred_element_type=f32),
                         jnp.dot(xb, as_bf16(wu[...]), preferred_element_type=f32))
            ffn_out(act, idx, base, mx, o16)
            late_copies.wait()
            fix_copy(base).start()
            fix_copy(base).wait()
        mark(None)

    lhs_buf = pltpu.VMEM((T // 2, D), u32)
    q_buf = pltpu.VMEM((8, T + padq, 128), f32)
    kv_buf = pltpu.VMEM((8, T + HALO + padk, 128), f32)
    l_buf = pltpu.VMEM((NW, T + padl, 128), f32)
    scratch = [
        pltpu.VMEM((S // 2, D), u32),
        pltpu.VMEM((D // 2, 3 * D), u32),
        pltpu.VMEM((D // 2, 3 * D), u32),
        pltpu.VMEM((NJ, D // 2, 128), u32),
        pltpu.VMEM((D // 2, D), u32),
        pltpu.VMEM((D,), bf16),
        pltpu.VMEM((1280 + 2048 * 7,), bf16),
        pltpu.VMEM((64, D), f32),
        pltpu.VMEM((D // 2, F), u32),
        pltpu.VMEM((D // 2, F), u32),
        pltpu.VMEM((F // 2, D), u32),
        lhs_buf, lhs_buf,
        q_buf, q_buf,
        pltpu.VMEM((64, 128), u32),
        kv_buf, kv_buf,
        pltpu.VMEM((8, 8, 128), f32),
        kv_buf, kv_buf,
        l_buf, l_buf,
        lhs_buf, lhs_buf,
        pltpu.VMEM((S, D), f32),
        pltpu.VMEM((S, D), bf16),
        pltpu.VMEM((128, D), bf16),
        pltpu.SemaphoreType.DMA((3 + NWQ,)),
    ]
    return kernel, scratch


def build(**kw):
    kernel, scratch = make_kernel(**kw)

    def fn(A_x, A_wqkv, A_wo, B_x, B_w_r, B_w_gate, B_w_up, B_w_down):
        x2 = A_x.reshape(S, D)
        out = pl.pallas_call(
            kernel,
            in_specs=[pl.BlockSpec(memory_space=pl.ANY)] * 7,
            out_specs=pl.BlockSpec(memory_space=pl.ANY),
            out_shape=jax.ShapeDtypeStruct((S, D), bf16),
            scratch_shapes=scratch,
            name="fused",
            compiler_params=pltpu.CompilerParams(vmem_limit_bytes=100 * 2**20, disable_bounds_checks=True),
        )(x2, A_wqkv, A_wo, B_w_r, B_w_gate, B_w_up, B_w_down)
        return out.reshape(1, S, D)
    return fn


_fn = build()


@jax.jit
def pallas_sequential_preLN__sliding_local_dilated__moe_arch_mod__prompt_kernel(
    A_x: jax.Array,
    A_wqkv: jax.Array,
    A_wo: jax.Array,
    B_x: jax.Array,
    B_w_r: jax.Array,
    B_w_gate: jax.Array,
    B_w_up: jax.Array,
    B_w_down: jax.Array,
):
    return _fn(A_x, A_wqkv, A_wo, B_x, B_w_r, B_w_gate, B_w_up, B_w_down)
```

```python
import functools
import math
import jax
import jax.numpy as jnp
from jax.experimental import pallas as pl
from jax.experimental.pallas import tpu as pltpu

S, D, H, DH, F = 2048, 640, 32, 20, 1536
NW, DIL = 8, 2
HALO = 16
NJ = D // 128
EPS = 1e-5
QSCALE = (DH ** -0.5) * math.log2(math.e)
f32, bf16, u32, i32 = jnp.float32, jnp.bfloat16, jnp.uint32, jnp.int32


_PV, _QK = (0, 3, 4, 5, 6, 7, 8, 9), (9, 10, 11, 11, 12, 13, 13, 14)
STEP = [
    dict(e=(-1, 0), ed=4, pv=_PV, lag=2, qk=_QK, a=(16, 17), ad=2),
    dict(e=(1, 3), ed=5, pv=_PV, lag=2, qk=_QK, a=(16, 17), ad=2),
    dict(e=(1, 3), ed=5, pv=_PV, lag=2, qk=(9, 10, 11, 12, 13, 13, 13, 16), a=(16, 17), ad=2),
    dict(e=(1, 3), ed=5, pv=_PV, lag=2, qk=(9, 10, 11, 12, 13, 13, 14, 16), a=(17, 17), ad=2),
]


def interleave(slots, pieces):
    pieces = sorted(pieces, key=lambda kp: kp[0])
    for k, p in pieces:
        if k < 0:
            p()
    for c, s in enumerate(slots):
        s()
        for k, p in pieces:
            if k == c:
                p()
    for k, p in pieces:
        if k >= len(slots):
            p()


def spread(pieces, lo, hi):
    n = len(pieces)
    return [(lo + (k * (hi - lo)) // n, p) for k, p in enumerate(pieces)]


def at(sched, pieces):
    k = len(pieces) // len(sched)
    sched = [c for c in sched for _ in range(k)]
    return list(zip(sched, pieces, strict=True))


def pack2(even, odd):
    p = pltpu.pack_elementwise([even, odd], packed_dtype=bf16)
    return p if p.dtype == u32 else pltpu.bitcast(p, u32)


def as_bf16(x_u32):
    return pltpu.bitcast(x_u32, bf16)


def or_bits(x, g):
    return pltpu.bitcast(pltpu.bitcast(x, u32) | g, f32)


def tree_sum(xs):
    while len(xs) > 1:
        xs = [xs[i] + xs[i + 1] if i + 1 < len(xs) else xs[i] for i in range(0, len(xs), 2)]
    return xs[0]


def rsqrt(v):
    return jnp.exp2(jnp.log(v) * (-0.5 * math.log2(math.e)))


def make_kernel(T=128, LNB=64, unroll=4, WQB=(0, 256, 512, 640),
                x_qk=(4, 4, 5, 5, 6, 6, 7, 7),
                y_qk1=(1, 2, 4, 5, 6, 7, 7, 7), y_a=(7, 8), y_ad=1, t_lag=2,
                z_pv0=(0, 1, 2, 3, 4, 5, 6, 6), z_lag0=3, z_pv1=(4, 6, 7, 8, 9, 10, 11, 12), z_lag1=2,
                z_qk=(14, 16, 16, 17, 17, 18, 19, 20), z_e=(17, 18), z_ed=0, z_a=(21, 22), z_ad=2,
                t_e0=(-1, 2), t_ed0=5, t_pv0=(3, 4, 5, 6, 7, 8, 9, 10), t_qk=(9, 10, 10, 11, 11, 11, 12, 14),
                t_pv=(16, 17, 18, 19, 19, 19, 19, 19), t_pvtok=False, t_e=(21, 22), t_ed=2, t_in=6,
                t_act=(8, 9, 10, 11, 12, 13, 14, 15, 16, 17, 18, 19, 20, 21, 22, 23, 23, 24, 24, 24, 24, 24, 24, 24),
                padq=8, padl=8, padk=24):
    NT = S // T
    NWQ = len(WQB) - 1
    NG = T // 16

    def kernel(x_hbm, wqkv_hbm, wo_hbm, wr_hbm, wg_hbm, wu_hbm, wd_hbm, out_hbm,
               xs, wraw, wp, woraw, wop, wr, filler, wrf, wg, wu, wd,
               xn0, xn1, qs, qa, zv_, ks, ka, best, vs, va, ls, lsa, os_, osa, hs, outs, fixbuf,
               sems):
        x_u, wqkv_u, wo_u, wg_u, wu_u, wd_u = [r.bitcast(u32) for r in
                                               (x_hbm, wqkv_hbm, wo_hbm, wg_hbm, wu_hbm, wd_hbm)]
        xn, qq, kk = (xn0, xn1), (qs, qa), (ks, ka)

        zv = zv_.at[pl.ds(0, 8)]
        pending = []
        hist = []

        def new_block():
            hist.clear()
            pending.clear()

        def emit_token(val_u32, d=1):
            pending.append((len(hist) + d - 1, val_u32))

        def gated(w_u32):
            due = [v for (c, v) in pending if c <= len(hist)]
            pending[:] = [(c, v) for (c, v) in pending if c > len(hist)]
            if not due:
                return w_u32
            t = due.pop()
            while due:
                t = t | due.pop()
            return jnp.concatenate([w_u32[0:8] | (t & zv[...]), w_u32[8:]], axis=0)

        def zero_of(v):
            return pltpu.bitcast(v, u32) & zv[...]

        def gate_after(lag):
            return zero_of(hist[-1 - lag]) if len(hist) > lag else None

        def row0(i):
            return i * T if isinstance(i, int) else pl.multiple_of(i * T, T)

        def xrows(r, n):
            return pl.ds(r // 2 if isinstance(r, int) else pl.multiple_of(r // 2, 8), n // 2)

        S_A, S_B, S_C = 0, 1, 2
        S_Q = [3 + c for c in range(NWQ)]
        NLAST = 2

        def x_copy(t0, t1, sem):
            rows = pl.ds(t0 * T // 2, (t1 - t0) * T // 2)
            return pltpu.make_async_copy(x_u.at[rows], xs.at[rows], sems.at[sem])

        def w_copy(p, sem):
            return pltpu.make_async_copy(wqkv_u.at[:, pl.ds(p * D, D)], wraw.at[:, pl.ds(p * D, D)], sems.at[sem])

        def wq_copy(c):
            rows = pl.ds(WQB[c] // 2, (WQB[c + 1] - WQB[c]) // 2)
            return pltpu.make_async_copy(wqkv_u.at[rows, pl.ds(0, D)], wraw.at[rows, pl.ds(0, D)], sems.at[S_Q[c]])

        x0_copy = x_copy(0, 1, S_A)
        x1_copy = x_copy(1, 2, S_B)
        wk_copy = w_copy(1, S_C)
        grp_wv = [x_copy(2, 3, S_A), w_copy(2, S_A)]
        grp_wo = [pltpu.make_async_copy(wr_hbm, wr, sems.at[S_Q[0]]),
                  x_copy(3, 4, S_Q[0])]
        grp_wo += [pltpu.make_async_copy(wo_u.at[:, pl.ds(j * 128, 128)], woraw.at[j], sems.at[S_Q[0]])
                   for j in range(NJ)]
        xr_copy = x_copy(4, NT, S_Q[1])
        grp_ffn = [pltpu.make_async_copy(wg_u, wg, sems.at[S_B]),
                   pltpu.make_async_copy(wu_u, wu, sems.at[S_B]),
                   pltpu.make_async_copy(wd_u, wd, sems.at[S_B])]

        def o_copy(r, n, late):
            return pltpu.make_async_copy(outs.at[pl.ds(r, n)], out_hbm.at[pl.ds(r, n)],
                                         sems.at[S_B if late else S_C])

        def fix_copy(base):
            return pltpu.make_async_copy(fixbuf.at[pl.ds(0, 16)], out_hbm.at[pl.ds(base, 16)], sems.at[S_A])

        def prep_j(p, j, lo=0, hi=D):
            rows = slice(lo // 2, hi // 2)
            lane = jax.lax.broadcasted_iota(i32, ((hi - lo) // 2, 128), 1)
            r5 = (lane // 4) % 5
            t = wraw[rows, p * D + 4 * 128: p * D + 5 * 128]
            for jj in range(4):
                t = jnp.where(r5 == (j - 2 * jj) % 5, wraw[rows, p * D + jj * 128: p * D + (jj + 1) * 128], t)
            head = (lane % 32) // 2 + 16 * (lane % 2)
            idx = (20 * head + 4 * j + lane // 32) % 128
            wp[rows, p * D + j * 128: p * D + (j + 1) * 128] = jnp.take_along_axis(t, idx, axis=1)

        def with_prep(preps, slots):
            return [lambda f=f, g=g: (f(), g()) for f, g in zip(preps, slots, strict=True)]

        def prep_w(p):
            return [functools.partial(prep_j, p, j) for j in range(NJ)]

        def prep_wo_pieces():
            def piece(j):
                for d in range(0, DH, 2):
                    lo = woraw[j, pl.ds(d // 2, H // 2, stride=DH // 2), :]
                    hi = woraw[j, pl.ds(d // 2 + (DH // 2) * (H // 2), H // 2, stride=DH // 2), :]
                    cols = slice(j * 128, (j + 1) * 128)
                    wop[d * 16:(d + 1) * 16, cols] = (lo & jnp.uint32(0xFFFF)) | (hi << 16)
                    wop[(d + 1) * 16:(d + 2) * 16, cols] = (lo >> 16) | (hi & jnp.uint32(0xFFFF0000))
            return [functools.partial(piece, j) for j in range(NJ)]

        def ln_stats(x):
            m = jnp.sum(x, axis=-1, keepdims=True) * (1.0 / D)
            v = jnp.maximum(jnp.sum(x * x, axis=-1, keepdims=True) * (1.0 / D) - m * m, 0.0)
            return m, rsqrt(v + EPS)

        def a_pieces(i, dst, d=0):
            r = row0(i)

            def piece(b):
                xu = xs[xrows(r + b * LNB, LNB), :]
                ys = []
                for half in range(2):
                    x = pltpu.bitcast((xu & jnp.uint32(0xFFFF0000)) if half else (xu << 16), f32)
                    m, rs = ln_stats(x)
                    ys.append(x * rs - m * rs)
                yu = pack2(ys[0], ys[1])
                dst[b * LNB // 2:(b + 1) * LNB // 2, :] = yu
                if d:
                    for r8 in range(LNB // 16):
                        emit_token(yu[r8 * 8:r8 * 8 + 8, D - 128:D], d)
            return [functools.partial(piece, b) for b in range(T // LNB)]

        def b_slots(p, src, dst, halo=None):
            def slot(j):
                c = p * D + j * 128
                res = jnp.dot(as_bf16(src[...]), as_bf16(gated(wp[:, c:c + 128])), preferred_element_type=f32)
                hist.append(res[0:8])
                if p == 0:
                    dst[j, 0:T, :] = res
                else:
                    dst[j, 0:HALO, :] = jnp.zeros((HALO, 128), f32) if halo is None else halo[j, T:T + HALO, :]
                    dst[j, HALO:HALO + T, :] = res
            return [functools.partial(slot, j) for j in range(NJ)]

        def ld16(ref, j, start):
            return jnp.concatenate([ref[j, pl.ds(start, 8, stride=2), :],
                                    ref[j, pl.ds(start + 1, 8, stride=2), :]], axis=0)

        def times8(x, v8):
            return (x.reshape(2, 8, 128) * v8[None]).reshape(16, 128)

        def qk_pieces(qr, kr, lr, first=False):
            def piece(g16):
                r0 = g16 * 16
                sv = jnp.full((8, 128), QSCALE, f32)
                gate = gate_after(0)
                if gate is not None:
                    sv = or_bits(sv, gate)
                q = [times8(ld16(qr, j, r0), sv) for j in range(NJ)]
                for w in range(NW):
                    a = tree_sum([q[j] * ld16(kr, j, HALO + r0 - DIL * w) for j in range(NJ)])
                    a = a + pltpu.roll(a, 64, 1)
                    a = a + pltpu.roll(a, 32, 1)
                    if first and r0 < DIL * w:
                        rows = jax.lax.broadcasted_iota(i32, (16, 128), 0)
                        rows = (rows % 8) * 2 + rows // 8 + r0
                        a = jnp.where(rows >= DIL * w, a, -1e9)
                    lr[w, r0:r0 + 16, :] = a
            return [functools.partial(piece, g) for g in range(NG)]

        def pv_pieces(lr, vr, orf, tok=True, lag=2):
            def piece(g16):
                r0 = g16 * 16
                lw = [lr[w, r0:r0 + 16, :] for w in range(NW)]
                gate = gate_after(lag) if tok else None
                m = functools.reduce(jnp.maximum, lw)
                if gate is not None:
                    m = pltpu.bitcast((pltpu.bitcast(m, u32).reshape(2, 8, 128) | gate[None]).reshape(16, 128), f32)
                es = [jnp.exp2(l - m) for l in lw]
                inv = pl.reciprocal(functools.reduce(jnp.add, es), approx=True)
                acc = [None] * NJ
                for w in range(NW):
                    for j in range(NJ):
                        t = es[w] * ld16(vr, j, HALO + r0 - DIL * w)
                        acc[j] = t if acc[j] is None else acc[j] + t
                for j in range(NJ):
                    o = acc[j] * inv
                    ob = pack2(o[0:8], o[8:16])
                    orf[r0 // 2:r0 // 2 + 8, j * 128:(j + 1) * 128] = ob
                    if tok:
                        emit_token(ob)
            return [functools.partial(piece, g) for g in range(NG)]

        def d_slots(i, orf):
            r = row0(i)

            def slot(j):
                cols = slice(j * 128, (j + 1) * 128)
                res = jnp.dot(as_bf16(orf[...]), as_bf16(gated(wop[:, cols])), preferred_element_type=f32)
                hist.append(res[0:8])
                hs[pl.ds(r, T), cols] = res + as_bf16(xs[xrows(r, T), cols]).astype(f32)
            return [functools.partial(slot, j) for j in range(NJ)]

        def e_pieces(i, par, d=0):
            r = row0(i)

            def piece(b):
                rr = r + b * LNB
                h = hs[pl.ds(rr, LNB), :]
                m, rs = ln_stats(h)
                hw = (h.reshape(LNB // 8, 8, D) * wrf[0:8, :][None]).reshape(LNB, D)
                rv_all = (jnp.sum(hw, axis=-1, keepdims=True) - m * wrf[8:9, 0:1]) * rs
                ov = h * (1.0 + rs) - m * rs
                outs[pl.ds(rr, LNB), :] = ov.astype(bf16)
                bv = best[2 * par]
                bi = best[2 * par + 1]
                rows = (jax.lax.broadcasted_iota(i32, (8, 128), 0) + rr).astype(f32)
                for rb in range(LNB // 8):
                    rv = jnp.broadcast_to(rv_all[rb * 8:(rb + 1) * 8, :], (8, 128))
                    upd = rv > bv
                    bv = jnp.where(upd, rv, bv)
                    bi = jnp.where(upd, rows + float(rb * 8), bi)
                if d:
                    for r8 in range(LNB // 8):
                        emit_token(pltpu.bitcast(ov[r8 * 8:r8 * 8 + 8, D - 128:D], u32), d)
                    emit_token(pltpu.bitcast(bv, u32), d)
                best[2 * par] = bv
                best[2 * par + 1] = bi
                late = isinstance(i, int) and i >= NT - NLAST
                if isinstance(i, int) and i == NT - 1:
                    o_copy(rr, LNB, late).start()
                elif b == T // LNB - 1:
                    o_copy(r, T, late).start()
            return [functools.partial(piece, b) for b in range(T // LNB)]

        def step(i, par, pos):
            sc = STEP[pos]
            src = xn[1 - par]
            qn, kn, kp = qq[1 - par], kk[1 - par], kk[par]
            interleave(b_slots(0, src, qn) + b_slots(1, src, kn, kp) + d_slots(i, os_) + b_slots(2, src, vs, vs),
                       at(sc['e'], e_pieces(i - 1, par, sc['ed']))
                       + at(sc['pv'], pv_pieces(ls, vs, os_, True, sc['lag']))
                       + at(sc['qk'], qk_pieces(qn, kn, ls))
                       + at(sc['a'], a_pieces(i + 2, xn[par], sc['ad'])))

        def pick():
            bv = jnp.concatenate([best[0], best[2]], axis=0)
            bi = jnp.concatenate([best[1], best[3]], axis=0)
            mx = jnp.max(bv, axis=0, keepdims=True)
            cand = jnp.where(bv == mx, bi, float(S))
            idx_v = jnp.min(cand, axis=0, keepdims=True)
            return jnp.clip(idx_v.astype(i32)[0, 0], 0, S - 1), mx

        def ffn_in(idx, nrows):
            base = pl.multiple_of(jnp.clip(idx >> 4, 0, nrows // 16 - 1) * 16, 16)
            h16 = hs[pl.ds(base, 16), :]
            m16, rs16 = ln_stats(h16)
            hn16 = (h16 - m16) * rs16
            return base, h16 + hn16, hn16.astype(bf16)

        def swiglu(g, u):
            return (g * jax.nn.sigmoid(g) * u).astype(bf16)

        def ffn_out(y, idx, base, mx, o16):
            gate = jax.nn.sigmoid(mx[:, 0:1])
            rows16 = jax.lax.broadcasted_iota(i32, (16, D), 0)
            fixbuf[0:16, :] = (o16 + jnp.where(rows16 == idx - base, y * gate, 0.0)).astype(bf16)

        x0_copy.start()
        for c in range(NWQ):
            wq_copy(c).start()
        x1_copy.start()
        wk_copy.start()
        zv[...] = jnp.zeros((8, 128), u32)
        filler[pl.ds(0, 1280)] = jnp.zeros((1280,), bf16)
        for par in range(2):
            best[2 * par] = jnp.full((8, 128), -jnp.inf, f32)
            best[2 * par + 1] = jnp.zeros((8, 128), f32)
        x0_copy.wait()
        for p in a_pieces(0, xn[0]):
            p()
        for c in range(NWQ):
            wq_copy(c).wait()
            if c == NWQ - 1:
                for cp in grp_wv:
                    cp.start()
                x1_copy.wait()
                new_block()
            for j in range(NJ):
                prep_j(0, j, WQB[c], WQB[c + 1])
        interleave(b_slots(0, xn[0], qq[0]) + b_slots(0, xn[1], qq[1]),
                             spread(a_pieces(1, xn[1]), 0, 2))
        for c in grp_wo:
            c.start()
        wk_copy.wait()
        new_block()
        interleave(with_prep(prep_w(1), b_slots(1, xn[0], kk[0])) + b_slots(1, xn[1], kk[1], kk[0]),
                              at(x_qk, qk_pieces(qq[0], kk[0], lsa, True)))
        xr_copy.start()
        for c in grp_wv:
            c.wait()
        new_block()
        interleave(with_prep(prep_w(2), b_slots(2, xn[0], va)) + b_slots(2, xn[1], vs, va),
                             at(y_qk1, qk_pieces(qq[1], kk[1], ls))
                             + at(y_a, a_pieces(2, xn[0], y_ad)))
        for c in grp_ffn:
            c.start()
        for c in grp_wo:
            c.wait()
        new_block()
        wrv = jnp.broadcast_to((wr[...].astype(f32) + filler[pl.ds(0, D)].astype(f32)).reshape(1, D), (8, D))
        wrf[0:8, :] = wrv
        wrf[8:16, :] = jnp.broadcast_to(jnp.sum(wrv, axis=-1, keepdims=True), (8, D))
        interleave(b_slots(0, xn[0], qq[0]) + b_slots(1, xn[0], kk[0], kk[1])
                             + with_prep(prep_wo_pieces(), d_slots(0, osa)) + d_slots(1, os_)
                             + b_slots(2, xn[0], vs, vs),
                             at(z_pv0, pv_pieces(lsa, va, osa, True, z_lag0))
                             + at(z_pv1, pv_pieces(ls, vs, os_, True, z_lag1))
                             + at(z_qk, qk_pieces(qq[0], kk[0], ls))
                             + at(z_e, e_pieces(0, 0, z_ed))
                             + at(z_a, a_pieces(3, xn[1], z_ad)))

        first = 2
        assert (NT - 2 - first) % unroll == 0 and unroll % 2 == 0

        def body(k, c):
            new_block()
            for u in range(unroll):
                step(first + k * unroll + u, (first + u) % 2, u)
            return c

        xr_copy.wait()
        jax.lax.fori_loop(0, (NT - 2 - first) // unroll, body, 0)

        for c in grp_ffn:
            c.wait()
        new_block()
        L = NT - 1
        src = xn[L % 2]
        qn, kn, kp = qq[L % 2], kk[L % 2], kk[1 - L % 2]
        sp = {}

        def sp_in():
            sp['idx'], sp['mx'] = pick()
            sp['base'], sp['o16'], sp['xb'] = ffn_in(sp['idx'], S - NLAST * T)
            sp['act'] = []

        def sp_half(k):
            c0 = (k // 2) * 128
            r = jnp.dot(sp['xb'], as_bf16((wu if k % 2 else wg)[:, c0:c0 + 128]), preferred_element_type=f32)
            if k % 2:
                sp['act'].append(swiglu(sp['g'], r))
            else:
                sp['g'] = r

        def sp_down(kg, j):
            a = jnp.concatenate(sp['act'][4 * kg:4 * kg + 4], axis=1)
            r = jnp.dot(a, as_bf16(wd[kg * 256:(kg + 1) * 256, j * 128:(j + 1) * 128]), preferred_element_type=f32)
            sp['y', j] = r if kg == 0 else sp['y', j] + r

        def sp_out():
            y = jnp.concatenate([sp['y', j] for j in range(NJ)], axis=1)
            ffn_out(y, sp['idx'], sp['base'], sp['mx'], sp['o16'])

        interleave(b_slots(0, src, qn) + b_slots(1, src, kn, kp) + b_slots(2, src, va, vs)
                                + d_slots(L - 1, os_) + d_slots(L, osa),
                                at(t_e0, e_pieces(L - 2, L % 2, t_ed0))
                                + [(t_in, sp_in)]
                                + at(t_pv0, pv_pieces(ls, vs, os_, True, t_lag))
                                + at(t_qk, qk_pieces(qn, kn, lsa))
                                + at(t_pv, pv_pieces(lsa, va, osa, t_pvtok))
                                + at(t_act, [functools.partial(sp_half, k) for k in range(2 * F // 128)])
                                + [(24, functools.partial(sp_down, kg, j)) for kg in range(3) for j in range(NJ)]
                                + at(t_e, e_pieces(L - 1, (L - 1) % 2, t_ed))
                                + [(25, sp_out)]
                                + spread(e_pieces(L, L % 2), 25, 26))

        idx, mx = pick()
        o_copy(0, S - NLAST * T, False).wait()
        late_copies = o_copy(S - NLAST * T, NLAST * T, True)
        hit = idx == sp['idx']

        @pl.when(hit)
        def _():
            fix_copy(sp['base']).start()
            late_copies.wait()
            fix_copy(sp['base']).wait()

        @pl.when(jnp.logical_not(hit))
        def _():
            base, o16, xb = ffn_in(idx, S)
            act = swiglu(jnp.dot(xb, as_bf16(wg[...]), preferred_element_type=f32),
                         jnp.dot(xb, as_bf16(wu[...]), preferred_element_type=f32))
            ffn_out(jnp.dot(act, as_bf16(wd[...]), preferred_element_type=f32), idx, base, mx, o16)
            late_copies.wait()
            fix_copy(base).start()
            fix_copy(base).wait()

    lhs_buf = pltpu.VMEM((T // 2, D), u32)
    q_buf = pltpu.VMEM((8, T + padq, 128), f32)
    kv_buf = pltpu.VMEM((8, T + HALO + padk, 128), f32)
    l_buf = pltpu.VMEM((NW, T + padl, 128), f32)
    scratch = [
        pltpu.VMEM((S // 2, D), u32),
        pltpu.VMEM((D // 2, 3 * D), u32),
        pltpu.VMEM((D // 2, 3 * D), u32),
        pltpu.VMEM((NJ, D // 2, 128), u32),
        pltpu.VMEM((D // 2, D), u32),
        pltpu.VMEM((D,), bf16),
        pltpu.VMEM((1280 + 2048 * 7,), bf16),
        pltpu.VMEM((64, D), f32),
        pltpu.VMEM((D // 2, F), u32),
        pltpu.VMEM((D // 2, F), u32),
        pltpu.VMEM((F // 2, D), u32),
        lhs_buf, lhs_buf,
        q_buf, q_buf,
        pltpu.VMEM((64, 128), u32),
        kv_buf, kv_buf,
        pltpu.VMEM((8, 8, 128), f32),
        kv_buf, kv_buf,
        l_buf, l_buf,
        lhs_buf, lhs_buf,
        pltpu.VMEM((S, D), f32),
        pltpu.VMEM((S, D), bf16),
        pltpu.VMEM((128, D), bf16),
        pltpu.SemaphoreType.DMA((3 + NWQ,)),
    ]
    return kernel, scratch


def build(**kw):
    kernel, scratch = make_kernel(**kw)

    def fn(A_x, A_wqkv, A_wo, B_x, B_w_r, B_w_gate, B_w_up, B_w_down):
        x2 = A_x.reshape(S, D)
        out = pl.pallas_call(
            kernel,
            in_specs=[pl.BlockSpec(memory_space=pl.ANY)] * 7,
            out_specs=pl.BlockSpec(memory_space=pl.ANY),
            out_shape=jax.ShapeDtypeStruct((S, D), bf16),
            scratch_shapes=scratch,
            name="fused",
            compiler_params=pltpu.CompilerParams(vmem_limit_bytes=100 * 2**20, disable_bounds_checks=True),
        )(x2, A_wqkv, A_wo, B_w_r, B_w_gate, B_w_up, B_w_down)
        return out.reshape(1, S, D)
    return fn


_fn = build()


@jax.jit
def pallas_sequential_preLN__sliding_local_dilated__moe_arch_mod__prompt_kernel(
    A_x: jax.Array,
    A_wqkv: jax.Array,
    A_wo: jax.Array,
    B_x: jax.Array,
    B_w_r: jax.Array,
    B_w_gate: jax.Array,
    B_w_up: jax.Array,
    B_w_down: jax.Array,
):
    return _fn(A_x, A_wqkv, A_wo, B_x, B_w_r, B_w_gate, B_w_up, B_w_down)
```

```python
import functools
import math
import jax
import jax.numpy as jnp
from jax.experimental import pallas as pl
from jax.experimental.pallas import tpu as pltpu

S, D, H, DH, F = 2048, 640, 32, 20, 1536
NW, DIL = 8, 2
HALO = 16
NJ = D // 128
EPS = 1e-5
QSCALE = (DH ** -0.5) * math.log2(math.e)
f32, bf16, u32, i32 = jnp.float32, jnp.bfloat16, jnp.uint32, jnp.int32


_PV, _QK = (0, 3, 4, 5, 6, 7, 8, 9), (9, 10, 11, 11, 12, 13, 13, 14)
STEP = [
    dict(e=(-1, -1), ed=5, pv=_PV, lag=2, qk=(9, 10, 11, 11, 12, 13, 14, 15), a=(17, 18), ad=2),
    dict(e=(2, 4), ed=5, pv=_PV, lag=4, qk=_QK, a=(15, 19), ad=0),
    dict(e=(1, 3), ed=5, pv=_PV, lag=2, qk=(9, 9, 11, 11, 13, 13, 13, 16), a=(16, 17), ad=2),
    dict(e=(1, 4), ed=5, pv=_PV, lag=2, qk=(9, 10, 11, 11, 12, 13, 14, 16), a=(17, 18), ad=1),
]


def interleave(slots, pieces):
    pieces = sorted(pieces, key=lambda kp: kp[0])
    for k, p in pieces:
        if k < 0:
            p()
    for c, s in enumerate(slots):
        s()
        for k, p in pieces:
            if k == c:
                p()
    for k, p in pieces:
        if k >= len(slots):
            p()


def spread(pieces, lo, hi):
    n = len(pieces)
    return [(lo + (k * (hi - lo)) // n, p) for k, p in enumerate(pieces)]


def at(sched, pieces):
    k = len(pieces) // len(sched)
    sched = [c for c in sched for _ in range(k)]
    return list(zip(sched, pieces, strict=True))


def store_bf16(ref, r0, c0, y):
    n, w = y.shape
    for r in range(0, n, 8):
        ref[(r0 + r) // 2:(r0 + r) // 2 + 4, c0:c0 + w] = pltpu.bitcast(y[r:r + 8].astype(bf16), u32)


def as_bf16(x_u32):
    return pltpu.bitcast(x_u32, bf16)


def or_bits(x, g):
    return pltpu.bitcast(pltpu.bitcast(x, u32) | g, f32)


def tree_sum(xs):
    while len(xs) > 1:
        xs = [xs[i] + xs[i + 1] if i + 1 < len(xs) else xs[i] for i in range(0, len(xs), 2)]
    return xs[0]


def rsqrt(v):
    return jnp.exp2(jnp.log(v) * (-0.5 * math.log2(math.e)))


def make_kernel(T=128, LNB=64, unroll=4, WQB=(0, 256, 512, 640),
                x_qk=(4, 4, 5, 5, 6, 6, 7, 7),
                y_qk1=(1, 4, 4, 5, 6, 7, 7, 7), y_a=(7, 8), y_ad=1, t_lag=3,
                z_pv0=(0, 1, 3, 4, 4, 5, 6, 6), z_lag0=3, z_pv1=(4, 6, 7, 8, 9, 10, 11, 12), z_lag1=2,
                z_qk=(14, 16, 17, 17, 18, 19, 21, 21), z_e=(18, 18), z_ed=0, z_a=(20, 22), z_ad=4,
                t_e0=(-1, 2), t_ed0=6, t_pv0=(3, 4, 5, 6, 8, 9, 9, 10), t_qk=(9, 10, 10, 11, 12, 13, 14, 14),
                t_pv=(16, 18, 18, 19, 19, 19, 19, 19), t_pvtok=False, t_e=(21, 22), t_ed=2, t_in=6,
                t_act=(8, 9, 10, 11, 12, 13, 14, 15, 16, 17, 18, 19, 20, 21, 22, 23, 23, 24, 24, 24, 24, 24, 24, 24),
                padq=8, padl=8, padk=8):
    NT = S // T
    NWQ = len(WQB) - 1
    NG = T // 16

    def kernel(x_hbm, wqkv_hbm, wo_hbm, wr_hbm, wg_hbm, wu_hbm, wd_hbm, out_hbm,
               xs, wraw, wp, woraw, wop, wr, filler, wrf, wg, wu, wd,
               xn0, xn1, qs, qa, zv_, ks, ka, best, vs, va, ls, lsa, os_, osa, hs, outs, fixbuf,
               sems):
        x_u, wqkv_u, wo_u, wg_u, wu_u, wd_u = [r.bitcast(u32) for r in
                                               (x_hbm, wqkv_hbm, wo_hbm, wg_hbm, wu_hbm, wd_hbm)]
        xn, qq, kk = (xn0, xn1), (qs, qa), (ks, ka)

        zv = zv_.at[pl.ds(0, 8)]
        pending = []
        hist = []

        def new_block():
            hist.clear()
            pending.clear()

        def emit_token(val_u32, d=1):
            pending.append((len(hist) + d - 1, val_u32))

        def gated(w_u32):
            due = [v for (c, v) in pending if c <= len(hist)]
            pending[:] = [(c, v) for (c, v) in pending if c > len(hist)]
            if not due:
                return w_u32
            t = due.pop()
            while due:
                t = t | due.pop()
            return jnp.concatenate([w_u32[0:8] | (t & zv[...]), w_u32[8:]], axis=0)

        def zero_of(v):
            return pltpu.bitcast(v, u32) & zv[...]

        def gate_after(lag):
            return zero_of(hist[-1 - lag]) if len(hist) > lag else None

        def row0(i):
            return i * T if isinstance(i, int) else pl.multiple_of(i * T, T)

        def xrows(r, n):
            return pl.ds(r // 2 if isinstance(r, int) else pl.multiple_of(r // 2, 8), n // 2)

        S_A, S_B, S_C = 0, 1, 2
        S_Q = [3 + c for c in range(NWQ)]
        NLAST = 2

        def x_copy(t0, t1, sem):
            rows = pl.ds(t0 * T // 2, (t1 - t0) * T // 2)
            return pltpu.make_async_copy(x_u.at[rows], xs.at[rows], sems.at[sem])

        def w_copy(p, sem):
            return pltpu.make_async_copy(wqkv_u.at[:, pl.ds(p * D, D)], wraw.at[:, pl.ds(p * D, D)], sems.at[sem])

        def wq_copy(c):
            rows = pl.ds(WQB[c] // 2, (WQB[c + 1] - WQB[c]) // 2)
            return pltpu.make_async_copy(wqkv_u.at[rows, pl.ds(0, D)], wraw.at[rows, pl.ds(0, D)], sems.at[S_Q[c]])

        x0_copy = x_copy(0, 1, S_A)
        x1_copy = x_copy(1, 2, S_B)
        wk_copy = w_copy(1, S_C)
        grp_wv = [x_copy(2, 3, S_A), w_copy(2, S_A)]
        grp_wo = [pltpu.make_async_copy(wr_hbm, wr, sems.at[S_Q[0]]),
                  x_copy(3, 4, S_Q[0])]
        grp_wo += [pltpu.make_async_copy(wo_u.at[:, pl.ds(j * 128, 128)], woraw.at[j], sems.at[S_Q[0]])
                   for j in range(NJ)]
        xr_copy = x_copy(4, NT, S_Q[1])
        grp_ffn = [pltpu.make_async_copy(wg_u, wg, sems.at[S_B]),
                   pltpu.make_async_copy(wu_u, wu, sems.at[S_B]),
                   pltpu.make_async_copy(wd_u, wd, sems.at[S_B])]

        def o_copy(r, n, late):
            return pltpu.make_async_copy(outs.at[pl.ds(r, n)], out_hbm.at[pl.ds(r, n)],
                                         sems.at[S_B if late else S_C])

        def fix_copy(base):
            return pltpu.make_async_copy(fixbuf.at[pl.ds(0, 16)], out_hbm.at[pl.ds(base, 16)], sems.at[S_A])

        def prep_j(p, j, lo=0, hi=D):
            rows = slice(lo // 2, hi // 2)
            lane = jax.lax.broadcasted_iota(i32, ((hi - lo) // 2, 128), 1)
            r5 = (lane // 4) % 5
            t = wraw[rows, p * D + 4 * 128: p * D + 5 * 128]
            for jj in range(4):
                t = jnp.where(r5 == (j - 2 * jj) % 5, wraw[rows, p * D + jj * 128: p * D + (jj + 1) * 128], t)
            head = (lane % 32) // 2 + 16 * (lane % 2)
            idx = (20 * head + 4 * j + lane // 32) % 128
            wp[rows, p * D + j * 128: p * D + (j + 1) * 128] = jnp.take_along_axis(t, idx, axis=1)

        def with_prep(preps, slots):
            return [lambda f=f, g=g: (f(), g()) for f, g in zip(preps, slots, strict=True)]

        def prep_w(p):
            return [functools.partial(prep_j, p, j) for j in range(NJ)]

        def prep_wo_pieces():
            def piece(j):
                for d in range(0, DH, 2):
                    lo = woraw[j, pl.ds(d // 2, H // 2, stride=DH // 2), :]
                    hi = woraw[j, pl.ds(d // 2 + (DH // 2) * (H // 2), H // 2, stride=DH // 2), :]
                    cols = slice(j * 128, (j + 1) * 128)
                    wop[d * 16:(d + 1) * 16, cols] = (lo & jnp.uint32(0xFFFF)) | (hi << 16)
                    wop[(d + 1) * 16:(d + 2) * 16, cols] = (lo >> 16) | (hi & jnp.uint32(0xFFFF0000))
            return [functools.partial(piece, j) for j in range(NJ)]

        def ln_stats(x):
            m = jnp.sum(x, axis=-1, keepdims=True) * (1.0 / D)
            v = jnp.maximum(jnp.sum(x * x, axis=-1, keepdims=True) * (1.0 / D) - m * m, 0.0)
            return m, rsqrt(v + EPS)

        def a_pieces(i, dst, d=0):
            r = row0(i)

            def piece(b):
                x = as_bf16(xs[xrows(r + b * LNB, LNB), :]).astype(f32)
                m, rs = ln_stats(x)
                y = x * rs - m * rs
                yu = pltpu.bitcast(y.astype(bf16), u32)
                dst[b * LNB // 2:(b + 1) * LNB // 2, :] = yu
                for r8 in range(LNB // 16) if d else ():
                    emit_token(yu[r8 * 8:r8 * 8 + 8, D - 128:D], d)
            return [functools.partial(piece, b) for b in range(T // LNB)]

        def b_slots(p, src, dst, halo=None):
            def slot(j):
                c = p * D + j * 128
                res = jnp.dot(as_bf16(src[...]), as_bf16(gated(wp[:, c:c + 128])), preferred_element_type=f32)
                hist.append(res[0:8])
                if p == 0:
                    dst[j, 0:T, :] = res
                else:
                    dst[j, 0:HALO, :] = jnp.zeros((HALO, 128), f32) if halo is None else halo[j, T:T + HALO, :]
                    dst[j, HALO:HALO + T, :] = res
            return [functools.partial(slot, j) for j in range(NJ)]

        def ld16(ref, j, start):
            return ref[j, start:start + 16, :]

        def times8(x, v8):
            return (x.reshape(2, 8, 128) * v8[None]).reshape(16, 128)

        def qk_pieces(qr, kr, lr, first=False):
            def piece(g16):
                r0 = g16 * 16
                sv = jnp.full((8, 128), QSCALE, f32)
                gate = gate_after(0)
                if gate is not None:
                    sv = or_bits(sv, gate)
                q = [times8(ld16(qr, j, r0), sv) for j in range(NJ)]
                for w in range(NW):
                    a = tree_sum([q[j] * ld16(kr, j, HALO + r0 - DIL * w) for j in range(NJ)])
                    a = a + pltpu.roll(a, 64, 1)
                    a = a + pltpu.roll(a, 32, 1)
                    if first and r0 < DIL * w:
                        rows = jax.lax.broadcasted_iota(i32, (16, 128), 0)
                        rows = rows + r0
                        a = jnp.where(rows >= DIL * w, a, -1e9)
                    lr[w, r0:r0 + 16, :] = a
            return [functools.partial(piece, g) for g in range(NG)]

        def pv_pieces(lr, vr, orf, tok=True, lag=2):
            def piece(g16):
                r0 = g16 * 16
                lw = [lr[w, r0:r0 + 16, :] for w in range(NW)]
                gate = gate_after(lag) if tok else None
                m = functools.reduce(jnp.maximum, lw)
                if gate is not None:
                    m = pltpu.bitcast((pltpu.bitcast(m, u32).reshape(2, 8, 128) | gate[None]).reshape(16, 128), f32)
                es = [jnp.exp2(l - m) for l in lw]
                inv = pl.reciprocal(functools.reduce(jnp.add, es), approx=True)
                acc = [None] * NJ
                for w in range(NW):
                    for j in range(NJ):
                        t = es[w] * ld16(vr, j, HALO + r0 - DIL * w)
                        acc[j] = t if acc[j] is None else acc[j] + t
                for j in range(NJ):
                    o = acc[j] * inv
                    store_bf16(orf, r0, j * 128, o)
                    ob = pltpu.bitcast(o[8:16], u32)
                    if tok:
                        emit_token(ob)
            return [functools.partial(piece, g) for g in range(NG)]

        def d_slots(i, orf):
            r = row0(i)

            def slot(j):
                cols = slice(j * 128, (j + 1) * 128)
                res = jnp.dot(as_bf16(orf[...]), as_bf16(gated(wop[:, cols])), preferred_element_type=f32)
                hist.append(res[0:8])
                hs[pl.ds(r, T), cols] = res + as_bf16(xs[xrows(r, T), cols]).astype(f32)
            return [functools.partial(slot, j) for j in range(NJ)]

        def e_pieces(i, par, d=0):
            r = row0(i)

            def piece(b):
                rr = r + b * LNB
                h = hs[pl.ds(rr, LNB), :]
                m, rs = ln_stats(h)
                hw = (h.reshape(LNB // 8, 8, D) * wrf[0:8, :][None]).reshape(LNB, D)
                rv_all = (jnp.sum(hw, axis=-1, keepdims=True) - m * wrf[8:9, 0:1]) * rs
                ov = h * (1.0 + rs) - m * rs
                outs[pl.ds(rr, LNB), :] = ov.astype(bf16)
                bv = best[2 * par]
                bi = best[2 * par + 1]
                rows = (jax.lax.broadcasted_iota(i32, (8, 128), 0) + rr).astype(f32)
                for rb in range(LNB // 8):
                    rv = jnp.broadcast_to(rv_all[rb * 8:(rb + 1) * 8, :], (8, 128))
                    upd = rv > bv
                    bv = jnp.where(upd, rv, bv)
                    bi = jnp.where(upd, rows + float(rb * 8), bi)
                if d:
                    for r8 in range(LNB // 8):
                        emit_token(pltpu.bitcast(ov[r8 * 8:r8 * 8 + 8, D - 128:D], u32), d)
                    emit_token(pltpu.bitcast(bv, u32), d)
                best[2 * par] = bv
                best[2 * par + 1] = bi
                late = isinstance(i, int) and i >= NT - NLAST
                if isinstance(i, int) and i == NT - 1:
                    o_copy(rr, LNB, late).start()
                elif b == T // LNB - 1:
                    o_copy(r, T, late).start()
            return [functools.partial(piece, b) for b in range(T // LNB)]

        def step(i, par, pos):
            sc = STEP[pos]
            src = xn[1 - par]
            qn, kn, kp = qq[1 - par], kk[1 - par], kk[par]
            interleave(b_slots(0, src, qn) + b_slots(1, src, kn, kp) + d_slots(i, os_) + b_slots(2, src, vs, vs),
                       at(sc['e'], e_pieces(i - 1, par, sc['ed']))
                       + at(sc['pv'], pv_pieces(ls, vs, os_, True, sc['lag']))
                       + at(sc['qk'], qk_pieces(qn, kn, ls))
                       + at(sc['a'], a_pieces(i + 2, xn[par], sc['ad'])))

        def pick():
            bv = jnp.concatenate([best[0], best[2]], axis=0)
            bi = jnp.concatenate([best[1], best[3]], axis=0)
            mx = jnp.max(bv, axis=0, keepdims=True)
            cand = jnp.where(bv == mx, bi, float(S))
            idx_v = jnp.min(cand, axis=0, keepdims=True)
            return jnp.clip(idx_v.astype(i32)[0, 0], 0, S - 1), mx

        def ffn_in(idx, nrows):
            base = pl.multiple_of(jnp.clip(idx >> 4, 0, nrows // 16 - 1) * 16, 16)
            h16 = hs[pl.ds(base, 16), :]
            m16, rs16 = ln_stats(h16)
            hn16 = (h16 - m16) * rs16
            return base, h16 + hn16, hn16.astype(bf16)

        def swiglu(g, u):
            return (g * jax.nn.sigmoid(g) * u).astype(bf16)

        def ffn_out(y, idx, base, mx, o16):
            gate = jax.nn.sigmoid(mx[:, 0:1])
            rows16 = jax.lax.broadcasted_iota(i32, (16, D), 0)
            fixbuf[0:16, :] = (o16 + jnp.where(rows16 == idx - base, y * gate, 0.0)).astype(bf16)

        x0_copy.start()
        for c in range(NWQ):
            wq_copy(c).start()
        x1_copy.start()
        wk_copy.start()
        zv[...] = jnp.zeros((8, 128), u32)
        filler[pl.ds(0, 1280)] = jnp.zeros((1280,), bf16)
        for par in range(2):
            best[2 * par] = jnp.full((8, 128), -jnp.inf, f32)
            best[2 * par + 1] = jnp.zeros((8, 128), f32)
        x0_copy.wait()
        for p in a_pieces(0, xn[0]):
            p()
        for c in range(NWQ):
            wq_copy(c).wait()
            if c == NWQ - 1:
                for cp in grp_wv:
                    cp.start()
                x1_copy.wait()
                new_block()
            for j in range(NJ):
                prep_j(0, j, WQB[c], WQB[c + 1])
        interleave(b_slots(0, xn[0], qq[0]) + b_slots(0, xn[1], qq[1]),
                             spread(a_pieces(1, xn[1]), 0, 2))
        for c in grp_wo:
            c.start()
        wk_copy.wait()
        new_block()
        interleave(with_prep(prep_w(1), b_slots(1, xn[0], kk[0])) + b_slots(1, xn[1], kk[1], kk[0]),
                              at(x_qk, qk_pieces(qq[0], kk[0], lsa, True)))
        xr_copy.start()
        for c in grp_wv:
            c.wait()
        new_block()
        interleave(with_prep(prep_w(2), b_slots(2, xn[0], va)) + b_slots(2, xn[1], vs, va),
                             at(y_qk1, qk_pieces(qq[1], kk[1], ls))
                             + at(y_a, a_pieces(2, xn[0], y_ad)))
        for c in grp_ffn:
            c.start()
        for c in grp_wo:
            c.wait()
        new_block()
        wrv = jnp.broadcast_to((wr[...].astype(f32) + filler[pl.ds(0, D)].astype(f32)).reshape(1, D), (8, D))
        wrf[0:8, :] = wrv
        wrf[8:16, :] = jnp.broadcast_to(jnp.sum(wrv, axis=-1, keepdims=True), (8, D))
        interleave(b_slots(0, xn[0], qq[0]) + b_slots(1, xn[0], kk[0], kk[1])
                             + with_prep(prep_wo_pieces(), d_slots(0, osa)) + d_slots(1, os_)
                             + b_slots(2, xn[0], vs, vs),
                             at(z_pv0, pv_pieces(lsa, va, osa, True, z_lag0))
                             + at(z_pv1, pv_pieces(ls, vs, os_, True, z_lag1))
                             + at(z_qk, qk_pieces(qq[0], kk[0], ls))
                             + at(z_e, e_pieces(0, 0, z_ed))
                             + at(z_a, a_pieces(3, xn[1], z_ad)))

        first = 2
        assert (NT - 2 - first) % unroll == 0 and unroll % 2 == 0

        def body(k, c):
            new_block()
            for u in range(unroll):
                step(first + k * unroll + u, (first + u) % 2, u)
            return c

        xr_copy.wait()
        jax.lax.fori_loop(0, (NT - 2 - first) // unroll, body, 0)

        for c in grp_ffn:
            c.wait()
        new_block()
        L = NT - 1
        src = xn[L % 2]
        qn, kn, kp = qq[L % 2], kk[L % 2], kk[1 - L % 2]
        sp = {}

        def sp_in():
            sp['idx'], sp['mx'] = pick()
            sp['base'], sp['o16'], sp['xb'] = ffn_in(sp['idx'], S - NLAST * T)
            sp['act'] = []

        def sp_half(k):
            c0 = (k // 2) * 128
            r = jnp.dot(sp['xb'], as_bf16((wu if k % 2 else wg)[:, c0:c0 + 128]), preferred_element_type=f32)
            if k % 2:
                sp['act'].append(swiglu(sp['g'], r))
            else:
                sp['g'] = r

        def sp_down(kg, j):
            a = jnp.concatenate(sp['act'][4 * kg:4 * kg + 4], axis=1)
            r = jnp.dot(a, as_bf16(wd[kg * 256:(kg + 1) * 256, j * 128:(j + 1) * 128]), preferred_element_type=f32)
            sp['y', j] = r if kg == 0 else sp['y', j] + r

        def sp_out():
            y = jnp.concatenate([sp['y', j] for j in range(NJ)], axis=1)
            ffn_out(y, sp['idx'], sp['base'], sp['mx'], sp['o16'])

        interleave(b_slots(0, src, qn) + b_slots(1, src, kn, kp) + b_slots(2, src, va, vs)
                                + d_slots(L - 1, os_) + d_slots(L, osa),
                                at(t_e0, e_pieces(L - 2, L % 2, t_ed0))
                                + [(t_in, sp_in)]
                                + at(t_pv0, pv_pieces(ls, vs, os_, True, t_lag))
                                + at(t_qk, qk_pieces(qn, kn, lsa))
                                + at(t_pv, pv_pieces(lsa, va, osa, t_pvtok))
                                + at(t_act, [functools.partial(sp_half, k) for k in range(2 * F // 128)])
                                + [(24, functools.partial(sp_down, kg, j)) for kg in range(3) for j in range(NJ)]
                                + at(t_e, e_pieces(L - 1, (L - 1) % 2, t_ed))
                                + [(25, sp_out)]
                                + spread(e_pieces(L, L % 2), 25, 26))

        idx, mx = pick()
        o_copy(0, S - NLAST * T, False).wait()
        late_copies = o_copy(S - NLAST * T, NLAST * T, True)
        hit = idx == sp['idx']

        def on_hit():
            fix_copy(sp['base']).start()
            late_copies.wait()
            fix_copy(sp['base']).wait()

        def on_miss():
            base, o16, xb = ffn_in(idx, S)
            act = swiglu(jnp.dot(xb, as_bf16(wg[...]), preferred_element_type=f32),
                         jnp.dot(xb, as_bf16(wu[...]), preferred_element_type=f32))
            ffn_out(jnp.dot(act, as_bf16(wd[...]), preferred_element_type=f32), idx, base, mx, o16)
            late_copies.wait()
            fix_copy(base).start()
            fix_copy(base).wait()

        jax.lax.cond(hit, on_hit, on_miss)

    lhs_buf = pltpu.VMEM((T // 2, D), u32)
    q_buf = pltpu.VMEM((8, T + padq, 128), f32)
    kv_buf = pltpu.VMEM((8, T + HALO + padk, 128), f32)
    l_buf = pltpu.VMEM((NW, T + padl, 128), f32)
    scratch = [
        pltpu.VMEM((S // 2, D), u32),
        pltpu.VMEM((D // 2, 3 * D), u32),
        pltpu.VMEM((D // 2, 3 * D), u32),
        pltpu.VMEM((NJ, D // 2, 128), u32),
        pltpu.VMEM((D // 2, D), u32),
        pltpu.VMEM((D,), bf16),
        pltpu.VMEM((1280 + 2048 * 7,), bf16),
        pltpu.VMEM((64, D), f32),
        pltpu.VMEM((D // 2, F), u32),
        pltpu.VMEM((D // 2, F), u32),
        pltpu.VMEM((F // 2, D), u32),
        lhs_buf, lhs_buf,
        q_buf, q_buf,
        pltpu.VMEM((64, 128), u32),
        kv_buf, kv_buf,
        pltpu.VMEM((8, 8, 128), f32),
        kv_buf, kv_buf,
        l_buf, l_buf,
        lhs_buf, lhs_buf,
        pltpu.VMEM((S, D), f32),
        pltpu.VMEM((S, D), bf16),
        pltpu.VMEM((128, D), bf16),
        pltpu.SemaphoreType.DMA((3 + NWQ,)),
    ]
    return kernel, scratch


def build(**kw):
    kernel, scratch = make_kernel(**kw)

    def fn(A_x, A_wqkv, A_wo, B_x, B_w_r, B_w_gate, B_w_up, B_w_down):
        x2 = A_x.reshape(S, D)
        out = pl.pallas_call(
            kernel,
            in_specs=[pl.BlockSpec(memory_space=pl.ANY)] * 7,
            out_specs=pl.BlockSpec(memory_space=pl.ANY),
            out_shape=jax.ShapeDtypeStruct((S, D), bf16),
            scratch_shapes=scratch,
            name="fused",
            compiler_params=pltpu.CompilerParams(vmem_limit_bytes=100 * 2**20, disable_bounds_checks=True),
        )(x2, A_wqkv, A_wo, B_w_r, B_w_gate, B_w_up, B_w_down)
        return out.reshape(1, S, D)
    return fn


_fn = build()


@jax.jit
def pallas_sequential_preLN__sliding_local_dilated__moe_arch_mod__prompt_kernel(
    A_x: jax.Array,
    A_wqkv: jax.Array,
    A_wo: jax.Array,
    B_x: jax.Array,
    B_w_r: jax.Array,
    B_w_gate: jax.Array,
    B_w_up: jax.Array,
    B_w_down: jax.Array,
):
    return _fn(A_x, A_wqkv, A_wo, B_x, B_w_r, B_w_gate, B_w_up, B_w_down)
```
